```python
import jax
import jax.numpy as jnp

def _softmax(x, axis=-1):
    return jax.nn.softmax(x, axis=axis)
def _gelu(x):
    return jax.nn.gelu(x, approximate=True)
def _silu(x):
    return jax.nn.silu(x)
def _sigmoid(x):
    return jax.nn.sigmoid(x)
def _layernorm(x, axis=-1, eps=1e-5):
    m = jnp.mean(x, axis=axis, keepdims=True)
    v = jnp.var(x, axis=axis, keepdims=True)
    return (x - m) / jnp.sqrt(v + eps)
def _scatter_add(tgt, idx, src, axis=0):
    return tgt.at[idx].add(src)
def _segment_sum(src, seg, n):
    return jax.ops.segment_sum(src, seg, n)
class _Rng:
    def __init__(self, key):
        self._k = key
    def _next(self):
        self._k, sub = jax.random.split(self._k)
        return sub
    def normal(self, shape):
        return jax.random.normal(self._next(), shape, dtype=jnp.bfloat16)
    def randint(self, lo, hi, shape):
        return jax.random.randint(self._next(), shape, lo, hi, dtype=jnp.int32)
    def uniform(self, shape, lo=0.0, hi=1.0):
        return jax.random.uniform(self._next(), shape, jnp.bfloat16, lo, hi)
    def permutation(self, n):
        return jax.random.permutation(self._next(), n)


kernel_name = 'sequential_preLN__sliding_local_dilated__moe_arch_mod__prompt'

def setup_inputs():
    _rng = _Rng(jax.random.key(int.from_bytes(__import__("os").urandom(4), "little")))
    _w = (lambda a: (lambda t: t.astype(jnp.bfloat16) if jnp.issubdtype(t.dtype, jnp.floating) else t)(jnp.asarray(a)))
    def _A_setup():
        B, S, D = 1, 2048, 640
        return {
            "x": _w((lambda *s: _rng.normal(s) * 0.05)(B, S, D)),
            "wqkv": _w((lambda *s: _rng.normal(s) * 0.05)(D, 3 * D)),
            "wo": _w((lambda *s: _rng.normal(s) * 0.05)(D, D)),
        }
    _A_in = _A_setup()

    def _B_setup():
        B, S, D, F, C = 1, 2048, 640, 1536, 1
        return {
            "x": _w((lambda *s: _rng.normal(s) * 0.05)(B, S, D)),
            "w_r": _w((lambda *s: _rng.normal(s) * 0.05)(D)),
            "w_gate": _w((lambda *s: _rng.normal(s) * 0.05)(D, F)),
            "w_up": _w((lambda *s: _rng.normal(s) * 0.05)(D, F)),
            "w_down": _w((lambda *s: _rng.normal(s) * 0.05)(F, D)),
        }
    _B_in = _B_setup()

    return {
        "A_x": _A_in["x"],
        "A_wqkv": _A_in["wqkv"],
        "A_wo": _A_in["wo"],
        "B_x": _B_in["x"],
        "B_w_r": _B_in["w_r"],
        "B_w_gate": _B_in["w_gate"],
        "B_w_up": _B_in["w_up"],
        "B_w_down": _B_in["w_down"],
    }

def reference(A_x, A_wqkv, A_wo, B_x, B_w_r, B_w_gate, B_w_up, B_w_down):
    def _A_ref(x, wqkv, wo):
        B, S, D = x.shape
        H = 32; Dh = D // H
        W, dil = 8, 2
        qkv = (lambda x, *d: x.transpose(*d))((x @ wqkv).reshape(B, S, 3, H, Dh), 2, 0, 3, 1, 4)
        q, k, v = qkv[0], qkv[1], qkv[2]
        scale = Dh ** -0.5
        pos = jnp.arange(S)
        off = jnp.arange(W) * dil
        idx = pos[:, None] - off[None, :]
        mask = idx >= 0
        idx_c = jnp.where(mask, idx, 0).reshape(-1)
        kg = k[:, :, idx_c, :].reshape(B, H, S, W, Dh)
        vg = v[:, :, idx_c, :].reshape(B, H, S, W, Dh)
        logits = jnp.einsum("bhsd,bhswd->bhsw", q, kg) * scale
        logits = jnp.where(mask[None, None, :, :], logits, -1e9)
        attn = _softmax(logits, axis=-1)
        o = jnp.einsum("bhsw,bhswd->bhsd", attn, vg)
        return (lambda x, *d: x.transpose(*d))(o, 0, 2, 1, 3).reshape(B, S, D) @ wo

    def _B_ref(x, w_r, w_gate, w_up, w_down):
        B, S, D = x.shape
        C = 1
        r = x @ w_r
        idx = jnp.argsort(-r, axis=-1)[:, :C]
        idx_e = jnp.repeat(idx.reshape(B, C, 1), D, axis=2)
        x_sel = jnp.take_along_axis(x, idx_e, axis=1)
        g = _silu(x_sel @ w_gate)
        u = x_sel @ w_up
        y = (g * u) @ w_down
        r_sel = _sigmoid(jnp.take_along_axis(r, idx, axis=1))
        y = y * r_sel.reshape(B, C, 1)
        b_off = (jnp.arange(B) * S).reshape(B, 1)
        flat_idx = (idx + b_off).reshape(B * C)
        zero = (x * 0.0).reshape(B * S, D)
        upd = _scatter_add(zero, flat_idx, y.reshape(B * C, D), axis=0)
        return x + upd.reshape(B, S, D)

    x = A_x
    h = x + _A_ref(_layernorm(x, axis=-1), A_wqkv, A_wo)
    h2 = h + _B_ref(_layernorm(h, axis=-1), B_w_r, B_w_gate, B_w_up, B_w_down)
    return h2
```

```python
import functools
import math
import jax
import jax.numpy as jnp
from jax import lax
import jax.experimental.pallas as pl
import jax.experimental.pallas.tpu as pltpu

S, D, F = 2048, 640, 1536
H, DH, W, DIL = 32, 20, 8, 2
NT = D // 128
HALO = 16
EPS = 1e-5
F32, BF16, U32 = jnp.float32, jnp.bfloat16, jnp.uint32
QSCALE = DH ** -0.5 * math.log2(math.e)
R = 16
T = 128
NS = S // T
NC = T // R


def _or_all(u):
    t = None
    for i in range(u.shape[0] // 8):
        for j in range(u.shape[1] // 128):
            p = u[8 * i:8 * i + 8, 128 * j:128 * (j + 1)]
            t = p if t is None else t | p
    return t


def _tree(f, xs):
    xs = list(xs)
    while len(xs) > 1:
        xs = [f(xs[i], xs[i + 1]) for i in range(0, len(xs) - 1, 2)] + ([xs[-1]] if len(xs) % 2 else [])
    return xs[0]


def interleave(segs, tasks):
    out = []
    tasks = sorted(tasks, key=lambda t: t[0])
    i = 0
    pos = 0
    for sg in segs:
        n = (sg[-1] - sg[-2]) // 16
        while i < len(tasks) and tasks[i][0] < pos + n:
            out.append(tasks[i][1] + (max(tasks[i][0] - pos, 0),))
            i += 1
        out.append(sg)
        pos += n
    out += [t[1] + (0,) for t in tasks[i:]]
    return out


def build_program(C0, CP, LS, SO, PO, PS, EDL, ADL, RL, SPEC, GL, GS, PRE, TL):
    def B(b, g):
        return [("B", b, n, 0, T) for n in range(NT * g, NT * g + NT)]

    def Dm(b, lo=0, hi=T):
        return [("D", b, n, lo, hi) for n in range(NT)]

    def parts(kind, b, dls, lo=0, hi=T):
        n = (hi - lo) // len(dls)
        return [(8 * dl, (kind, b, lo + i * n, lo + (i + 1) * n)) for i, dl in enumerate(dls)]

    def LSt(b, c0, cp, chunks=range(NC)):
        t = []
        for i, c in enumerate(chunks):
            base = c0 + cp * i
            for h in range(0, R, RL):
                sh = -(R - RL - h) * cp / R
                t += [(int(base + sh + LS * w), ("L", b, c, h, w, GL)) for w in range(W)]
                t += [(int(base + sh + SO), ("S", b, c, h, GS))]
        return t

    def Pt(b, c0, cp, chunks=range(NC)):
        t = []
        for i, c in enumerate(chunks):
            t += [(int(c0 + cp * i + PS * j), ("P", b, c, j, True)) for j in range(NT)]
        return t

    def Cf(b, c0=C0, cp=CP):
        return LSt(b, c0, cp) + Pt(b, c0 + PO, cp)

    p = [("wait", "x0")] + [("A", b, 0, T, 0) for b in range(3)]
    p += [("wait", "wq"), ("perm", 0)] + B(0, 0) + B(1, 0)
    p += [("wait", "wk"), ("perm", 1)]
    p += interleave(B(2, 0) + B(0, 1) + B(1, 1), LSt(0, 999, 0))
    p += [("wait", "wv"), ("perm", 2)]
    p += interleave(B(2, 1) + B(0, 2) + B(1, 2), LSt(1, 60, 6) + Pt(0, 999, 0))
    p += [("wait", "wo"), ("wait", "wr"), ("wait", "x1"), ("permo",)]
    p += interleave(B(2, 2) + Dm(0) + Dm(1) + B(3, 0) + B(3, 1) + B(3, 2),
                    Pt(1, 36, 5) + parts("A", 3, (13,)) + parts("E", 0, (16, 19)) + parts("E", 1, (22, 25))
                    + Cf(2, 84, 17.5) + parts("A", 4, (20, 28)))
    for s in range(3, NS - 2):
        segs = Dm(s - 1) + B(s + 1, 0) + B(s + 1, 1) + B(s + 1, 2)
        tasks = parts("E", s - 1, EDL) + Cf(s)
        if s == 7:
            pre = [t for t in tasks if t[1][0] in "LS" and t[1][2] < PRE]
            tasks = [t for t in tasks if t not in pre]
            p += [t[1] + (0,) for t in pre]
            p += [("wait", "x2"), ("wait", "ffn")]
        if s + 2 < NS:
            tasks += parts("A", s + 2, ADL)
        p += interleave(segs, tasks)
    s = NS - 2
    big = Dm(s - 1) + B(s + 1, 0) + B(s + 1, 1) + B(s + 1, 2) + Dm(s)
    small = [("G", k, n, 0, 0) for n in range(F // 128) for k in range(2)] if SPEC else []
    segs = []
    for g, sg in enumerate(big):
        segs.append(sg)
        if g >= 12:
            k = 2 if g % 4 else 1
            segs += small[:k]
            small = small[k:]
    segs += small
    segs += Dm(s + 1, 0, T // 2) + Dm(s + 1, T // 2, T)
    tasks = (parts("E", s - 1, (9, 11)) + ([(8 * 12, ("spec",))] if SPEC else [])
             + Cf(s, 14, 13.5) + LSt(s + 1, 136, 4) + Pt(s + 1, 170, 3.5)
             + parts("E", s, (28, 31)) + parts("E", s + 1, (99,), 0, T // 2))
    p += interleave(segs, tasks)
    if SPEC:
        p += [("H", n) for n in range(NT)]
    p += [("E", s + 1, T // 2, T, 0)]
    return p


def make_kernel(C0=16, CP=17.5, LS=0, SO=8, PO=10, PS=1, EDL=(12, 18), ADL=(7, 16), X0=384, X1=896,
                prof=0, pins=1, RL=16, FA=3, FS=0, SPEC=1, ALT=1, HD=1, GL=1, GS=1, PRE=2, TL=(), G=2):
    XCH = (X0, X1, S - X0 - X1)
    prog = build_program(C0, CP, LS, SO, PO, PS, EDL, ADL, RL, SPEC, GL, GS, PRE, TL)

    def wait(c, name):
        if prof:
            with jax.named_scope("w_" + name):
                c.wait()
        else:
            c.wait()

    def kernel(x_hbm, wqkv_hbm, wo_hbm, wr_hbm, wg_hbm, wu_hbm, wd_hbm, out_hbm,
               x_s, wqkv_s, wo_s, wr_s, wg_s, wu_s, wd_s, wp_s, wop_s,
               k_s, v_s, xn_s, o_s, hn_s, out_s, y_s, sem_in, sem_out):
        pid = pl.program_id(0)
        step = pid - (1 if G == 2 else 0)
        cp = {}
        semi = dict(x0=0, wq=1, wk=2, wv=3, wo=4, wr=4, x1=4, x2=5, ffn=5)
        r0 = 0
        for i, n in enumerate(XCH):
            nm = "x%d" % i
            cp[nm] = [pltpu.make_async_copy(x_hbm.at[pl.ds(r0, n)], x_s.at[pl.ds(r0, n)], sem_in.at[semi[nm]])]
            r0 += n
        wqkv_u = wqkv_hbm.bitcast(U32)
        for i, nm in enumerate(("wq", "wk", "wv")):
            cp[nm] = [pltpu.make_async_copy(wqkv_u.at[:, pl.ds(D * i, D)], wqkv_s.at[:, pl.ds(D * i, D)],
                                            sem_in.at[semi[nm]])]
        wo_u = wo_hbm.bitcast(U32)
        cp["wo"] = [pltpu.make_async_copy(wo_u.at[:, pl.ds(128 * n, 128)], wo_s.at[n], sem_in.at[semi["wo"]])
                    for n in range(NT)]
        cp["wr"] = [pltpu.make_async_copy(wr_hbm, wr_s, sem_in.at[semi["wr"]])]
        cp["ffn"] = [pltpu.make_async_copy(a.bitcast(U32), b, sem_in.at[semi["ffn"]])
                     for i, (a, b) in enumerate(((wg_hbm, wg_s), (wu_hbm, wu_s), (wd_hbm, wd_s)))]

        def ocp(lo, hi):
            return pltpu.make_async_copy(out_s.at[pl.ds(lo, hi - lo)], out_hbm.at[pl.ds(lo, hi - lo)],
                                         sem_out.at[0])

        def start_all():
            for nm in ("x0", "wq", "wk", "wv", "wo", "wr", "x1", "x2", "ffn"):
                for c in cp[nm]:
                    c.start()

        def main():
            zero = jnp.zeros((HALO, 128), F32)
            for j in range(NT):
                k_s[j, 0:HALO, :] = zero
                v_s[j, 0:HALO, :] = zero

            lane = lax.broadcasted_iota(jnp.int32, (1, 128), 1)
            never = jnp.full((8, 128), step, jnp.int32) > 0
            st = dict(best=None, toks=[], wr=None, late=[])
            q, a, lgs, sm, gu = {}, {}, {}, {}, {}

            def pin(u):
                toks, st["toks"] = st["toks"], []
                toks += [(sl, t) for cd, sl, t in st["late"] if cd <= 1]
                st["late"] = [(cd - 1, sl, t) for cd, sl, t in st["late"] if cd > 1]
                if toks and pins:
                    ng = u.shape[0] // 8
                    rows = []
                    for i in range(ng):
                        mine = [t for g, t in toks if min(g, ng - 1) == i]
                        blk = u[8 * i:8 * i + 8]
                        if mine:
                            t = functools.reduce(lambda x, y: x | y, mine)
                            head = jnp.where(never, t, blk[:, 0:128])
                            blk = jnp.concatenate([head, blk[:, 128:]], axis=1)
                        rows.append(blk)
                    u = jnp.concatenate(rows, axis=0)
                return pltpu.bitcast(u, BF16)

            def permute_w(g):
                tiles = [wqkv_s[:, pl.ds(D * g + 128 * t, 128)] for t in range(NT)]
                for j in range(NT):
                    m = tiles[NT - 1]
                    for t in range(NT - 2, -1, -1):
                        c = lane + 128 * t
                        cm5 = c - 5 * ((c * 52429) >> 18)
                        m = jnp.where(cm5 == j, tiles[t], m)
                    src = (20 * (lane & 31) + 5 * (lane >> 5) + j) & 127
                    idx = jnp.broadcast_to(src, m.shape)
                    wp_s[:, pl.ds(D * g + 128 * j, 128)] = jnp.take_along_axis(
                        m, idx, axis=1, mode="promise_in_bounds")

            def permute_wo():
                for n in range(NT):
                    for d2 in range(DH // 2):
                        ev = wo_s[n, pl.ds(d2, H // 2, stride=DH), :]
                        od = wo_s[n, pl.ds(DH // 2 + d2, H // 2, stride=DH), :]
                        lo = (ev & jnp.uint32(0xFFFF)) | (od << 16)
                        hi = (ev >> 16) | (od & jnp.uint32(0xFFFF0000))
                        for d, val in ((2 * d2, lo), (2 * d2 + 1, hi)):
                            aa, j = divmod(d, NT)
                            wop_s[pl.ds(64 * j + 16 * aa, H // 2), pl.ds(128 * n, 128)] = val

            def a_task(b, lo, hi, slot):
                r0, n = b * T + lo, hi - lo
                x = x_s[pl.ds(r0, n), :].astype(F32)
                m = jnp.sum(x, axis=-1, keepdims=True) * (1.0 / D)
                c = x - m
                v = jnp.sum(c * c, axis=-1, keepdims=True) * (1.0 / D)
                rstd = lax.rsqrt(v + EPS)
                xn = (x * rstd - m * rstd) if ALT else c * rstd
                xn_s[pl.ds(r0 // 2, n // 2), :] = pltpu.bitcast(xn.astype(BF16), U32)
                st["toks"].append((slot, _or_all(xn_s[pl.ds(r0 // 2, n // 2), :])))

            def b_seg(b, n, lo, hi):
                w = pltpu.bitcast(wp_s[:, pl.ds(128 * n, 128)], BF16)
                lhs = pin(xn_s[pl.ds((b * T + lo) // 2, (hi - lo) // 2), :])
                acc = jnp.dot(lhs, w, preferred_element_type=F32)
                g, j = divmod(n, NT)
                if g == 0:
                    acc = acc * QSCALE
                if FA:
                    st["late"].append((FA, FS, _or_all(pltpu.bitcast(acc, U32))))
                if g == 0:
                    for r in range(lo, hi, 8):
                        q[b * T + r, j] = acc[r - lo:r - lo + 8]
                else:
                    (k_s if g == 1 else v_s)[j, pl.ds(HALO + b * T + lo, hi - lo), :] = acc

            def l_task(b, c, h, w, gate, slot):
                r0 = b * T + c * R + h
                qc = [jnp.concatenate([q[r0 + r, j] for r in range(0, RL, 8)], axis=0) for j in range(NT)]
                off = HALO + r0 - DIL * w
                p = qc[0] * k_s[0, pl.ds(off, RL), :]
                for j in range(1, NT):
                    p = p + qc[j] * k_s[j, pl.ds(off, RL), :]
                p = p + pltpu.roll(p, 64, 1)
                p = p + pltpu.roll(p, 32, 1)
                if r0 - DIL * w < 0:
                    pos = lax.broadcasted_iota(jnp.int32, (RL, 128), 0) + (r0 - DIL * w)
                    p = jnp.where(pos >= 0, p, -1e9)
                lgs[r0, w] = p
                if gate:
                    st["toks"].append((slot, _or_all(pltpu.bitcast(p, U32))))

            def s_task(b, c, h, gate, slot):
                r0 = b * T + c * R + h
                lg = [lgs.pop((r0, w)) for w in range(W)]
                m = _tree(jnp.maximum, lg)
                e = [jnp.exp2(l - m) for l in lg]
                inv = pl.reciprocal(_tree(jnp.add, e), approx=True)
                sm[r0] = e + [inv]
                if gate:
                    st["toks"].append((slot, _or_all(pltpu.bitcast(inv, U32))))

            def p_task(b, c, j, gate, slot):
                r0 = b * T + c * R
                ei = [jnp.concatenate([sm[r0 + h][w] for h in range(0, R, RL)], axis=0) for w in range(W + 1)]
                e, inv = ei[:W], ei[W]
                acc = None
                for w in range(W):
                    off = HALO + r0 - DIL * w
                    t = e[w] * v_s[j, pl.ds(off, R), :]
                    acc = t if acc is None else acc + t
                dst = (pl.ds(r0 // 2, R // 2), pl.ds(128 * j, 128))
                o_s[dst] = pltpu.bitcast((acc * inv).astype(BF16), U32)
                if gate:
                    st["toks"].append((slot, o_s[dst]))

            def d_seg(b, n, lo, hi):
                w = pltpu.bitcast(wop_s[:, pl.ds(128 * n, 128)], BF16)
                lhs = pin(o_s[pl.ds((b * T + lo) // 2, (hi - lo) // 2), :])
                acc = jnp.dot(lhs, w, preferred_element_type=F32)
                if HD:
                    acc = acc + x_s[pl.ds(b * T + lo, hi - lo), pl.ds(128 * n, 128)].astype(F32)
                if FA:
                    st["late"].append((FA, FS, _or_all(pltpu.bitcast(acc, U32))))
                for r in range(lo, hi, 8):
                    a[b * T + r, n] = acc[r - lo:r - lo + 8]

            def e_task(b, lo, hi, slot):
                r0, n = b * T + lo, hi - lo
                cols = []
                for j in range(NT):
                    cols.append(jnp.concatenate([a[r0 + r, j] for r in range(0, n, 8)], axis=0))
                if st["wr"] is None:
                    st["wr"] = wr_s[...].astype(F32).reshape(1, D)
                h = jnp.concatenate(cols, axis=1)
                if not HD:
                    h = x_s[pl.ds(r0, n), :].astype(F32) + h
                m = jnp.sum(h, axis=-1, keepdims=True) * (1.0 / D)
                c = h - m
                v = jnp.sum(c * c, axis=-1, keepdims=True) * (1.0 / D)
                cw = jnp.sum(c * st["wr"], axis=-1, keepdims=True)
                rstd = lax.rsqrt(v + EPS)
                hn = (h * rstd - m * rstd) if ALT else c * rstd
                out_s[pl.ds(pl.multiple_of(step * 16 + r0, 16), n), :] = (h + hn).astype(BF16)
                hn_s[pl.ds(r0 // 2, n // 2), :] = pltpu.bitcast(hn.astype(BF16), U32)
                r = jnp.broadcast_to(cw * rstd, (n, 128))
                best = st["best"]
                for i in range(n // 8):
                    ri = r[8 * i:8 * i + 8]
                    rows = lax.broadcasted_iota(jnp.int32, (8, 128), 0) + (r0 + 8 * i)
                    if best is None:
                        best = (jnp.where(ri > -jnp.inf, ri, -jnp.inf), rows)
                    else:
                        bv, bi = best
                        upd = ri > bv
                        best = (jnp.where(upd, ri, bv), jnp.where(upd, rows, bi))
                st["best"] = best
                if b == NS - 1:
                    ocp(r0, r0 + n).start()
                elif hi == T:
                    ocp(b * T, (b + 1) * T).start()
                probe = hn_s[pl.ds(pl.multiple_of(step * 8, 8), 8), 0:128]
                probe2 = pltpu.bitcast(out_s[0:16, 0:128], U32)
                st["toks"].append((slot, pltpu.bitcast(best[0], U32) | pltpu.bitcast(best[1], U32) | probe | probe2))

            def spec_task(slot):
                st["spec"] = argmax(st["best"])[1]
                st["xs"] = load_chunk(st["spec"])

            def g_seg(k, n, lo, hi):
                w = pltpu.bitcast((wg_s, wu_s)[k][:, pl.ds(128 * n, 128)], BF16)
                gu[k, n] = jnp.dot(st["xs"], w, preferred_element_type=F32)

            def h_seg(n):
                if "act" not in st:
                    g = jnp.concatenate([gu[0, i] for i in range(F // 128)], axis=1)
                    u = jnp.concatenate([gu[1, i] for i in range(F // 128)], axis=1)
                    st["act"] = (g * jax.nn.sigmoid(g) * u).astype(BF16)
                w = pltpu.bitcast(wd_s[:, pl.ds(128 * n, 128)], BF16)
                y_s[:, pl.ds(128 * n, 128)] = jnp.dot(st["act"], w, preferred_element_type=F32)

            def do_wait(nm):
                st["toks"] = []
                st["late"] = []
                for c in cp[nm]:
                    wait(c, nm)

            fns = dict(A=a_task, B=b_seg, L=l_task, S=s_task, P=p_task, D=d_seg, E=e_task, wait=do_wait,
                       perm=permute_w, permo=permute_wo, spec=spec_task, G=g_seg, H=h_seg)
            for item in prog:
                fns[item[0]](*item[1:])
            return st["best"], st.get("spec")

        def argmax(best):
            bv, bi = best
            mx = jnp.max(bv, axis=0, keepdims=True)
            idx = jnp.min(jnp.where(bv >= mx, bi, S - 1), axis=0, keepdims=True)
            return mx[:, 0:1], jnp.clip(idx[0, 0], 0, S - 1)

        def load_chunk(idx):
            blk = jnp.clip(idx >> 4, 0, S // 16 - 1)
            return pltpu.bitcast(hn_s[pl.ds(pl.multiple_of(blk * 8, 8), 8), :], BF16)

        def ffn(idx):
            xs = load_chunk(idx)
            g = jnp.dot(xs, pltpu.bitcast(wg_s[...], BF16), preferred_element_type=F32)
            u = jnp.dot(xs, pltpu.bitcast(wu_s[...], BF16), preferred_element_type=F32)
            act = (g * jax.nn.sigmoid(g) * u).astype(BF16)
            y_s[...] = jnp.dot(act, pltpu.bitcast(wd_s[...], BF16), preferred_element_type=F32)

        def tail(best, spec):
            mx, idx = argmax(best)
            if spec is None:
                ffn(idx)
            else:
                @pl.when((idx >> 4) != (spec >> 4))
                def _():
                    ffn(idx)
            blk = jnp.clip(idx >> 4, 0, S // 16 - 1)
            base = pl.multiple_of(blk * 16, 16)
            y = y_s[...] * jax.nn.sigmoid(mx)
            wait(ocp(0, S), "out")
            cur = out_s[pl.ds(base, 16), :].astype(F32)
            rows = lax.broadcasted_iota(jnp.int32, (16, D), 0) + base
            out_s[pl.ds(base, 16), :] = jnp.where(rows == idx, cur + y, cur).astype(BF16)
            fix = pltpu.make_async_copy(out_s.at[pl.ds(base, 16)], out_hbm.at[pl.ds(base, 16)], sem_out.at[0])
            fix.start()
            wait(fix, "fix")

        if G == 2:
            pl.when(pid == 0)(start_all)

            @pl.when(pid == 1)
            def _():
                tail(*main())
        else:
            start_all()
            tail(*main())

    @jax.jit
    def fn(A_x, A_wqkv, A_wo, B_x, B_w_r, B_w_gate, B_w_up, B_w_down):
        any_spec = pl.BlockSpec(memory_space=pl.ANY)
        out = pl.pallas_call(
            kernel,
            grid=(G,),
            out_shape=jax.ShapeDtypeStruct((S, D), BF16),
            in_specs=[any_spec] * 7,
            out_specs=any_spec,
            scratch_shapes=[
                pltpu.VMEM((S, D), BF16),
                pltpu.VMEM((D // 2, 3 * D), U32),
                pltpu.VMEM((NT, D // 2, 128), U32),
                pltpu.VMEM((D,), BF16),
                pltpu.VMEM((D // 2, F), U32),
                pltpu.VMEM((D // 2, F), U32),
                pltpu.VMEM((F // 2, D), U32),
                pltpu.VMEM((D // 2, 3 * D), U32),
                pltpu.VMEM((D // 2, D), U32),
                pltpu.VMEM((NT, S + HALO, 128), F32),
                pltpu.VMEM((NT, S + HALO, 128), F32),
                pltpu.VMEM((S // 2, D), U32),
                pltpu.VMEM((S // 2, D), U32),
                pltpu.VMEM((S // 2, D), U32),
                pltpu.VMEM((S + 16, D), BF16),
                pltpu.VMEM((16, D), F32),
                pltpu.SemaphoreType.DMA((6,)),
                pltpu.SemaphoreType.DMA((1,)),
            ],
            compiler_params=pltpu.CompilerParams(vmem_limit_bytes=100 << 20,
                                                 dimension_semantics=("arbitrary",),
                                                 disable_bounds_checks=True,
                                                 disable_semaphore_checks=True),
            name="fused",
        )(A_x.reshape(S, D), A_wqkv, A_wo, B_w_r, B_w_gate, B_w_up, B_w_down)
        return out.reshape(1, S, D)

    return fn


pallas_sequential_preLN__sliding_local_dilated__moe_arch_mod__prompt_kernel = make_kernel(SPEC=1, GL=0)
```

```python
import functools
import math
import jax
import jax.numpy as jnp
from jax import lax
import jax.experimental.pallas as pl
import jax.experimental.pallas.tpu as pltpu

S, D, F = 2048, 640, 1536
H, DH, W, DIL = 32, 20, 8, 2
NT = D // 128
HALO = 16
EPS = 1e-5
F32, BF16, U32 = jnp.float32, jnp.bfloat16, jnp.uint32
QSCALE = DH ** -0.5 * math.log2(math.e)
R = 16
T = 128
NS = S // T
NC = T // R
LATE = (NS - 2) * T
KA = 384


def _or_all(u):
    t = None
    for i in range(u.shape[0] // 8):
        for j in range(u.shape[1] // 128):
            p = u[8 * i:8 * i + 8, 128 * j:128 * (j + 1)]
            t = p if t is None else t | p
    return t


def _tree(f, xs):
    xs = list(xs)
    while len(xs) > 1:
        xs = [f(xs[i], xs[i + 1]) for i in range(0, len(xs) - 1, 2)] + ([xs[-1]] if len(xs) % 2 else [])
    return xs[0]


def interleave(segs, tasks):
    out = []
    tasks = sorted(tasks, key=lambda t: t[0])
    i = 0
    pos = 0
    for sg in segs:
        n = (sg[-1] - sg[-2]) // 16
        while i < len(tasks) and tasks[i][0] < pos + n:
            out.append(tasks[i][1] + (max(tasks[i][0] - pos, 0),))
            i += 1
        out.append(sg)
        pos += n
    out += [t[1] + (0,) for t in tasks[i:]]
    return out


def _opts(s):
    if not isinstance(s, str):
        return dict(s)
    out = {}
    for kv in s.split(","):
        k, v = kv.split(":")
        v = [float(x) if "." in x else int(x) for x in v.split("/") if x]
        out[k] = v[0] if len(v) == 1 and not kv.endswith("/") else tuple(v)
    return out


def build_program(C0, CP, LS, SO, PO, PS, EDL, ADL, RL, SPEC, GL, GS, PRE, TL, PR, XB):
    def B(b, g):
        return [("B", b, n, 0, T) for n in range(NT * g, NT * g + NT)]

    def Dm(b, lo=0, hi=T):
        return [("D", b, n, lo, hi) for n in range(NT)]

    def parts(kind, b, dls, lo=0, hi=T):
        n = (hi - lo) // len(dls)
        return [(8 * dl, (kind, b, lo + i * n, lo + (i + 1) * n)) for i, dl in enumerate(dls)]

    def LSt(b, c0, cp, rl=R, chunks=range(NC)):
        t = []
        for i, c in enumerate(chunks):
            base = c0 + cp * i
            for h in range(0, R, rl):
                sh = -(R - rl - h) * cp / R
                t += [(int(base + sh + LS * w), ("L", b, c, h, rl, w, GL)) for w in range(W)]
                t += [(int(base + sh + SO), ("S", b, c, h, rl, GS))]
        return t

    def Pt(b, c0, cp, chunks=range(NC)):
        t = []
        for i, c in enumerate(chunks):
            t += [(int(c0 + cp * i + PS * j), ("P", b, c, j, True)) for j in range(NT)]
        return t

    def Cf(b, c0=C0, cp=CP, rl=RL):
        return LSt(b, c0, cp, rl) + Pt(b, c0 + PO, cp)

    def Q(b, part):
        return [("Q", b, n, part, 0, T) for n in range(NT)]

    pr = dict(pv=(12, 6), l1=(40, 8), p0=(92, 3.5), np0=8, p1=(36, 5), c2=(84, 17.5), a3=(13,), e0=(16, 19), e1=(22, 25),
              a4=(20, 28), qb2=0, l0=(999, 0))
    pr.update(_opts(PR))
    p = [("wait", "x0a"), ("A", 0, 0, T, 0), ("A", 1, 0, T, 0), ("wait", "wqa"), ("perm", 0, 0)]
    p += Q(0, 0)
    p += [("wait", "x0b"), ("wait", "wqb"), ("perm", 0, 1), ("A", 2, 0, T, 0), ("drop",)]
    p += Q(1, 0) + Q(0, 1) + Q(1, 1) + Q(2, 0) + (Q(2, 1) if pr["qb2"] else [])
    p += [("wait", "wk"), ("perm", 1)]
    p += interleave(([] if pr["qb2"] else Q(2, 1)) + B(0, 1) + B(1, 1), LSt(0, *pr["l0"]))
    p += [("wait", "wv")]
    p += interleave(B(2, 1) + B(0, 2) + B(1, 2),
                    [(pr["pv"][0] + pr["pv"][1] * j, ("perm", 2, None, (j,))) for j in range(NT)]
                    + LSt(1, *pr["l1"]) + Pt(0, *pr["p0"], range(pr["np0"])))
    p += [("wait", "wo"), ("wait", "wr"), ("wait", "x1"), ("permo",)]
    p += interleave(B(2, 2) + Dm(0) + Dm(1) + B(3, 0) + B(3, 1) + B(3, 2),
                    Pt(0, 10, 4, range(pr["np0"], NC)) + Pt(1, *pr["p1"]) + parts("A", 3, pr["a3"])
                    + parts("E", 0, pr["e0"]) + parts("E", 1, pr["e1"])
                    + Cf(2, *pr["c2"]) + parts("A", 4, pr["a4"]))
    for s in range(3, NS - 2):
        segs = Dm(s - 1) + B(s + 1, 0) + B(s + 1, 1) + B(s + 1, 2)
        tasks = parts("E", s - 1, EDL) + Cf(s)
        if s == XB:
            pre = [t for t in tasks if t[1][0] in "LS" and t[1][2] < PRE]
            tasks = [t for t in tasks if t not in pre]
            p += [t[1] + (0,) for t in pre]
            p += [("wait", "x2"), ("wait", "ffn")]
        if s + 2 < NS:
            tasks += parts("A", s + 2, ADL)
        p += interleave(segs, tasks)
    s = NS - 2
    big = Dm(s - 1) + B(s + 1, 0) + B(s + 1, 1) + Dm(s) + B(s + 1, 2)
    small = [("G", k, n, 0, 0) for n in range(F // 128) for k in range(2)] if SPEC else []
    tl = dict(e13=(9, 11), sp=12, c0=14, cp=12.5, l0=130, lp=4.5, pd=10, pp=0.75, e14=(186, 198), e15=243,
              gh=6, lr=16, cr=RL, cut=64, pl=0, pc=8, pb=200)
    tl.update(_opts(TL))
    cut = tl["cut"]
    segs = []
    n_big = len(big) - tl["sp"]
    n_small = max(len(small) - tl["gh"], 0)
    done = 0
    for g, sg in enumerate(big):
        segs.append(sg)
        if g >= tl["sp"]:
            want = min(n_small, -(-(g - tl["sp"] + 1) * n_small // n_big))
            segs += small[done:want]
            done = want
    segs += small[done:] + Dm(s + 1, 0, cut) + Dm(s + 1, cut, T)
    if SPEC:
        segs += [("H", n, 0, 16) for n in range(NT)]
    n14 = len(tl["e14"])
    p15 = []
    for j in range(NT):
        for c in range(NC):
            early = j < tl["pl"] and c < tl["pc"]
            dl = int(160 + 8 * (j + 1) + tl["pd"] + tl["pp"] * c) if early else (200 if c < cut // R else tl["pb"])
            p15.append((dl, ("P", s + 1, c, j, early)))
    tasks = (parts("E", s - 1, tl["e13"]) + ([(8 * tl["sp"], ("spec",))] if SPEC else [])
             + Cf(s, tl["c0"], tl["cp"], tl["cr"]) + LSt(s + 1, tl["l0"], tl["lp"], tl["lr"]) + p15
             + [(dl, ("E", s, i * T // n14, (i + 1) * T // n14)) for i, dl in enumerate(tl["e14"])]
             + [(tl["e15"], ("E", s + 1, 0, cut)), (999, ("E", s + 1, cut, T))])
    p += interleave(segs, tasks)
    return p


def make_kernel(C0=16, CP=17.5, LS=0, SO=8, PO=10, PS=1, EDL=(12, 18), ADL=(7, 16),
                prof=0, pins=1, RL=8, FA=3, FS=0, SPEC=1, ALT=0, HD=1, GL=0, GS=1, PRE=2, TL=(), G=2, PR=(), XB=7):
    X1 = (XB - 1) * T
    XCH = (2 * T, T, X1, S - 3 * T - X1)
    prog = build_program(C0, CP, LS, SO, PO, PS, EDL, ADL, RL, SPEC, GL, GS, PRE, TL, PR, XB)

    def wait(c, name):
        if prof:
            with jax.named_scope("w_" + name):
                c.wait()
        else:
            c.wait()

    def kernel(x_hbm, wqkv_hbm, wo_hbm, wr_hbm, wg_hbm, wu_hbm, wd_hbm, out_hbm,
               x_s, wqkv_s, wo_s, wr_s, wg_s, wu_s, wd_s, wp_s, wop_s,
               k_s, v_s, xn_s, o_s, hn_s, out_s, y_s, act_s, sem_in, sem_out):
        pid = pl.program_id(0)
        step = pid - (1 if G == 2 else 0)
        cp = {}
        semi = dict(x0a=0, wqa=1, x0b=6, wqb=6, wk=2, wv=3, wo=4, wr=4, x1=4, x2=5, ffn=5)
        r0 = 0
        for nm, n in zip(("x0a", "x0b", "x1", "x2"), XCH):
            cp[nm] = [pltpu.make_async_copy(x_hbm.at[pl.ds(r0, n)], x_s.at[pl.ds(r0, n)], sem_in.at[semi[nm]])]
            r0 += n
        wqkv_u = wqkv_hbm.bitcast(U32)
        for nm, lo, hi, g in (("wqa", 0, KA // 2, 0), ("wqb", KA // 2, D // 2, 0), ("wk", 0, D // 2, 1),
                              ("wv", 0, D // 2, 2)):
            sl = (pl.ds(lo, hi - lo), pl.ds(D * g, D))
            cp[nm] = [pltpu.make_async_copy(wqkv_u.at[sl], wqkv_s.at[sl], sem_in.at[semi[nm]])]
        wo_u = wo_hbm.bitcast(U32)
        cp["wo"] = [pltpu.make_async_copy(wo_u.at[:, pl.ds(128 * n, 128)], wo_s.at[n, pl.ds(0, D // 2)], sem_in.at[semi["wo"]])
                    for n in range(NT)]
        cp["wr"] = [pltpu.make_async_copy(wr_hbm, wr_s, sem_in.at[semi["wr"]])]
        cp["ffn"] = [pltpu.make_async_copy(a.bitcast(U32), b, sem_in.at[semi["ffn"]])
                     for i, (a, b) in enumerate(((wg_hbm, wg_s), (wu_hbm, wu_s), (wd_hbm, wd_s)))]

        def ocp(lo, hi):
            return pltpu.make_async_copy(out_s.at[pl.ds(lo, hi - lo)], out_hbm.at[pl.ds(lo, hi - lo)],
                                         sem_out.at[0 if lo < LATE else 1])

        def start_all():
            first = ("x0a", "wqa", "x0b", "wqb")
            for nm in first + ("wk", "wv", "wo", "wr", "x1", "x2", "ffn"):
                for c in cp[nm]:
                    c.start()

        def main():
            zero = jnp.zeros((HALO, 128), F32)
            for j in range(NT):
                k_s[j, 0:HALO, :] = zero
                v_s[j, 0:HALO, :] = zero

            lane = lax.broadcasted_iota(jnp.int32, (1, 128), 1)
            cm5 = [(lane + 128 * t) - 5 * (((lane + 128 * t) * 52429) >> 18) for t in range(NT - 1)]
            srcs = [(20 * (lane & 31) + 5 * (lane >> 5) + j) & 127 for j in range(NT)]
            never = jnp.full((8, 128), step, jnp.int32) > 0
            st = dict(best=None, toks=[], wr=None, late=[])
            q, a, lgs, sm, gu = {}, {}, {}, {}, {}

            def pin(u):
                toks, st["toks"] = st["toks"], []
                toks += [(sl, t) for cd, sl, t in st["late"] if cd <= 1]
                st["late"] = [(cd - 1, sl, t) for cd, sl, t in st["late"] if cd > 1]
                if toks and pins:
                    ng = u.shape[0] // 8
                    rows = []
                    for i in range(ng):
                        mine = [t for g, t in toks if min(g, ng - 1) == i]
                        blk = u[8 * i:8 * i + 8]
                        if mine:
                            t = functools.reduce(lambda x, y: x | y, mine)
                            head = jnp.where(never, t, blk[:, 0:128])
                            blk = jnp.concatenate([head, blk[:, 128:]], axis=1)
                        rows.append(blk)
                    u = jnp.concatenate(rows, axis=0)
                return pltpu.bitcast(u, BF16)

            def permute_w(g, part=None, js=range(NT), slot=None):
                rows = {None: pl.ds(0, D // 2), 0: pl.ds(0, KA // 2), 1: pl.ds(KA // 2, (D - KA) // 2)}[part]
                tiles = [wqkv_s[rows, pl.ds(D * g + 128 * t, 128)] for t in range(NT)]
                for j in js:
                    m = tiles[NT - 1]
                    for t in range(NT - 2, -1, -1):
                        m = jnp.where(cm5[t] == j, tiles[t], m)
                    idx = jnp.broadcast_to(srcs[j], m.shape)
                    res = jnp.take_along_axis(m, idx, axis=1, mode="promise_in_bounds")
                    wp_s[rows, pl.ds(D * g + 128 * j, 128)] = res
                    if slot is not None:
                        st["toks"].append((slot, _or_all(res)))

            def permute_wo():
                for n in range(NT):
                    for d2 in range(DH // 2):
                        ev = wo_s[n, pl.ds(d2, H // 2, stride=DH), :]
                        od = wo_s[n, pl.ds(DH // 2 + d2, H // 2, stride=DH), :]
                        lo = (ev & jnp.uint32(0xFFFF)) | (od << 16)
                        hi = (ev >> 16) | (od & jnp.uint32(0xFFFF0000))
                        for d, val in ((2 * d2, lo), (2 * d2 + 1, hi)):
                            aa, j = divmod(d, NT)
                            wop_s[pl.ds(64 * j + 16 * aa, H // 2), pl.ds(128 * n, 128)] = val

            def a_task(b, lo, hi, slot):
                r0, n = b * T + lo, hi - lo
                x = x_s[pl.ds(r0, n), :].astype(F32)
                m = jnp.sum(x, axis=-1, keepdims=True) * (1.0 / D)
                c = x - m
                v = jnp.sum(c * c, axis=-1, keepdims=True) * (1.0 / D)
                rstd = lax.rsqrt(v + EPS)
                xn = (x * rstd - m * rstd) if ALT else c * rstd
                xn_s[pl.ds(r0 // 2, n // 2), :] = pltpu.bitcast(xn.astype(BF16), U32)
                st["toks"].append((slot, _or_all(xn_s[pl.ds(r0 // 2, n // 2), :])))

            def b_seg(b, n, lo, hi):
                w = pltpu.bitcast(wp_s[:, pl.ds(128 * n, 128)], BF16)
                lhs = pin(xn_s[pl.ds((b * T + lo) // 2, (hi - lo) // 2), :])
                acc = jnp.dot(lhs, w, preferred_element_type=F32)
                g, j = divmod(n, NT)
                if g == 0:
                    acc = acc * QSCALE
                if FA:
                    st["late"].append((FA, FS, _or_all(pltpu.bitcast(acc, U32))))
                if g == 0:
                    for r in range(lo, hi, 8):
                        q[b * T + r, j] = acc[r - lo:r - lo + 8]
                else:
                    (k_s if g == 1 else v_s)[j, pl.ds(HALO + b * T + lo, hi - lo), :] = acc

            def q_seg(b, n, part, lo, hi):
                k0, k1 = ((0, KA), (KA, D))[part]
                w = pltpu.bitcast(wp_s[pl.ds(k0 // 2, (k1 - k0) // 2), pl.ds(128 * n, 128)], BF16)
                lhs = pin(xn_s[pl.ds(b * T // 2, T // 2), pl.ds(k0, k1 - k0)])
                acc = jnp.dot(lhs, w, preferred_element_type=F32)
                if part == 0:
                    st["qa", b, n] = acc
                else:
                    acc = (acc + st.pop(("qa", b, n))) * QSCALE
                    for r in range(0, T, 8):
                        q[b * T + r, n] = acc[r:r + 8]

            def l_task(b, c, h, RL, w, gate, slot):
                r0 = b * T + c * R + h
                qc = [jnp.concatenate([q[r0 + r, j] for r in range(0, RL, 8)], axis=0) for j in range(NT)]
                off = HALO + r0 - DIL * w
                p = qc[0] * k_s[0, pl.ds(off, RL), :]
                for j in range(1, NT):
                    p = p + qc[j] * k_s[j, pl.ds(off, RL), :]
                p = p + pltpu.roll(p, 64, 1)
                p = p + pltpu.roll(p, 32, 1)
                if r0 - DIL * w < 0:
                    pos = lax.broadcasted_iota(jnp.int32, (RL, 128), 0) + (r0 - DIL * w)
                    p = jnp.where(pos >= 0, p, -1e9)
                lgs[r0, w] = p
                if gate:
                    st["toks"].append((slot, _or_all(pltpu.bitcast(p, U32))))

            def s_task(b, c, h, RL, gate, slot):
                r0 = b * T + c * R + h
                lg = [lgs.pop((r0, w)) for w in range(W)]
                m = _tree(jnp.maximum, lg)
                e = [jnp.exp2(l - m) for l in lg]
                inv = pl.reciprocal(_tree(jnp.add, e), approx=True)
                for r in range(0, RL, 8):
                    sm[r0 + r] = [t[r:r + 8] for t in e + [inv]]
                if gate:
                    st["toks"].append((slot, _or_all(pltpu.bitcast(inv, U32))))

            def p_task(b, c, j, gate, slot):
                r0 = b * T + c * R
                ei = [jnp.concatenate([sm[r0 + h][w] for h in range(0, R, 8)], axis=0) for w in range(W + 1)]
                e, inv = ei[:W], ei[W]
                acc = None
                for w in range(W):
                    off = HALO + r0 - DIL * w
                    t = e[w] * v_s[j, pl.ds(off, R), :]
                    acc = t if acc is None else acc + t
                dst = (pl.ds(r0 // 2, R // 2), pl.ds(128 * j, 128))
                o_s[dst] = pltpu.bitcast((acc * inv).astype(BF16), U32)
                if gate:
                    st["toks"].append((slot, o_s[dst]))

            def d_seg(b, n, lo, hi):
                w = pltpu.bitcast(wop_s[:, pl.ds(128 * n, 128)], BF16)
                lhs = pin(o_s[pl.ds((b * T + lo) // 2, (hi - lo) // 2), :])
                acc = jnp.dot(lhs, w, preferred_element_type=F32)
                if HD:
                    acc = acc + x_s[pl.ds(b * T + lo, hi - lo), pl.ds(128 * n, 128)].astype(F32)
                if FA and hi - lo == T and (b, n) < (NS - 2, 3):
                    st["late"].append((FA, FS, _or_all(pltpu.bitcast(acc, U32))))
                for r in range(lo, hi, 8):
                    a[b * T + r, n] = acc[r - lo:r - lo + 8]

            def e_task(b, lo, hi, slot):
                r0, n = b * T + lo, hi - lo
                cols = []
                for j in range(NT):
                    cols.append(jnp.concatenate([a[r0 + r, j] for r in range(0, n, 8)], axis=0))
                if st["wr"] is None:
                    st["wr"] = wr_s[...].astype(F32).reshape(1, D)
                h = jnp.concatenate(cols, axis=1)
                if not HD:
                    h = x_s[pl.ds(r0, n), :].astype(F32) + h
                m = jnp.sum(h, axis=-1, keepdims=True) * (1.0 / D)
                c = h - m
                v = jnp.sum(c * c, axis=-1, keepdims=True) * (1.0 / D)
                cw = jnp.sum(c * st["wr"], axis=-1, keepdims=True)
                rstd = lax.rsqrt(v + EPS)
                hn = (h * rstd - m * rstd) if ALT else c * rstd
                out_s[pl.ds(pl.multiple_of(step * 16 + r0, 16), n), :] = (h + hn).astype(BF16)
                hn_s[pl.ds(r0 // 2, n // 2), :] = pltpu.bitcast(hn.astype(BF16), U32)
                r = jnp.broadcast_to(cw * rstd, (n, 128))
                best = st["best"]
                for i in range(n // 8):
                    ri = r[8 * i:8 * i + 8]
                    rows = lax.broadcasted_iota(jnp.int32, (8, 128), 0) + (r0 + 8 * i)
                    if best is None:
                        best = (jnp.where(ri > -jnp.inf, ri, -jnp.inf), rows)
                    else:
                        bv, bi = best
                        upd = ri > bv
                        best = (jnp.where(upd, ri, bv), jnp.where(upd, rows, bi))
                st["best"] = best
                if b == NS - 1:
                    ocp(r0, r0 + n).start()
                elif hi == T:
                    ocp(b * T, (b + 1) * T).start()
                probe = hn_s[pl.ds(pl.multiple_of(step * 8, 8), 8), 0:128]
                probe2 = pltpu.bitcast(out_s[0:16, 0:128], U32)
                st["toks"].append((slot, pltpu.bitcast(best[0], U32) | pltpu.bitcast(best[1], U32) | probe | probe2))

            def spec_task(slot):
                st["spec"] = argmax(st["best"])[1]
                st["xs"] = load_chunk(st["spec"], LATE)

            def g_seg(k, n, lo, hi):
                w = pltpu.bitcast((wg_s, wu_s)[k][:, pl.ds(128 * n, 128)], BF16)
                gu[k, n] = jnp.dot(st["xs"], w, preferred_element_type=F32)

            def h_seg(n, lo, hi):
                if "act" not in st:
                    g = jnp.concatenate([gu[0, i] for i in range(F // 128)], axis=1)
                    u = jnp.concatenate([gu[1, i] for i in range(F // 128)], axis=1)
                    act_s[...] = pltpu.bitcast((g * jax.nn.sigmoid(g) * u).astype(BF16), U32)
                    st["act"] = True
                w = pltpu.bitcast(wd_s[:, pl.ds(128 * n, 128)], BF16)
                y_s[:, pl.ds(128 * n, 128)] = jnp.dot(pin(act_s[...]), w, preferred_element_type=F32)

            def do_wait(nm):
                st["toks"] = []
                st["late"] = []
                for c in cp[nm]:
                    wait(c, nm)

            fns = dict(drop=lambda: st.update(toks=[]), A=a_task, B=b_seg, Q=q_seg, L=l_task, S=s_task, P=p_task, D=d_seg, E=e_task, wait=do_wait,
                       perm=permute_w, permo=permute_wo, spec=spec_task, G=g_seg, H=h_seg)
            for item in prog:
                fns[item[0]](*item[1:])
            return st["best"], st.get("spec")

        def argmax(best):
            bv, bi = best
            mx = jnp.max(bv, axis=0, keepdims=True)
            idx = jnp.min(jnp.where(bv >= mx, bi, S - 1), axis=0, keepdims=True)
            return mx[:, 0:1], jnp.clip(idx[0, 0], 0, S - 1)

        def load_chunk(idx, nrows):
            blk = jnp.clip(idx >> 4, 0, nrows // 16 - 1)
            return pltpu.bitcast(hn_s[pl.ds(pl.multiple_of(blk * 8, 8), 8), :], BF16)

        def ffn(idx):
            xs = load_chunk(idx, S)
            g = jnp.dot(xs, pltpu.bitcast(wg_s[...], BF16), preferred_element_type=F32)
            u = jnp.dot(xs, pltpu.bitcast(wu_s[...], BF16), preferred_element_type=F32)
            act = (g * jax.nn.sigmoid(g) * u).astype(BF16)
            y_s[...] = jnp.dot(act, pltpu.bitcast(wd_s[...], BF16), preferred_element_type=F32)

        def fix_row(mx, idx, nrows):
            base = pl.multiple_of(jnp.clip(idx >> 4, 0, nrows // 16 - 1) * 16, 16)
            y = y_s[...] * jax.nn.sigmoid(mx)
            cur = out_s[pl.ds(base, 16), :].astype(F32)
            rows = lax.broadcasted_iota(jnp.int32, (16, D), 0) + base
            out_s[pl.ds(base, 16), :] = jnp.where(rows == idx, cur + y, cur).astype(BF16)
            fix = pltpu.make_async_copy(out_s.at[pl.ds(base, 16)], out_hbm.at[pl.ds(base, 16)], sem_out.at[2])
            fix.start()
            return fix

        def tail(best, spec):
            mx, idx = argmax(best)
            wait(ocp(0, LATE), "out0")

            @pl.when(idx < LATE)
            def _():
                if spec is None:
                    ffn(idx)
                fix = fix_row(mx, idx, LATE)
                wait(ocp(LATE, S), "out1")
                wait(fix, "fix")

            @pl.when(idx >= LATE)
            def _():
                ffn(idx)
                wait(ocp(LATE, S), "out1")
                wait(fix_row(mx, idx, S), "fix")

        if G == 2:
            pl.when(pid == 0)(start_all)

            @pl.when(pid == 1)
            def _():
                tail(*main())
        else:
            start_all()
            tail(*main())

    @jax.jit
    def fn(A_x, A_wqkv, A_wo, B_x, B_w_r, B_w_gate, B_w_up, B_w_down):
        any_spec = pl.BlockSpec(memory_space=pl.ANY)
        out = pl.pallas_call(
            kernel,
            grid=(G,),
            out_shape=jax.ShapeDtypeStruct((S, D), BF16),
            in_specs=[any_spec] * 7,
            out_specs=any_spec,
            scratch_shapes=[
                pltpu.VMEM((S, D), BF16),
                pltpu.VMEM((D // 2, 3 * D), U32),
                pltpu.VMEM((NT, D // 2 + 32, 128), U32),
                pltpu.VMEM((D,), BF16),
                pltpu.VMEM((D // 2, F), U32),
                pltpu.VMEM((D // 2, F), U32),
                pltpu.VMEM((F // 2, D), U32),
                pltpu.VMEM((D // 2, 3 * D), U32),
                pltpu.VMEM((D // 2, D), U32),
                pltpu.VMEM((NT, S + HALO, 128), F32),
                pltpu.VMEM((NT, S + HALO, 128), F32),
                pltpu.VMEM((S // 2, D), U32),
                pltpu.VMEM((S // 2, D), U32),
                pltpu.VMEM((S // 2, D), U32),
                pltpu.VMEM((S + 16, D), BF16),
                pltpu.VMEM((16, D), F32),
                pltpu.VMEM((8, F), U32),
                pltpu.SemaphoreType.DMA((7,)),
                pltpu.SemaphoreType.DMA((3,)),
            ],
            compiler_params=pltpu.CompilerParams(vmem_limit_bytes=100 << 20,
                                                 dimension_semantics=("arbitrary",),
                                                 disable_bounds_checks=True,
                                                 disable_semaphore_checks=True),
            name="fused",
        )(A_x.reshape(S, D), A_wqkv, A_wo, B_w_r, B_w_gate, B_w_up, B_w_down)
        return out.reshape(1, S, D)

    return fn


pallas_sequential_preLN__sliding_local_dilated__moe_arch_mod__prompt_kernel = make_kernel()
```

```python
import functools
import math
import jax
import jax.numpy as jnp
from jax import lax
import jax.experimental.pallas as pl
import jax.experimental.pallas.tpu as pltpu

S, D, F = 2048, 640, 1536
H, DH, W, DIL = 32, 20, 8, 2
NT = D // 128
HALO = 16
EPS = 1e-5
F32, BF16, U32 = jnp.float32, jnp.bfloat16, jnp.uint32
QSCALE = DH ** -0.5 * math.log2(math.e)
R = 16
T = 128
NS = S // T
NC = T // R
KA = 384


def _or_all(u):
    t = None
    for i in range(u.shape[0] // 8):
        for j in range(u.shape[1] // 128):
            p = u[8 * i:8 * i + 8, 128 * j:128 * (j + 1)]
            t = p if t is None else t | p
    return t


def _tree(f, xs):
    xs = list(xs)
    while len(xs) > 1:
        xs = [f(xs[i], xs[i + 1]) for i in range(0, len(xs) - 1, 2)] + ([xs[-1]] if len(xs) % 2 else [])
    return xs[0]


def _needs(item):
    k = item[0]
    if k == "L":
        return lambda sg: sg[0] in "BQ" and sg[1] == item[1] and sg[2] < 2 * NT
    if k == "P":
        return lambda sg: sg[0] == "B" and sg[1] == item[1] and sg[2] == 2 * NT + item[3]
    if k == "E":
        return lambda sg: sg[0] == "D" and sg[1] == item[1] and sg[3] < item[3] and item[2] < sg[4]
    return lambda sg: False


def interleave(segs, tasks, lead=0):
    tasks = sorted(tasks, key=lambda t: t[0])
    starts, pos = [], 0
    for sg in segs:
        starts.append(pos)
        pos += (sg[-1] - sg[-2]) // 16
    pinned = [g for g, sg in enumerate(segs) if sg[-1] > sg[-2]]
    before = [[] for _ in range(len(segs) + 1)]
    prev = 0
    for slot, item in tasks:
        gs = [g for g in pinned if slot < starts[g] + (segs[g][-1] - segs[g][-2]) // 16]
        if not gs:
            before[len(segs)].append(item + ((0, 0),))
            continue
        g = gs[0]
        need = _needs(item)
        lo = max([i + 1 for i, sg in enumerate(segs) if need(sg)] + [0])
        ld = 0 if item[0] == "spec" else lead
        e = min(g, max(g - ld, lo, prev))
        prev = e
        cd = len([i for i in pinned if e <= i <= g])
        before[e].append(item + ((cd, max(slot - starts[g], 0)),))
    out = []
    for g, sg in enumerate(segs):
        out += before[g] + [sg]
    return out + before[len(segs)]


def _opts(s):
    if not isinstance(s, str):
        return dict(s)
    out = {}
    for kv in s.split(","):
        k, v = kv.split(":")
        v = [float(x) if "." in x else int(x) for x in v.split("/") if x]
        out[k] = v[0] if len(v) == 1 and not kv.endswith("/") else tuple(v)
    return out


def build_program(C0, CP, LS, SO, PO, PS, EDL, ADL, RL, SPEC, GL, GS, PRE, TL, PR, XB, NL, PF, LEAD):
    def B(b, g):
        return [("B", b, n, 0, T) for n in range(NT * g, NT * g + NT)]

    def Dm(b, lo=0, hi=T):
        return [("D", b, n, lo, hi) for n in range(NT)]

    def parts(kind, b, dls, lo=0, hi=T):
        n = (hi - lo) // len(dls)
        return [(8 * dl, (kind, b, lo + i * n, lo + (i + 1) * n)) for i, dl in enumerate(dls)]

    def LSt(b, c0, cp, rl=R, chunks=range(NC)):
        t = []
        for i, c in enumerate(chunks):
            base = c0 + cp * i
            for h in range(0, R, rl):
                sh = -(R - rl - h) * cp / R
                t += [(int(base + sh + LS * w), ("L", b, c, h, rl, w, GL)) for w in range(W)]
                t += [(int(base + sh + SO), ("S", b, c, h, rl, GS))]
        return t

    def Pt(b, c0, cp, chunks=range(NC)):
        t = []
        for i, c in enumerate(chunks):
            t += [(int(c0 + cp * i + PS * j), ("P", b, c, j, True)) for j in range(NT)]
        return t

    def Cf(b, c0=C0, cp=CP, rl=RL):
        return LSt(b, c0, cp, rl) + Pt(b, c0 + PO, cp)

    def Q(b, part):
        return [("Q", b, n, part, 0, T) for n in range(NT)]

    pr = dict(pv=(14, 6), l1=(40, 8), p0=(92, 3.5), np0=8, p1=(36, 5), c2=(84, 17.5), a3=(13,), e0=(16, 19), e1=(22, 25),
              a4=(20, 28), mv=(0, 0, 0, 0), mv1=(), mv2=(), pk=(39, 0), po=(16, 6), l0=(999, 0))
    pr.update(_opts(PR))
    mb, mc, md, me = pr["mv"]
    q21, k2, v2 = Q(2, 1), B(2, 1), B(2, 2)
    p = [("wait", "x0a"), ("A", 0, 0, T, (0, 0)), ("A", 1, 0, T, (0, 0)), ("wait", "wqa"), ("perm", 0, 0, KA)]
    p += Q(0, 0)
    p += [("wait", "x0b"), ("wait", "wqb"), ("perm", 0, KA, D), ("A", 2, 0, T, (0, 0)), ("drop",)]
    p += Q(1, 0) + Q(0, 1) + Q(1, 1) + Q(2, 0) + q21[:mb]
    p += [("wait", "wk")]
    mt = lambda g, d: [(d[0] + d[1] * i, ("merge", g, 128 * i, 128 * i + 128)) for i in range(NT)] if d else []
    p += interleave(q21[mb:] + B(0, 1) + B(1, 1) + k2[:mc],
                    mt(1, pr["mv1"]) + [(pr["pk"][0] + pr["pk"][1] * j, ("perm", 1, 0, D, (j,), None))
                                        for j in range(NT)] + LSt(0, *pr["l0"]))
    p += [("wait", "wv")]
    sh = lambda ts, d: [(t - d, it) for t, it in ts]
    p += interleave(k2[mc:] + B(0, 2) + B(1, 2) + v2[:md],
                    mt(2, pr["mv2"]) + [(pr["pv"][0] + pr["pv"][1] * j, ("perm", 2, 0, D, (j,))) for j in range(NT)]
                    + sh(LSt(1, *pr["l1"]) + Pt(0, *pr["p0"], range(pr["np0"])), 8 * mc), LEAD[0])
    p += [("wait", "wo"), ("wait", "wr"), ("wait", "x1")]
    p += interleave(v2[md:] + Dm(0) + Dm(1) + B(3, 0) + B(3, 1) + B(3, 2),
                    [(pr["po"][0] + pr["po"][1] * n, ("permo", n)) for n in range(NT)]
                    + sh(Pt(0, 10, 4, range(pr["np0"], NC)) + Pt(1, *pr["p1"]) + parts("A", 3, pr["a3"])
                       + parts("E", 0, pr["e0"]) + parts("E", 1, pr["e1"])
                       + Cf(2, *pr["c2"]) + parts("A", 4, pr["a4"]), 8 * md), LEAD[0])
    pf = [("PF", k, n) for n in range(F // 128) for k in range(2)] + [("PF", 2, n) for n in range(NT)]
    for s in range(3, NS - 2):
        segs = Dm(s - 1) + B(s + 1, 0) + B(s + 1, 1) + B(s + 1, 2)
        tasks = parts("E", s - 1, EDL) + Cf(s)
        if PF and s > XB:
            mine = pf[(s - XB - 1) * 5:(s - XB) * 5]
            tasks += [(PF + 28 * i, it) for i, it in enumerate(mine)]
        if s == XB:
            pre = [t for t in tasks if t[1][0] in "LS" and t[1][2] < PRE]
            tasks = sh([t for t in tasks if t not in pre], 8 * me)
            p += segs[:me] + [t[1] + ((0, 0),) for t in pre]
            segs = segs[me:]
            p += [("wait", "x2"), ("wait", "ffn")]
        if s + 2 < NS:
            tasks += sh(parts("A", s + 2, ADL), 8 * me if s == XB else 0)
        p += interleave(segs, tasks, LEAD[1])
    s = NS - 2
    big = Dm(s - 1) + B(s + 1, 0) + B(s + 1, 1) + Dm(s) + B(s + 1, 2)
    small = [("G", k, n, 0, 0) for n in range(F // 128) for k in range(2)] if SPEC else []
    tl = dict(e13=(9, 11), sp=12, c0=14, cp=12.5, l0=130, lp=4.5, pd=10, pp=0.75, e14=(186, 198), e15=243,
              gh=6, lr=16, cr=RL, cut=64, pl=0, pc=8, pb=200)
    if NL == 3:
        tl.update(e13=EDL, sp=1, gh=2)
    tl.update(_opts(TL))
    cut = tl["cut"]
    segs = []
    n_big = len(big) - tl["sp"]
    n_small = max(len(small) - tl["gh"], 0)
    done = 0
    for g, sg in enumerate(big):
        segs.append(sg)
        if g >= tl["sp"]:
            want = min(n_small, -(-(g - tl["sp"] + 1) * n_small // n_big))
            segs += small[done:want]
            done = want
    segs += small[done:] + Dm(s + 1, 0, cut) + Dm(s + 1, cut, T)
    if SPEC:
        segs += [("H", n, 0, 16) for n in range(NT)]
    n14 = len(tl["e14"])
    p15 = []
    for j in range(NT):
        for c in range(NC):
            early = j < tl["pl"] and c < tl["pc"]
            dl = int(160 + 8 * (j + 1) + tl["pd"] + tl["pp"] * c) if early else (200 if c < cut // R else tl["pb"])
            p15.append((dl, ("P", s + 1, c, j, early)))
    tasks = (parts("E", s - 1, tl["e13"]) + ([(8 * tl["sp"], ("spec",))] if SPEC else [])
             + Cf(s, tl["c0"], tl["cp"], tl["cr"]) + LSt(s + 1, tl["l0"], tl["lp"], tl["lr"]) + p15
             + [(dl, ("E", s, i * T // n14, (i + 1) * T // n14)) for i, dl in enumerate(tl["e14"])]
             + [(tl["e15"], ("E", s + 1, 0, cut)), (999, ("E", s + 1, cut, T))])
    p += interleave(segs, tasks, LEAD[2])
    return p


def make_kernel(C0=16, CP=17.5, LS=0, SO=8, PO=10, PS=1, EDL=(12, 18), ADL=(7, 16),
                prof=0, pins=1, RL=8, FA=3, FS=0, SPEC=1, ALT=0, HD=1, GL=0, GS=1, PRE=2, TL=(), G=2, PR=(), XB=7, NL=2, RB=0, PO_GATE=0, PF=0, LEAD=(0, 0, 0)):
    X1 = (XB - 1) * T
    XCH = (2 * T, T, X1, S - 3 * T - X1)
    prog = build_program(C0, CP, LS, SO, PO, PS, EDL, ADL, RL, SPEC, GL, GS, PRE, TL, PR, XB, NL, PF, LEAD)
    LATE = (NS - NL) * T

    def wait(c, name):
        if prof:
            with jax.named_scope("w_" + name):
                c.wait()
        else:
            c.wait()

    def kernel(x_hbm, wqkv_hbm, wo_hbm, wr_hbm, wg_hbm, wu_hbm, wd_hbm, out_hbm,
               x_s, wqkv_s, wo_s, wob_s, wr_s, wg_s, wu_s, wd_s, wp_s, wop_s,
               k_s, v_s, xn_s, o_s, hn_s, out_s, y_s, act_s, sem_in, sem_out):
        pid = pl.program_id(0)
        step = pid - (1 if G == 2 else 0)
        cp = {}
        semi = dict(x0a=0, wqa=1, x0b=6, wqb=6, wk=2, wv=3, wo=4, wr=4, x1=4, x2=5, ffn=5)
        r0 = 0
        for nm, n in zip(("x0a", "x0b", "x1", "x2"), XCH):
            cp[nm] = [pltpu.make_async_copy(x_hbm.at[pl.ds(r0, n)], x_s.at[pl.ds(r0, n)], sem_in.at[semi[nm]])]
            r0 += n
        f = 2 if RB else 1
        view = (lambda r: r.bitcast(U32)) if RB else (lambda r: r)
        asu32 = (lambda v: v) if RB else (lambda v: pltpu.bitcast(v, U32))
        asbf16 = (lambda v: pltpu.bitcast(v, BF16)) if RB else (lambda v: v)
        for nm, lo, hi, g in (("wqa", 0, KA, 0), ("wqb", KA, D, 0), ("wk", 0, D, 1), ("wv", 0, D, 2)):
            sl = (pl.ds(lo // f, (hi - lo) // f), pl.ds(D * g, D))
            cp[nm] = [pltpu.make_async_copy(view(wqkv_hbm).at[sl], wqkv_s.at[sl], sem_in.at[semi[nm]])]
        if RB:
            cp["wo"] = [pltpu.make_async_copy(view(wo_hbm).at[:, pl.ds(128 * n, 128)],
                                              wo_s.at[n, pl.ds(0, D // 2)], sem_in.at[semi["wo"]])
                        for n in range(NT)]
        else:
            cp["wo"] = [pltpu.make_async_copy(wo_hbm, wob_s, sem_in.at[semi["wo"]])]
        cp["wr"] = [pltpu.make_async_copy(wr_hbm, wr_s, sem_in.at[semi["wr"]])]
        cp["ffn"] = [pltpu.make_async_copy(view(a), b, sem_in.at[semi["ffn"]])
                     for i, (a, b) in enumerate(((wg_hbm, wg_s), (wu_hbm, wu_s), (wd_hbm, wd_s)))]

        def ocp(lo, hi):
            return pltpu.make_async_copy(out_s.at[pl.ds(lo, hi - lo)], out_hbm.at[pl.ds(lo, hi - lo)],
                                         sem_out.at[0 if lo < LATE else 1])

        def start_all():
            first = ("x0a", "wqa", "x0b", "wqb")
            for nm in first + ("wk", "wv", "wo", "wr", "x1", "x2", "ffn"):
                for c in cp[nm]:
                    c.start()

        def main():
            zero = jnp.zeros((HALO, 128), F32)
            for j in range(NT):
                k_s[j, 0:HALO, :] = zero
                v_s[j, 0:HALO, :] = zero

            lane = lax.broadcasted_iota(jnp.int32, (1, 128), 1)
            cm5 = [(lane + 128 * t) - 5 * (((lane + 128 * t) * 52429) >> 18) for t in range(NT - 1)]
            srcs = [(20 * (lane & 31) + 5 * (lane >> 5) + j) & 127 for j in range(NT)]
            never = jnp.full((8, 128), step, jnp.int32) > 0
            st = dict(best=None, toks=[], wr=None, late=[])
            q, a, lgs, sm, gu = {}, {}, {}, {}, {}

            def pin(u):
                st["late"] += [(cd, sl, t) for (cd, sl), t in st["toks"]]
                st["toks"] = []
                toks = [(sl, t) for cd, sl, t in st["late"] if cd <= 1]
                st["late"] = [(cd - 1, sl, t) for cd, sl, t in st["late"] if cd > 1]
                if toks and pins:
                    ng = u.shape[0] // 8
                    rows = []
                    for i in range(ng):
                        mine = [t for g, t in toks if min(g, ng - 1) == i]
                        blk = u[8 * i:8 * i + 8]
                        if mine:
                            t = functools.reduce(lambda x, y: x | y, mine)
                            head = jnp.where(never, t, blk[:, 0:128])
                            blk = jnp.concatenate([head, blk[:, 128:]], axis=1)
                        rows.append(blk)
                    u = jnp.concatenate(rows, axis=0)
                return pltpu.bitcast(u, BF16)

            def merge_w(g, k0, k1, slot=None):
                tiles = [asu32(wqkv_s[pl.ds(k0 // f, (k1 - k0) // f), pl.ds(D * g + 128 * t, 128)])
                         for t in range(NT)]
                for j in range(NT):
                    m = tiles[NT - 1]
                    for t in range(NT - 2, -1, -1):
                        m = jnp.where(cm5[t] == j, tiles[t], m)
                    st["mw", g, k0, j] = m
                    if slot is not None:
                        st["toks"].append((slot, _or_all(m)))

            def permute_w(g, k0, k1, js=range(NT), slot=None, *unused):
                for j in js:
                    ks = sorted(k[2] for k in st if k[:2] == ("mw", g) and k[3] == j and k0 <= k[2] < k1)
                    if not ks:
                        merge_w(g, k0, k1)
                        ks = [k0]
                    m = jnp.concatenate([st.pop(("mw", g, k, j)) for k in ks], axis=0)
                    idx = jnp.broadcast_to(srcs[j], m.shape)
                    res = jnp.take_along_axis(m, idx, axis=1, mode="promise_in_bounds")
                    wp_s[pl.ds(k0 // 2, (k1 - k0) // 2), pl.ds(D * g + 128 * j, 128)] = res
                    if slot is not None:
                        st["toks"].append((slot, _or_all(res)))

            def permute_wo(n, slot=None):
                if not RB:
                    wo_s[n, pl.ds(0, D // 2), :] = pltpu.bitcast(wob_s[:, pl.ds(128 * n, 128)], U32)
                vals = []
                for d2 in range(DH // 2):
                    ev = wo_s[n, pl.ds(d2, H // 2, stride=DH), :]
                    od = wo_s[n, pl.ds(DH // 2 + d2, H // 2, stride=DH), :]
                    lo = (ev & jnp.uint32(0xFFFF)) | (od << 16)
                    hi = (ev >> 16) | (od & jnp.uint32(0xFFFF0000))
                    for d, val in ((2 * d2, lo), (2 * d2 + 1, hi)):
                        aa, j = divmod(d, NT)
                        wop_s[pl.ds(64 * j + 16 * aa, H // 2), pl.ds(128 * n, 128)] = val
                        vals.append(val)
                if slot is not None and PO_GATE:
                    st["toks"].append((slot, _or_all(jnp.concatenate(vals, axis=0))))

            def a_task(b, lo, hi, slot):
                r0, n = b * T + lo, hi - lo
                x = x_s[pl.ds(r0, n), :].astype(F32)
                m = jnp.sum(x, axis=-1, keepdims=True) * (1.0 / D)
                c = x - m
                v = jnp.sum(c * c, axis=-1, keepdims=True) * (1.0 / D)
                rstd = lax.rsqrt(v + EPS)
                xn = (x * rstd - m * rstd) if ALT else c * rstd
                xn_s[pl.ds(r0 // 2, n // 2), :] = pltpu.bitcast(xn.astype(BF16), U32)
                st["toks"].append((slot, _or_all(xn_s[pl.ds(r0 // 2, n // 2), :])))

            def b_seg(b, n, lo, hi):
                w = pltpu.bitcast(wp_s[:, pl.ds(128 * n, 128)], BF16)
                lhs = pin(xn_s[pl.ds((b * T + lo) // 2, (hi - lo) // 2), :])
                acc = jnp.dot(lhs, w, preferred_element_type=F32)
                g, j = divmod(n, NT)
                if g == 0:
                    acc = acc * QSCALE
                if FA:
                    st["late"].append((FA, FS, _or_all(pltpu.bitcast(acc, U32))))
                if g == 0:
                    for r in range(lo, hi, 8):
                        q[b * T + r, j] = acc[r - lo:r - lo + 8]
                else:
                    (k_s if g == 1 else v_s)[j, pl.ds(HALO + b * T + lo, hi - lo), :] = acc

            def q_seg(b, n, part, lo, hi):
                k0, k1 = ((0, KA), (KA, D))[part]
                w = pltpu.bitcast(wp_s[pl.ds(k0 // 2, (k1 - k0) // 2), pl.ds(128 * n, 128)], BF16)
                lhs = pin(xn_s[pl.ds(b * T // 2, T // 2), pl.ds(k0, k1 - k0)])
                acc = jnp.dot(lhs, w, preferred_element_type=F32)
                if part == 0:
                    st["qa", b, n] = acc
                else:
                    acc = (acc + st.pop(("qa", b, n))) * QSCALE
                    for r in range(0, T, 8):
                        q[b * T + r, n] = acc[r:r + 8]

            def l_task(b, c, h, RL, w, gate, slot):
                r0 = b * T + c * R + h
                qc = [jnp.concatenate([q[r0 + r, j] for r in range(0, RL, 8)], axis=0) for j in range(NT)]
                off = HALO + r0 - DIL * w
                p = qc[0] * k_s[0, pl.ds(off, RL), :]
                for j in range(1, NT):
                    p = p + qc[j] * k_s[j, pl.ds(off, RL), :]
                p = p + pltpu.roll(p, 64, 1)
                p = p + pltpu.roll(p, 32, 1)
                if r0 - DIL * w < 0:
                    pos = lax.broadcasted_iota(jnp.int32, (RL, 128), 0) + (r0 - DIL * w)
                    p = jnp.where(pos >= 0, p, -1e9)
                lgs[r0, w] = p
                if gate:
                    st["toks"].append((slot, _or_all(pltpu.bitcast(p, U32))))

            def s_task(b, c, h, RL, gate, slot):
                r0 = b * T + c * R + h
                lg = [lgs.pop((r0, w)) for w in range(W)]
                m = _tree(jnp.maximum, lg)
                e = [jnp.exp2(l - m) for l in lg]
                inv = pl.reciprocal(_tree(jnp.add, e), approx=True)
                for r in range(0, RL, 8):
                    sm[r0 + r] = [t[r:r + 8] for t in e + [inv]]
                if gate:
                    st["toks"].append((slot, _or_all(pltpu.bitcast(inv, U32))))

            def p_task(b, c, j, gate, slot):
                r0 = b * T + c * R
                ei = [jnp.concatenate([sm[r0 + h][w] for h in range(0, R, 8)], axis=0) for w in range(W + 1)]
                e, inv = ei[:W], ei[W]
                acc = None
                for w in range(W):
                    off = HALO + r0 - DIL * w
                    t = e[w] * v_s[j, pl.ds(off, R), :]
                    acc = t if acc is None else acc + t
                dst = (pl.ds(r0 // 2, R // 2), pl.ds(128 * j, 128))
                o_s[dst] = pltpu.bitcast((acc * inv).astype(BF16), U32)
                if gate:
                    st["toks"].append((slot, o_s[dst]))

            def d_seg(b, n, lo, hi):
                w = pltpu.bitcast(wop_s[:, pl.ds(128 * n, 128)], BF16)
                lhs = pin(o_s[pl.ds((b * T + lo) // 2, (hi - lo) // 2), :])
                acc = jnp.dot(lhs, w, preferred_element_type=F32)
                if HD:
                    acc = acc + x_s[pl.ds(b * T + lo, hi - lo), pl.ds(128 * n, 128)].astype(F32)
                if FA and hi - lo == T and (b, n) < (NS - 2, 3):
                    st["late"].append((FA, FS, _or_all(pltpu.bitcast(acc, U32))))
                for r in range(lo, hi, 8):
                    a[b * T + r, n] = acc[r - lo:r - lo + 8]

            def e_task(b, lo, hi, slot):
                r0, n = b * T + lo, hi - lo
                cols = []
                for j in range(NT):
                    cols.append(jnp.concatenate([a[r0 + r, j] for r in range(0, n, 8)], axis=0))
                if st["wr"] is None:
                    st["wr"] = wr_s[...].astype(F32).reshape(1, D)
                h = jnp.concatenate(cols, axis=1)
                if not HD:
                    h = x_s[pl.ds(r0, n), :].astype(F32) + h
                m = jnp.sum(h, axis=-1, keepdims=True) * (1.0 / D)
                c = h - m
                v = jnp.sum(c * c, axis=-1, keepdims=True) * (1.0 / D)
                cw = jnp.sum(c * st["wr"], axis=-1, keepdims=True)
                rstd = lax.rsqrt(v + EPS)
                hn = (h * rstd - m * rstd) if ALT else c * rstd
                out_s[pl.ds(pl.multiple_of(step * 16 + r0, 16), n), :] = (h + hn).astype(BF16)
                hn_s[pl.ds(r0 // 2, n // 2), :] = pltpu.bitcast(hn.astype(BF16), U32)
                r = jnp.broadcast_to(cw * rstd, (n, 128))
                best = st["best"]
                for i in range(n // 8):
                    ri = r[8 * i:8 * i + 8]
                    rows = lax.broadcasted_iota(jnp.int32, (8, 128), 0) + (r0 + 8 * i)
                    if best is None:
                        best = (jnp.where(ri > -jnp.inf, ri, -jnp.inf), rows)
                    else:
                        bv, bi = best
                        upd = ri > bv
                        best = (jnp.where(upd, ri, bv), jnp.where(upd, rows, bi))
                st["best"] = best
                if b == NS - 1:
                    ocp(r0, r0 + n).start()
                elif hi == T:
                    ocp(b * T, (b + 1) * T).start()
                probe = hn_s[pl.ds(pl.multiple_of(step * 8, 8), 8), 0:128]
                probe2 = pltpu.bitcast(out_s[0:16, 0:128], U32)
                st["toks"].append((slot, pltpu.bitcast(best[0], U32) | pltpu.bitcast(best[1], U32) | probe | probe2))

            def spec_task(slot):
                st["spec"] = argmax(st["best"])[1]
                st["xs"] = load_chunk(st["spec"], LATE)

            def pf_task(k, n, slot):
                u = asu32((wg_s, wu_s, wd_s)[k][:, pl.ds(128 * n, 128)])
                st["pf", k, n] = u
                st["toks"].append((slot, _or_all(u)))

            def ffn_w(k, n):
                if ("pf", k, n) in st:
                    return pltpu.bitcast(st["pf", k, n], BF16)
                return asbf16((wg_s, wu_s, wd_s)[k][:, pl.ds(128 * n, 128)])

            def g_seg(k, n, lo, hi):
                w = ffn_w(k, n)
                gu[k, n] = jnp.dot(st["xs"], w, preferred_element_type=F32)

            def h_seg(n, lo, hi):
                if "act" not in st:
                    g = jnp.concatenate([gu[0, i] for i in range(F // 128)], axis=1)
                    u = jnp.concatenate([gu[1, i] for i in range(F // 128)], axis=1)
                    act_s[...] = pltpu.bitcast((g * jax.nn.sigmoid(g) * u).astype(BF16), U32)
                    st["act"] = True
                w = ffn_w(2, n)
                y_s[:, pl.ds(128 * n, 128)] = jnp.dot(pin(act_s[...]), w, preferred_element_type=F32)

            def do_wait(nm):
                st["toks"] = []
                st["late"] = []
                for c in cp[nm]:
                    wait(c, nm)

            fns = dict(drop=lambda: st.update(toks=[]), A=a_task, B=b_seg, Q=q_seg, L=l_task, S=s_task, P=p_task, D=d_seg, E=e_task, wait=do_wait,
                       perm=permute_w, merge=merge_w, permo=permute_wo, spec=spec_task, PF=pf_task, G=g_seg, H=h_seg)
            for item in prog:
                fns[item[0]](*item[1:])
            return st["best"], st.get("spec")

        def argmax(best):
            bv, bi = best
            mx = jnp.max(bv, axis=0, keepdims=True)
            idx = jnp.min(jnp.where(bv >= mx, bi, S - 1), axis=0, keepdims=True)
            return mx[:, 0:1], jnp.clip(idx[0, 0], 0, S - 1)

        def load_chunk(idx, nrows):
            blk = jnp.clip(idx >> 4, 0, nrows // 16 - 1)
            return pltpu.bitcast(hn_s[pl.ds(pl.multiple_of(blk * 8, 8), 8), :], BF16)

        def ffn(idx):
            xs = load_chunk(idx, S)
            g = jnp.dot(xs, asbf16(wg_s[...]), preferred_element_type=F32)
            u = jnp.dot(xs, asbf16(wu_s[...]), preferred_element_type=F32)
            act = (g * jax.nn.sigmoid(g) * u).astype(BF16)
            y_s[...] = jnp.dot(act, asbf16(wd_s[...]), preferred_element_type=F32)

        def fix_row(mx, idx, nrows):
            base = pl.multiple_of(jnp.clip(idx >> 4, 0, nrows // 16 - 1) * 16, 16)
            y = y_s[...] * jax.nn.sigmoid(mx)
            cur = out_s[pl.ds(base, 16), :].astype(F32)
            rows = lax.broadcasted_iota(jnp.int32, (16, D), 0) + base
            out_s[pl.ds(base, 16), :] = jnp.where(rows == idx, cur + y, cur).astype(BF16)
            fix = pltpu.make_async_copy(out_s.at[pl.ds(base, 16)], out_hbm.at[pl.ds(base, 16)], sem_out.at[2])
            fix.start()
            return fix

        def tail(best, spec):
            mx, idx = argmax(best)
            wait(ocp(0, LATE), "out0")

            def early():
                if spec is None:
                    ffn(idx)
                fix = fix_row(mx, idx, LATE)
                wait(ocp(LATE, S), "out1")
                wait(fix, "fix")

            def late():
                ffn(idx)
                wait(ocp(LATE, S), "out1")
                wait(fix_row(mx, idx, S), "fix")

            lax.cond(idx < LATE, early, late)

        if G == 2:
            pl.when(pid == 0)(start_all)

            @pl.when(pid == 1)
            def _():
                tail(*main())
        else:
            start_all()
            tail(*main())

    @jax.jit
    def fn(A_x, A_wqkv, A_wo, B_x, B_w_r, B_w_gate, B_w_up, B_w_down):
        any_spec = pl.BlockSpec(memory_space=pl.ANY)
        wsc = (lambda r, c: pltpu.VMEM((r // 2, c), U32)) if RB else (lambda r, c: pltpu.VMEM((r, c), BF16))
        out = pl.pallas_call(
            kernel,
            grid=(G,),
            out_shape=jax.ShapeDtypeStruct((S, D), BF16),
            in_specs=[any_spec] * 7,
            out_specs=any_spec,
            scratch_shapes=[
                pltpu.VMEM((S, D), BF16),
                wsc(D, 3 * D),
                pltpu.VMEM((NT, D // 2 + 32, 128), U32),
                pltpu.VMEM((D, D), BF16),
                pltpu.VMEM((D,), BF16),
                wsc(D, F),
                wsc(D, F),
                wsc(F, D),
                pltpu.VMEM((D // 2, 3 * D), U32),
                pltpu.VMEM((D // 2, D), U32),
                pltpu.VMEM((NT, S + HALO, 128), F32),
                pltpu.VMEM((NT, S + HALO, 128), F32),
                pltpu.VMEM((S // 2, D), U32),
                pltpu.VMEM((S // 2, D), U32),
                pltpu.VMEM((S // 2, D), U32),
                pltpu.VMEM((S + 16, D), BF16),
                pltpu.VMEM((16, D), F32),
                pltpu.VMEM((8, F), U32),
                pltpu.SemaphoreType.DMA((7,)),
                pltpu.SemaphoreType.DMA((3,)),
            ],
            compiler_params=pltpu.CompilerParams(vmem_limit_bytes=100 << 20,
                                                 dimension_semantics=("arbitrary",),
                                                 disable_bounds_checks=True,
                                                 disable_semaphore_checks=True),
            name="fused",
        )(A_x.reshape(S, D), A_wqkv, A_wo, B_w_r, B_w_gate, B_w_up, B_w_down)
        return out.reshape(1, S, D)

    return fn


pallas_sequential_preLN__sliding_local_dilated__moe_arch_mod__prompt_kernel = make_kernel()
```

```python
import functools
import math
import jax
import jax.numpy as jnp
from jax import lax
import jax.experimental.pallas as pl
import jax.experimental.pallas.tpu as pltpu

S, D, F = 2048, 640, 1536
H, DH, W, DIL = 32, 20, 8, 2
NT = D // 128
HALO = 16
EPS = 1e-5
F32, BF16, U32 = jnp.float32, jnp.bfloat16, jnp.uint32
QSCALE = DH ** -0.5 * math.log2(math.e)
R = 16
T = 128
NS = S // T
NC = T // R
KA = 384
LATE = (NS - 2) * T
XB = 7


def _or_all(u):
    t = None
    for i in range(u.shape[0] // 8):
        for j in range(u.shape[1] // 128):
            p = u[8 * i:8 * i + 8, 128 * j:128 * (j + 1)]
            t = p if t is None else t | p
    return t


def _tree(f, xs):
    xs = list(xs)
    while len(xs) > 1:
        xs = [f(xs[i], xs[i + 1]) for i in range(0, len(xs) - 1, 2)] + ([xs[-1]] if len(xs) % 2 else [])
    return xs[0]


def _opts(s):
    if not isinstance(s, str):
        return dict(s)
    out = {}
    for kv in s.split(","):
        k, v = kv.split(":")
        v = [float(x) if "." in x else int(x) for x in v.split("/") if x]
        out[k] = v[0] if len(v) == 1 and not kv.endswith("/") else tuple(v)
    return out


def _rows(lo, hi):
    return range(lo, hi, R)


def _io(it):
    k = it[0]
    lhs = lambda g, b, lo=0, hi=T: [("o" if g == 3 else "xn", b, r, j) for r in _rows(lo, hi) for j in range(NT)]
    out = lambda g, b, n, lo=0, hi=T: [("y", g, b, n, r) for r in _rows(lo, hi)]
    if k == "A":
        return [], lhs(0, *it[1:4])
    if k == "M":
        _, g, b, n, lo, hi = it
        return lhs(g, b, lo, hi) + [("w", g, n, 0), ("w", g, n, 1)], out(g, b, n, lo, hi)
    if k == "Q":
        _, b, n, part = it
        return lhs(0, b) + [("w", 0, n, part)], (out(0, b, n) if part else [])
    if k == "perm":
        _, g, k0, k1, js = it
        return [], [("w", g, j, p) for j in js for p in (0, 1) if (k0, k1)[p] == (0, D)[p]]
    if k == "permo":
        return [], [("w", 3, it[1], 0), ("w", 3, it[1], 1)]
    if k == "L":
        _, r0, n, w = it
        b, r = divmod(r0, T)
        return [("y", g, b, j, r // R * R) for g in (0, 1) for j in range(NT)], [("lg", r0, w)]
    if k == "S":
        _, r0, n = it
        return [("lg", r0, w) for w in range(W)], [("sm", r0 + r) for r in range(0, n, 8)]
    if k == "P":
        _, b, c, j = it
        return ([("sm", b * T + c * R + r) for r in range(0, R, 8)] + [("y", 2, b, j, c * R)],
                [("o", b, c * R, j)])
    if k == "E":
        _, b, lo, hi = it
        prev = [("e", b * T + lo - R)] if b * T + lo else []
        return ([("y", 3, b, n, r) for n in range(NT) for r in _rows(lo, hi)] + prev,
                [("e", b * T + r) for r in _rows(lo, hi)])
    if k == "spec":
        return [("e", LATE - R)], [("spec",)]
    if k == "G":
        return [("spec",)], [("g",) + it[1:]]
    if k == "H":
        return [("g", kk, n) for kk in range(2) for n in range(F // 128)], []
    return [], []


def _slots(it):
    k = it[0]
    if k == "M":
        return (it[5] - it[4]) / 16
    if k == "Q":
        return 1.6 * (3, 2)[it[3]]
    return {"G": 0.0, "H": 1.0}[k]


class Plan:
    def __init__(self):
        self.prog, self.pos, self.have, self.todo = [], 0.0, set(), []

    def _put(self, it, extra):
        self.prog.append(it + (extra,))
        self.have.update(_io(it)[1])

    def _emit_task(self, t, force=False):
        due, it = t
        for key in _io(it)[0]:
            if key not in self.have:
                src = [u for u in self.todo if key in _io(u[1])[1]]
                if not src or not self._emit_task(src[0], force):
                    assert not force, ("unsatisfied", it, key)
                    return False
        self.todo.remove(t)
        self._put(it, due)
        return True

    def tasks(self, ts):
        self.todo += [(None if d is None else self.pos + d, it) for d, it in ts]

    def mxu(self, segs):
        for sg in segs:
            end = self.pos + _slots(sg)
            for t in sorted([t for t in self.todo if t[0] is not None and t[0] < end], key=lambda t: t[0]):
                if t in self.todo:
                    self._emit_task(t)
            for key in _io(sg)[0]:
                if key not in self.have:
                    src = [u for u in self.todo if key in _io(u[1])[1]]
                    assert src, ("unsatisfied", sg, key)
                    self._emit_task(src[0], True)
            self._put(sg, (self.pos, end))
            self.pos = end

    def flush(self, pred=lambda it: True):
        for t in [t for t in self.todo if pred(t[1])]:
            if t in self.todo:
                self._emit_task(t, True)

    def wait(self, *names):
        self.prog += [("wait", n) for n in names]


def build_program(o):
    M = lambda g, b, lo=0, hi=T: [("M", g, b, n, lo, hi) for n in range(NT)]
    Q = lambda b, part: [("Q", b, n, part) for n in range(NT)]

    def parts(kind, b, dls):
        n = T // len(dls)
        return [(dl, (kind, b, i * n, (i + 1) * n)) for i, dl in enumerate(dls)]

    def LS(b, c0, cp, rl=R):
        t = []
        for c in range(NC):
            for h in range(0, R, rl):
                r0 = b * T + c * R + h
                t += [(None, ("L", r0, rl, w)) for w in range(W)]
                t += [(None if c0 is None else c0 + cp * c - (R - rl - h) * cp / R, ("S", r0, rl))]
        return t

    def Pt(b, c0, cp):
        return [(None if c0 is None else c0 + cp * c + o["ps"] * j, ("P", b, c, j))
                for c in range(NC) for j in range(NT)]

    def C(b, c0, cp):
        return LS(b, c0, cp, o["rl"]) + Pt(b, c0 + o["po"], cp)

    allj = tuple(range(NT))
    p = Plan()
    p.wait("x0a")
    p.tasks(parts("A", 0, (None,)) + parts("A", 1, (None,)))
    p.flush()
    p.wait("wqa")
    p.tasks([(None, ("perm", 0, 0, KA, allj))])
    p.mxu(Q(0, 0))
    p.wait("x0b", "wqb")
    p.tasks([(None, ("perm", 0, KA, D, allj))] + parts("A", 2, (None,)))
    p.flush()
    p.mxu(Q(1, 0) + Q(0, 1) + Q(1, 1) + Q(2, 0))
    p.wait("wk")
    p.tasks([(None, ("perm", 1, 0, D, allj))] + LS(0, None, 0))
    p.mxu(Q(2, 1) + M(1, 0) + M(1, 1))
    p.flush()
    p.wait("wv")
    p.tasks([(o["pv"][0] + o["pv"][1] * j, ("perm", 2, 0, D, (j,))) for j in range(NT)]
            + LS(1, *o["l1"]) + Pt(0, *o["p0"]))
    p.mxu(M(1, 2) + M(2, 0) + M(2, 1))
    p.flush()
    p.wait("wo", "wr", "x1")
    p.tasks([(None, ("permo", n)) for n in range(NT)])
    p.tasks(Pt(1, *o["p1"]) + parts("A", 3, o["a3"]) + parts("E", 0, o["e0"])
            + parts("E", 1, o["e1"]) + C(2, *o["c2"]) + parts("A", 4, o["a4"]))
    p.mxu(M(2, 2) + M(3, 0) + M(3, 1) + M(0, 3) + M(1, 3) + M(2, 3))
    for s in range(3, NS - 2):
        tasks = parts("E", s - 1, o["e"]) + C(s, *o["c"]) + parts("A", s + 2, o["a"])
        if s == XB:
            pre = [t for t in tasks if t[1][0] in "LS" and t[1][1] < s * T + o["pre"] * R]
            p.tasks([(None, t[1]) for t in pre])
            tasks = [t for t in tasks if t not in pre]
            p.flush()
            p.wait("x2", "ffn")
        p.tasks(tasks)
        p.mxu(M(3, s - 1) + M(0, s + 1) + M(1, s + 1) + M(2, s + 1))
    s = NS - 2
    big = M(3, s - 1) + M(0, s + 1) + M(1, s + 1) + M(3, s) + M(2, s + 1)
    small = [("G", k, n) for n in range(F // 128) for k in range(2)]
    cut = o["cut"]
    segs = []
    n_big, n_small, done = len(big) - o["sp"], len(small) - o["gh"], 0
    for g, sg in enumerate(big):
        segs.append(sg)
        if g >= o["sp"]:
            want = min(n_small, -(-(g - o["sp"] + 1) * n_small // n_big))
            segs += small[done:want]
            done = want
    segs += small[done:] + M(3, s + 1, 0, cut) + M(3, s + 1, cut, T) + [("H", n) for n in range(NT)]
    p.tasks(parts("E", s - 1, o["e13"]) + [(None, ("spec",))] + C(s, *o["c14"])
            + LS(s + 1, *o["l15"]) + Pt(s + 1, None, 0) + parts("E", s, o["e14"])
            + [(o["e15"], ("E", s + 1, 0, cut)), (None, ("E", s + 1, cut, T))])
    p.mxu(segs)
    p.flush()
    return p.prog


DEFAULTS = dict(
    mode="", rl=8, ps=3, po=2, fa=16, pre=2,
    pv=(13, 6), l1=(52, 8), p0=(92, 3.5),
    p1=(36, 17), a3=(100,), e0=(132, 152), e1=(176, 200), c2=(92, 17.5), a4=(160, 224),
    e=(96, 144), c=(24, 17.5), a=(64, 136),
    cut=64, sp=12, gh=6, e13=(72, 88), c14=(22, 12.25), l15=(138, 4.5), e14=(184, 198), e15=243)


def make_kernel(prof=0, O=(), **kw):
    o = dict(DEFAULTS)
    o.update(_opts(O))
    o.update(kw)
    prog = build_program(o)
    x1 = (XB - 1) * T
    xch = (2 * T, T, x1, S - 3 * T - x1)

    def wait(c, name):
        if prof:
            with jax.named_scope("w_" + name):
                c.wait()
        else:
            c.wait()

    def kernel(x_hbm, wqkv_hbm, wo_hbm, wr_hbm, wg_hbm, wu_hbm, wd_hbm, out_hbm,
               x_s, wqkv_s, wo_s, wob_s, wr_s, wg_s, wu_s, wd_s, wp_s,
               k_s, v_s, xn_s, o_s, hn_s, out_s, y_s, act_s, sem_in, sem_out):
        pid = pl.program_id(0)
        step = pid - 1
        cp = {}
        semi = dict(x0a=0, wqa=1, x0b=6, wqb=6, wk=2, wv=3, wo=4, wr=4, x1=4, x2=5, ffn=5)
        r0 = 0
        for nm, n in zip(("x0a", "x0b", "x1", "x2"), xch):
            cp[nm] = [pltpu.make_async_copy(x_hbm.at[pl.ds(r0, n)], x_s.at[pl.ds(r0, n)], sem_in.at[semi[nm]])]
            r0 += n
        for nm, lo, hi, g in (("wqa", 0, KA, 0), ("wqb", KA, D, 0), ("wk", 0, D, 1), ("wv", 0, D, 2)):
            sl = (pl.ds(lo, hi - lo), pl.ds(D * g, D))
            cp[nm] = [pltpu.make_async_copy(wqkv_hbm.at[sl], wqkv_s.at[sl], sem_in.at[semi[nm]])]
        cp["wo"] = [pltpu.make_async_copy(wo_hbm, wob_s, sem_in.at[semi["wo"]])]
        cp["wr"] = [pltpu.make_async_copy(wr_hbm, wr_s, sem_in.at[semi["wr"]])]
        cp["ffn"] = [pltpu.make_async_copy(a, b, sem_in.at[semi["ffn"]])
                     for a, b in ((wg_hbm, wg_s), (wu_hbm, wu_s), (wd_hbm, wd_s))]

        def ocp(lo, hi):
            return pltpu.make_async_copy(out_s.at[pl.ds(lo, hi - lo)], out_hbm.at[pl.ds(lo, hi - lo)],
                                         sem_out.at[0 if lo < LATE else 1])

        def start_all():
            for nm in ("x0a", "wqa", "x0b", "wqb", "wk", "wv", "wo", "wr", "x1", "x2", "ffn"):
                for c in cp[nm]:
                    c.start()

        def main():
            zero = jnp.zeros((HALO, 128), F32)
            for j in range(NT):
                k_s[j, 0:HALO, :] = zero
                v_s[j, 0:HALO, :] = zero

            lane = lax.broadcasted_iota(jnp.int32, (1, 128), 1)
            cm5 = [(lane + 128 * t) - 5 * (((lane + 128 * t) * 52429) >> 18) for t in range(NT - 1)]
            srcs = [(20 * (lane & 31) + 5 * (lane >> 5) + j) & 127 for j in range(NT)]
            never = jnp.full((8, 128), step, jnp.int32) > 0
            st = dict(best=None, toks=[], wr=None)
            q, hh, lgs, sm, gu, part = {}, {}, {}, {}, {}, {}
            pack = lambda v: pltpu.bitcast(v.astype(BF16), U32)
            rsqrt = lambda v: jnp.exp2(jnp.log(v) * (-0.5 / math.log(2.0)))

            def token(due, u):
                if due is not None:
                    st["toks"].append((due, u()))

            def mm(lhs, w, span):
                start, end = span
                toks = [t for t in st["toks"] if t[0] < end]
                st["toks"] = [t for t in st["toks"] if t[0] >= end]
                if toks:
                    ng = lhs.shape[0] // 8
                    rows = []
                    for i in range(ng):
                        mine = [t for d, t in toks if min(max(int(d - start), 0), ng - 1) == i]
                        blk = lhs[8 * i:8 * i + 8]
                        if mine:
                            head = jnp.where(never, functools.reduce(lambda x, y: x | y, mine), blk[:, 0:128])
                            blk = jnp.concatenate([head, blk[:, 128:]], axis=1)
                        rows.append(blk)
                    lhs = jnp.concatenate(rows, axis=0)
                if w.dtype == U32:
                    w = pltpu.bitcast(w, BF16)
                return jnp.dot(pltpu.bitcast(lhs, BF16), w, preferred_element_type=F32)

            def permute_w(g, k0, k1, js, due):
                if ("mw", g, k0) not in st:
                    tiles = [pltpu.bitcast(wqkv_s[pl.ds(k0, k1 - k0), pl.ds(D * g + 128 * t, 128)], U32)
                             for t in range(NT)]
                    st["mw", g, k0] = []
                    for j in range(NT):
                        m = tiles[NT - 1]
                        for t in range(NT - 2, -1, -1):
                            m = jnp.where(cm5[t] == j, tiles[t], m)
                        st["mw", g, k0].append(m)
                for j in js:
                    m = st["mw", g, k0][j]
                    res = jnp.take_along_axis(m, jnp.broadcast_to(srcs[j], m.shape), axis=1,
                                              mode="promise_in_bounds")
                    wp_s[pl.ds(k0 // 2, (k1 - k0) // 2), pl.ds(D * g + 128 * j, 128)] = res
                    token(due, lambda: _or_all(res))

            def permute_wo(n, due):
                wo_s[n, pl.ds(0, D // 2), :] = pltpu.bitcast(wob_s[:, pl.ds(128 * n, 128)], U32)
                for d2 in range(DH // 2):
                    ev = wo_s[n, pl.ds(d2, H // 2, stride=DH), :]
                    od = wo_s[n, pl.ds(DH // 2 + d2, H // 2, stride=DH), :]
                    lo = (ev & jnp.uint32(0xFFFF)) | (od << 16)
                    hi = (ev >> 16) | (od & jnp.uint32(0xFFFF0000))
                    for d, val in ((2 * d2, lo), (2 * d2 + 1, hi)):
                        aa, j = divmod(d, NT)
                        wp_s[pl.ds(64 * j + 16 * aa, H // 2), pl.ds(3 * D + 128 * n, 128)] = val

            def a_task(b, lo, hi, due):
                r0, n = b * T + lo, hi - lo
                x = x_s[pl.ds(r0, n), :].astype(F32)
                m = jnp.sum(x, axis=-1, keepdims=True) * (1.0 / D)
                c = x - m
                v = jnp.sum(c * c, axis=-1, keepdims=True) * (1.0 / D)
                xn_s[pl.ds(r0 // 2, n // 2), :] = pack(c * rsqrt(v + EPS))
                token(due, lambda: _or_all(xn_s[pl.ds(r0 // 2, n // 2), :]))

            def finish(g, b, n, lo, hi, acc, due):
                r0 = b * T + lo
                if g == 0:
                    acc = acc * QSCALE
                elif g == 3:
                    acc = acc + x_s[pl.ds(r0, hi - lo), pl.ds(128 * n, 128)].astype(F32)
                token(due, lambda: _or_all(pltpu.bitcast(acc, U32)))
                if g in (0, 3):
                    for r in range(0, hi - lo, 8):
                        (q if g == 0 else hh)[r0 + r, n] = acc[r:r + 8]
                else:
                    (k_s if g == 1 else v_s)[n, pl.ds(HALO + r0, hi - lo), :] = acc

            def m_seg(g, b, n, lo, hi, span):
                src = o_s if g == 3 else xn_s
                acc = mm(src[pl.ds((b * T + lo) // 2, (hi - lo) // 2), :],
                         wp_s[:, pl.ds(D * g + 128 * n, 128)], span)
                finish(g, b, n, lo, hi, acc, span[1] + o["fa"] if hi - lo == T else None)

            def q_seg(b, n, kpart, span):
                k0, k1 = ((0, KA), (KA, D))[kpart]
                acc = mm(xn_s[pl.ds(b * T // 2, T // 2), pl.ds(k0, k1 - k0)],
                         wp_s[pl.ds(k0 // 2, (k1 - k0) // 2), pl.ds(128 * n, 128)], span)
                if kpart == 0:
                    part[b, n] = acc
                else:
                    finish(0, b, n, 0, T, acc + part.pop((b, n)), None)

            def l_task(r0, n, w, due):
                qc = [jnp.concatenate([q[r0 + r, j] for r in range(0, n, 8)], axis=0) for j in range(NT)]
                off = HALO + r0 - DIL * w
                p = qc[0] * k_s[0, pl.ds(off, n), :]
                for j in range(1, NT):
                    p = p + qc[j] * k_s[j, pl.ds(off, n), :]
                p = p + pltpu.roll(p, 64, 1)
                p = p + pltpu.roll(p, 32, 1)
                if r0 - DIL * w < 0:
                    pos = lax.broadcasted_iota(jnp.int32, (n, 128), 0) + (r0 - DIL * w)
                    p = jnp.where(pos >= 0, p, -1e9)
                lgs[r0, w] = p

            def s_task(r0, n, due):
                lg = [lgs.pop((r0, w)) for w in range(W)]
                m = _tree(jnp.maximum, lg)
                e = [jnp.exp2(l - m) for l in lg]
                inv = pl.reciprocal(_tree(jnp.add, e), approx=True)
                for r in range(0, n, 8):
                    sm[r0 + r] = [t[r:r + 8] for t in e + [inv]]
                token(due, lambda: _or_all(pltpu.bitcast(inv, U32)))

            def p_task(b, c, j, due):
                r0 = b * T + c * R
                ei = [jnp.concatenate([sm[r0 + h][w] for h in range(0, R, 8)], axis=0) for w in range(W + 1)]
                acc = None
                for w in range(W):
                    t = ei[w] * v_s[j, pl.ds(HALO + r0 - DIL * w, R), :]
                    acc = t if acc is None else acc + t
                dst = (pl.ds(r0 // 2, R // 2), pl.ds(128 * j, 128))
                o_s[dst] = pack(acc * ei[W])
                token(due, lambda: o_s[dst])

            def e_task(b, lo, hi, due):
                r0, n = b * T + lo, hi - lo
                if st["wr"] is None:
                    st["wr"] = wr_s[...].astype(F32).reshape(1, D)
                h = jnp.concatenate([jnp.concatenate([hh.pop((r0 + r, j)) for r in range(0, n, 8)], axis=0)
                                     for j in range(NT)], axis=1)
                m = jnp.sum(h, axis=-1, keepdims=True) * (1.0 / D)
                c = h - m
                v = jnp.sum(c * c, axis=-1, keepdims=True) * (1.0 / D)
                cw = jnp.sum(c * st["wr"], axis=-1, keepdims=True)
                rstd = rsqrt(v + EPS)
                hn = c * rstd
                out_s[pl.ds(pl.multiple_of(step * 16 + r0, 16), n), :] = (h + hn).astype(BF16)
                hn_s[pl.ds(r0 // 2, n // 2), :] = pack(hn)
                r = jnp.broadcast_to(cw * rstd, (n, 128))
                best = st["best"]
                for i in range(n // 8):
                    ri = r[8 * i:8 * i + 8]
                    rows = lax.broadcasted_iota(jnp.int32, (8, 128), 0) + (r0 + 8 * i)
                    if best is None:
                        best = (jnp.where(ri > -jnp.inf, ri, -jnp.inf), rows)
                    else:
                        upd = ri > best[0]
                        best = (jnp.where(upd, ri, best[0]), jnp.where(upd, rows, best[1]))
                st["best"] = best
                if b == NS - 1:
                    ocp(r0, r0 + n).start()
                elif hi == T:
                    ocp(b * T, (b + 1) * T).start()
                token(due, lambda: (pltpu.bitcast(best[0], U32) | pltpu.bitcast(best[1], U32)
                                    | hn_s[pl.ds(pl.multiple_of(step * 8, 8), 8), 0:128]
                                    | pltpu.bitcast(out_s[0:16, 0:128], U32)))

            def spec_task(due):
                st["xs"] = load_chunk(argmax(st["best"])[1], LATE)

            def g_seg(k, n, span):
                gu[k, n] = jnp.dot(st["xs"], (wg_s, wu_s)[k][:, pl.ds(128 * n, 128)],
                                   preferred_element_type=F32)

            def h_seg(n, span):
                if "act" not in st:
                    g = jnp.concatenate([gu[0, i] for i in range(F // 128)], axis=1)
                    u = jnp.concatenate([gu[1, i] for i in range(F // 128)], axis=1)
                    act_s[...] = pack(g * jax.nn.sigmoid(g) * u)
                    st["act"] = True
                y_s[:, pl.ds(128 * n, 128)] = mm(act_s[...], wd_s[:, pl.ds(128 * n, 128)], span)

            def do_wait(nm):
                st["toks"] = []
                for c in cp[nm]:
                    wait(c, nm)

            fns = dict(A=a_task, M=m_seg, Q=q_seg, L=l_task, S=s_task, P=p_task, E=e_task, wait=do_wait,
                       perm=permute_w, permo=permute_wo, spec=spec_task, G=g_seg, H=h_seg)
            for item in prog:
                fns[item[0]](*item[1:])
            return st["best"]

        def argmax(best):
            bv, bi = best
            mx = jnp.max(bv, axis=0, keepdims=True)
            idx = jnp.min(jnp.where(bv >= mx, bi, S - 1), axis=0, keepdims=True)
            return mx[:, 0:1], jnp.clip(idx[0, 0], 0, S - 1)

        def load_chunk(idx, nrows):
            blk = jnp.clip(idx >> 4, 0, nrows // 16 - 1)
            return pltpu.bitcast(hn_s[pl.ds(pl.multiple_of(blk * 8, 8), 8), :], BF16)

        def fix_row(mx, idx, nrows):
            base = pl.multiple_of(jnp.clip(idx >> 4, 0, nrows // 16 - 1) * 16, 16)
            y = y_s[...] * jax.nn.sigmoid(mx)
            cur = out_s[pl.ds(base, 16), :].astype(F32)
            rows = lax.broadcasted_iota(jnp.int32, (16, D), 0) + base
            out_s[pl.ds(base, 16), :] = jnp.where(rows == idx, cur + y, cur).astype(BF16)
            fix = pltpu.make_async_copy(out_s.at[pl.ds(base, 16)], out_hbm.at[pl.ds(base, 16)], sem_out.at[2])
            fix.start()
            return fix

        def tail(best):
            mx, idx = argmax(best)
            wait(ocp(0, LATE), "out0")

            def early():
                fix = fix_row(mx, idx, LATE)
                wait(ocp(LATE, S), "out1")
                wait(fix, "fix")

            def late():
                xs = load_chunk(idx, S)
                g = jnp.dot(xs, wg_s[...], preferred_element_type=F32)
                u = jnp.dot(xs, wu_s[...], preferred_element_type=F32)
                act = (g * jax.nn.sigmoid(g) * u).astype(BF16)
                y_s[...] = jnp.dot(act, wd_s[...], preferred_element_type=F32)
                wait(ocp(LATE, S), "out1")
                wait(fix_row(mx, idx, S), "fix")

            lax.cond(idx < LATE, early, late)

        pl.when(pid == 0)(start_all)

        @pl.when(pid == 1)
        def _():
            tail(main())

    @jax.jit
    def fn(A_x, A_wqkv, A_wo, B_x, B_w_r, B_w_gate, B_w_up, B_w_down):
        any_spec = pl.BlockSpec(memory_space=pl.ANY)
        out = pl.pallas_call(
            kernel,
            grid=(2,),
            out_shape=jax.ShapeDtypeStruct((S, D), BF16),
            in_specs=[any_spec] * 7,
            out_specs=any_spec,
            scratch_shapes=[
                pltpu.VMEM((S, D), BF16),
                pltpu.VMEM((D, 3 * D), BF16),
                pltpu.VMEM((NT, D // 2 + 32, 128), U32),
                pltpu.VMEM((D, D), BF16),
                pltpu.VMEM((D,), BF16),
                pltpu.VMEM((D, F), BF16),
                pltpu.VMEM((D, F), BF16),
                pltpu.VMEM((F, D), BF16),
                pltpu.VMEM((D // 2, 4 * D), U32),
                pltpu.VMEM((NT, S + HALO, 128), F32),
                pltpu.VMEM((NT, S + HALO, 128), F32),
                pltpu.VMEM((S // 2, D), U32),
                pltpu.VMEM((S // 2, D), U32),
                pltpu.VMEM((S // 2, D), U32),
                pltpu.VMEM((S + 16, D), BF16),
                pltpu.VMEM((16, D), F32),
                pltpu.VMEM((8, F), U32),
                pltpu.SemaphoreType.DMA((7,)),
                pltpu.SemaphoreType.DMA((3,)),
            ],
            compiler_params=pltpu.CompilerParams(vmem_limit_bytes=100 << 20,
                                                 dimension_semantics=("arbitrary",),
                                                 disable_bounds_checks=True,
                                                 disable_semaphore_checks=True),
            name="fused",
        )(A_x.reshape(S, D), A_wqkv, A_wo, B_w_r, B_w_gate, B_w_up, B_w_down)
        return out.reshape(1, S, D)

    return fn


pallas_sequential_preLN__sliding_local_dilated__moe_arch_mod__prompt_kernel = make_kernel()
```

```python
import functools
import math
import jax
import jax.numpy as jnp
from jax import lax
import jax.experimental.pallas as pl
import jax.experimental.pallas.tpu as pltpu

S, D, F = 2048, 640, 1536
H, DH, W, DIL = 32, 20, 8, 2
NT = D // 128
HALO = 16
EPS = 1e-5
F32, BF16, U32 = jnp.float32, jnp.bfloat16, jnp.uint32
QSCALE = DH ** -0.5 * math.log2(math.e)
R = 16
T = 128
NS = S // T
NC = T // R
KA = 384
LATE = (NS - 2) * T
XB = 7


def _or_all(u):
    t = None
    for i in range(u.shape[0] // 8):
        for j in range(u.shape[1] // 128):
            p = u[8 * i:8 * i + 8, 128 * j:128 * (j + 1)]
            t = p if t is None else t | p
    return t


def _tree(f, xs):
    xs = list(xs)
    while len(xs) > 1:
        xs = [f(xs[i], xs[i + 1]) for i in range(0, len(xs) - 1, 2)] + ([xs[-1]] if len(xs) % 2 else [])
    return xs[0]


def _opts(s):
    if not isinstance(s, str):
        return dict(s)
    out = {}
    for kv in s.split(","):
        k, v = kv.split(":")
        v = [float(x) if "." in x else int(x) for x in v.split("/") if x]
        out[k] = v[0] if len(v) == 1 and not kv.endswith("/") else tuple(v)
    return out


def _rows(lo, hi):
    return range(lo, hi, R)


def _io(it):
    k = it[0]
    lhs = lambda g, b, lo=0, hi=T: [("o" if g == 3 else "xn", b, r, j) for r in _rows(lo, hi) for j in range(NT)]
    out = lambda g, b, n, lo=0, hi=T: [("y", g, b, n, r) for r in _rows(lo, hi)]
    if k == "A":
        return [], lhs(0, *it[1:4])
    if k == "M":
        _, g, b, n, lo, hi = it
        return lhs(g, b, lo, hi) + [("w", g, n, 0), ("w", g, n, 1)], out(g, b, n, lo, hi)
    if k == "Q":
        _, b, n, part = it
        return lhs(0, b) + [("w", 0, n, part)], (out(0, b, n) if part else [])
    if k == "perm":
        _, g, k0, k1, js = it
        return [], [("w", g, j, p) for j in js for p in (0, 1) if (k0, k1)[p] == (0, D)[p]]
    if k == "permo":
        return [], [("w", 3, it[1], 0), ("w", 3, it[1], 1)]
    if k == "L":
        _, r0, n, w = it
        b, r = divmod(r0, T)
        return [("y", g, b, j, r // R * R) for g in (0, 1) for j in range(NT)], [("lg", r0, w)]
    if k == "S":
        _, r0, n = it
        return [("lg", r0, w) for w in range(W)], [("sm", r0 + r) for r in range(0, n, 8)]
    if k == "P":
        _, b, c, j = it
        return ([("sm", b * T + c * R + r) for r in range(0, R, 8)] + [("y", 2, b, j, c * R)],
                [("o", b, c * R, j)])
    if k == "E":
        _, b, lo, hi = it
        prev = [("e", b * T + lo - R)] if b * T + lo else []
        return ([("y", 3, b, n, r) for n in range(NT) for r in _rows(lo, hi)] + prev,
                [("e", b * T + r) for r in _rows(lo, hi)])
    if k == "spec":
        return [("e", LATE - R)], [("spec",)]
    if k == "G":
        return [("spec",)], [("g",) + it[1:]]
    if k == "H":
        return [("g", kk, n) for kk in range(2) for n in range(F // 128)], []
    return [], []


def _slots(it):
    k = it[0]
    if k == "M":
        return (it[5] - it[4]) / 16
    if k == "Q":
        return 1.6 * (3, 2)[it[3]]
    return {"G": 0.0, "H": 1.0}[k]


class Plan:
    def __init__(self):
        self.prog, self.pos, self.have, self.todo = [], 0.0, set(), []

    def _put(self, it, extra):
        self.prog.append(it + (extra,))
        self.have.update(_io(it)[1])

    def _emit_task(self, t, force=False):
        due, it = t
        for key in _io(it)[0]:
            if key not in self.have:
                src = [u for u in self.todo if key in _io(u[1])[1]]
                if not src or not self._emit_task(src[0], force):
                    assert not force, ("unsatisfied", it, key)
                    return False
        self.todo.remove(t)
        self._put(it, due)
        return True

    def tasks(self, ts):
        self.todo += [(None if d is None else self.pos + d, it) for d, it in ts]

    def mxu(self, segs):
        for sg in segs:
            end = self.pos + _slots(sg)
            for t in sorted([t for t in self.todo if t[0] is not None and t[0] < end], key=lambda t: t[0]):
                if t in self.todo:
                    self._emit_task(t)
            for key in _io(sg)[0]:
                if key not in self.have:
                    src = [u for u in self.todo if key in _io(u[1])[1]]
                    assert src, ("unsatisfied", sg, key)
                    self._emit_task(src[0], True)
            self._put(sg, (self.pos, end))
            self.pos = end

    def flush(self, pred=lambda it: True):
        for t in [t for t in self.todo if pred(t[1])]:
            if t in self.todo:
                self._emit_task(t, True)

    def wait(self, *names):
        self.prog += [("wait", n) for n in names]


def build_program(o):
    M = lambda g, b, lo=0, hi=T: [("M", g, b, n, lo, hi) for n in range(NT)]
    Q = lambda b, part: [("Q", b, n, part) for n in range(NT)]

    def parts(kind, b, dls):
        n = T // len(dls)
        return [(dl, (kind, b, i * n, (i + 1) * n)) for i, dl in enumerate(dls)]

    def LS(b, c0, cp, rl=R):
        t = []
        for c in range(NC):
            for h in range(0, R, rl):
                r0 = b * T + c * R + h
                t += [(None, ("L", r0, rl, w)) for w in range(W)]
                t += [(None if c0 is None else c0 + cp * c - (R - rl - h) * cp / R, ("S", r0, rl))]
        return t

    def Pt(b, c0, cp):
        return [(None if c0 is None else c0 + cp * c + o["ps"] * j, ("P", b, c, j))
                for c in range(NC) for j in range(NT)]

    def C(b, c0, cp):
        return LS(b, c0, cp, o["rl"]) + Pt(b, c0 + o["po"], cp)

    allj = tuple(range(NT))
    p = Plan()
    p.wait("x0a")
    p.tasks(parts("A", 0, (None,)) + parts("A", 1, (None,)))
    p.flush()
    p.wait("wqa")
    p.tasks([(None, ("perm", 0, 0, KA, allj))])
    p.mxu(Q(0, 0))
    p.wait("x0b", "wqb")
    p.tasks([(None, ("perm", 0, KA, D, allj))] + parts("A", 2, (None,)))
    p.flush()
    p.mxu(Q(1, 0) + Q(0, 1) + Q(1, 1) + Q(2, 0))
    p.wait("wk")
    p.tasks([(None, ("perm", 1, 0, D, allj))] + LS(0, None, 0))
    p.mxu(Q(2, 1) + M(1, 0) + M(1, 1))
    p.flush()
    p.wait("wv")
    p.tasks([(o["pv"][0] + o["pv"][1] * j, ("perm", 2, 0, D, (j,))) for j in range(NT)]
            + LS(1, *o["l1"]) + Pt(0, *o["p0"]))
    p.mxu(M(1, 2) + M(2, 0) + M(2, 1))
    p.flush()
    p.wait("wo", "wr", "x1")
    p.tasks([(None, ("permo", n)) for n in range(NT)])
    p.tasks(Pt(1, *o["p1"]) + parts("A", 3, o["a3"]) + parts("E", 0, o["e0"])
            + parts("E", 1, o["e1"]) + C(2, *o["c2"]) + parts("A", 4, o["a4"]))
    p.mxu(M(2, 2) + M(3, 0) + M(3, 1) + M(0, 3) + M(1, 3) + M(2, 3))
    for s in range(3, NS - 2):
        tasks = parts("E", s - 1, o["e"]) + C(s, *o["c"]) + parts("A", s + 2, o["a"])
        if s == XB:
            pre = [t for t in tasks if t[1][0] in "LS" and t[1][1] < s * T + o["pre"] * R]
            p.tasks([(None, t[1]) for t in pre])
            tasks = [t for t in tasks if t not in pre]
            p.flush()
            p.wait("x2", "ffn")
        p.tasks(tasks)
        p.mxu(sum([M(g, s - 1 if g == 3 else s + 1) for g in o["mo"]], []))
    s = NS - 2
    big = M(3, s - 1) + M(0, s + 1) + M(1, s + 1) + M(3, s) + M(2, s + 1)
    small = [("G", k, n) for n in range(F // 128) for k in range(2)]
    cut = o["cut"]
    segs = []
    n_big, n_small, done = len(big) - o["sp"], len(small) - o["gh"], 0
    for g, sg in enumerate(big):
        segs.append(sg)
        if g >= o["sp"]:
            want = min(n_small, -(-(g - o["sp"] + 1) * n_small // n_big))
            segs += small[done:want]
            done = want
    segs += small[done:] + M(3, s + 1, 0, cut) + M(3, s + 1, cut, T) + [("H", n) for n in range(NT)]
    p.tasks(parts("E", s - 1, o["e13"]) + [(None, ("spec",))] + C(s, *o["c14"])
            + LS(s + 1, *o["l15"]) + Pt(s + 1, None, 0) + parts("E", s, o["e14"])
            + [(o["e15"], ("E", s + 1, 0, cut)), (None, ("E", s + 1, cut, T))])
    p.mxu(segs)
    p.flush()
    return p.prog


DEFAULTS = dict(
    mode="", rl=8, ps=3, po=2, fa=(16, 16, 16, 16), pre=2, mo=(3, 0, 1, 2),
    pv=(13, 6), l1=(52, 8), p0=(92, 3.5),
    p1=(36, 17), a3=(100,), e0=(132, 152), e1=(176, 200), c2=(92, 17.5), a4=(160, 223),
    e=(96, 144), c=(24, 17.5), a=(64, 136),
    cut=64, sp=12, gh=6, e13=(72, 88), c14=(22, 12.25), l15=(138, 4.5), e14=(184, 187), e15=241)


def make_kernel(prof=0, O=(), **kw):
    o = dict(DEFAULTS)
    o.update(_opts(O))
    o.update(kw)
    prog = build_program(o)
    x1 = (XB - 1) * T
    xch = (2 * T, T, x1, S - 3 * T - x1)

    def wait(c, name):
        if prof:
            with jax.named_scope("w_" + name):
                c.wait()
        else:
            c.wait()

    def kernel(x_hbm, wqkv_hbm, wo_hbm, wr_hbm, wg_hbm, wu_hbm, wd_hbm, out_hbm,
               x_s, wqkv_s, wo_s, wob_s, wr_s, wg_s, wu_s, wd_s, wp_s,
               k_s, v_s, xn_s, o_s, hn_s, out_s, y_s, act_s, sem_in, sem_out):
        pid = pl.program_id(0)
        step = pid - 1
        cp = {}
        semi = dict(x0a=0, wqa=1, x0b=6, wqb=6, wk=2, wv=3, wo=4, wr=4, x1=4, x2=5, ffn=5)
        r0 = 0
        for nm, n in zip(("x0a", "x0b", "x1", "x2"), xch):
            cp[nm] = [pltpu.make_async_copy(x_hbm.at[pl.ds(r0, n)], x_s.at[pl.ds(r0, n)], sem_in.at[semi[nm]])]
            r0 += n
        for nm, lo, hi, g in (("wqa", 0, KA, 0), ("wqb", KA, D, 0), ("wk", 0, D, 1), ("wv", 0, D, 2)):
            sl = (pl.ds(lo, hi - lo), pl.ds(D * g, D))
            cp[nm] = [pltpu.make_async_copy(wqkv_hbm.at[sl], wqkv_s.at[sl], sem_in.at[semi[nm]])]
        cp["wo"] = [pltpu.make_async_copy(wo_hbm, wob_s, sem_in.at[semi["wo"]])]
        cp["wr"] = [pltpu.make_async_copy(wr_hbm, wr_s, sem_in.at[semi["wr"]])]
        cp["ffn"] = [pltpu.make_async_copy(a, b, sem_in.at[semi["ffn"]])
                     for a, b in ((wg_hbm, wg_s), (wu_hbm, wu_s), (wd_hbm, wd_s))]

        def ocp(lo, hi):
            return pltpu.make_async_copy(out_s.at[pl.ds(lo, hi - lo)], out_hbm.at[pl.ds(lo, hi - lo)],
                                         sem_out.at[0 if lo < LATE else 1])

        def start_all():
            for nm in ("x0a", "wqa", "x0b", "wqb", "wk", "wv", "wo", "wr", "x1", "x2", "ffn"):
                for c in cp[nm]:
                    c.start()

        def main():
            zero = jnp.zeros((HALO, 128), F32)
            for j in range(NT):
                k_s[j, 0:HALO, :] = zero
                v_s[j, 0:HALO, :] = zero

            lane = lax.broadcasted_iota(jnp.int32, (1, 128), 1)
            cm5 = [(lane + 128 * t) - 5 * (((lane + 128 * t) * 52429) >> 18) for t in range(NT - 1)]
            srcs = [(20 * (lane & 31) + 5 * (lane >> 5) + j) & 127 for j in range(NT)]
            never = jnp.full((8, 128), step, jnp.int32) > 0
            st = dict(best=None, toks=[], wr=None)
            q, hh, lgs, sm, gu, part = {}, {}, {}, {}, {}, {}
            pack = lambda v: pltpu.bitcast(v.astype(BF16), U32)
            rsqrt = lambda v: jnp.exp2(jnp.log(v) * (-0.5 / math.log(2.0)))

            def token(due, u):
                if due is not None:
                    st["toks"].append((due, u()))

            def mm(lhs, w, span):
                start, end = span
                toks = [t for t in st["toks"] if t[0] < end]
                st["toks"] = [t for t in st["toks"] if t[0] >= end]
                if toks:
                    ng = lhs.shape[0] // 8
                    rows = []
                    for i in range(ng):
                        mine = [t for d, t in toks if min(max(int(d - start), 0), ng - 1) == i]
                        blk = lhs[8 * i:8 * i + 8]
                        if mine:
                            head = jnp.where(never, functools.reduce(lambda x, y: x | y, mine), blk[:, 0:128])
                            blk = jnp.concatenate([head, blk[:, 128:]], axis=1)
                        rows.append(blk)
                    lhs = jnp.concatenate(rows, axis=0)
                if w.dtype == U32:
                    w = pltpu.bitcast(w, BF16)
                return jnp.dot(pltpu.bitcast(lhs, BF16), w, preferred_element_type=F32)

            def permute_w(g, k0, k1, js, due):
                if ("mw", g, k0) not in st:
                    tiles = [pltpu.bitcast(wqkv_s[pl.ds(k0, k1 - k0), pl.ds(D * g + 128 * t, 128)], U32)
                             for t in range(NT)]
                    st["mw", g, k0] = []
                    for j in range(NT):
                        m = tiles[NT - 1]
                        for t in range(NT - 2, -1, -1):
                            m = jnp.where(cm5[t] == j, tiles[t], m)
                        st["mw", g, k0].append(m)
                for j in js:
                    m = st["mw", g, k0][j]
                    res = jnp.take_along_axis(m, jnp.broadcast_to(srcs[j], m.shape), axis=1,
                                              mode="promise_in_bounds")
                    wp_s[pl.ds(k0 // 2, (k1 - k0) // 2), pl.ds(D * g + 128 * j, 128)] = res
                    token(due, lambda: _or_all(res))

            def permute_wo(n, due):
                wo_s[n, pl.ds(0, D // 2), :] = pltpu.bitcast(wob_s[:, pl.ds(128 * n, 128)], U32)
                for d2 in range(DH // 2):
                    ev = wo_s[n, pl.ds(d2, H // 2, stride=DH), :]
                    od = wo_s[n, pl.ds(DH // 2 + d2, H // 2, stride=DH), :]
                    lo = (ev & jnp.uint32(0xFFFF)) | (od << 16)
                    hi = (ev >> 16) | (od & jnp.uint32(0xFFFF0000))
                    for d, val in ((2 * d2, lo), (2 * d2 + 1, hi)):
                        aa, j = divmod(d, NT)
                        wp_s[pl.ds(64 * j + 16 * aa, H // 2), pl.ds(3 * D + 128 * n, 128)] = val

            def a_task(b, lo, hi, due):
                r0, n = b * T + lo, hi - lo
                x = x_s[pl.ds(r0, n), :].astype(F32)
                m = jnp.sum(x, axis=-1, keepdims=True) * (1.0 / D)
                c = x - m
                v = jnp.sum(c * c, axis=-1, keepdims=True) * (1.0 / D)
                xn_s[pl.ds(r0 // 2, n // 2), :] = pack(c * rsqrt(v + EPS))
                token(due, lambda: _or_all(xn_s[pl.ds(r0 // 2, n // 2), :]))

            def finish(g, b, n, lo, hi, acc, due):
                r0 = b * T + lo
                if g == 0:
                    acc = acc * QSCALE
                elif g == 3:
                    acc = acc + x_s[pl.ds(r0, hi - lo), pl.ds(128 * n, 128)].astype(F32)
                token(due, lambda: _or_all(pltpu.bitcast(acc, U32)))
                if g in (0, 3):
                    for r in range(0, hi - lo, 8):
                        (q if g == 0 else hh)[r0 + r, n] = acc[r:r + 8]
                else:
                    (k_s if g == 1 else v_s)[n, pl.ds(HALO + r0, hi - lo), :] = acc

            def m_seg(g, b, n, lo, hi, span):
                src = o_s if g == 3 else xn_s
                acc = mm(src[pl.ds((b * T + lo) // 2, (hi - lo) // 2), :],
                         wp_s[:, pl.ds(D * g + 128 * n, 128)], span)
                fa = o["fa"][g]
                finish(g, b, n, lo, hi, acc, span[1] + fa if hi - lo == T and fa < 99 else None)

            def q_seg(b, n, kpart, span):
                k0, k1 = ((0, KA), (KA, D))[kpart]
                acc = mm(xn_s[pl.ds(b * T // 2, T // 2), pl.ds(k0, k1 - k0)],
                         wp_s[pl.ds(k0 // 2, (k1 - k0) // 2), pl.ds(128 * n, 128)], span)
                if kpart == 0:
                    part[b, n] = acc
                else:
                    finish(0, b, n, 0, T, acc + part.pop((b, n)), None)

            def l_task(r0, n, w, due):
                qc = [jnp.concatenate([q[r0 + r, j] for r in range(0, n, 8)], axis=0) for j in range(NT)]
                off = HALO + r0 - DIL * w
                p = qc[0] * k_s[0, pl.ds(off, n), :]
                for j in range(1, NT):
                    p = p + qc[j] * k_s[j, pl.ds(off, n), :]
                p = p + pltpu.roll(p, 64, 1)
                p = p + pltpu.roll(p, 32, 1)
                if r0 - DIL * w < 0:
                    pos = lax.broadcasted_iota(jnp.int32, (n, 128), 0) + (r0 - DIL * w)
                    p = jnp.where(pos >= 0, p, -1e9)
                lgs[r0, w] = p

            def s_task(r0, n, due):
                lg = [lgs.pop((r0, w)) for w in range(W)]
                m = _tree(jnp.maximum, lg)
                e = [jnp.exp2(l - m) for l in lg]
                inv = pl.reciprocal(_tree(jnp.add, e), approx=True)
                for r in range(0, n, 8):
                    sm[r0 + r] = [t[r:r + 8] for t in e + [inv]]
                token(due, lambda: _or_all(pltpu.bitcast(inv, U32)))

            def p_task(b, c, j, due):
                r0 = b * T + c * R
                ei = [jnp.concatenate([sm[r0 + h][w] for h in range(0, R, 8)], axis=0) for w in range(W + 1)]
                acc = None
                for w in range(W):
                    t = ei[w] * v_s[j, pl.ds(HALO + r0 - DIL * w, R), :]
                    acc = t if acc is None else acc + t
                dst = (pl.ds(r0 // 2, R // 2), pl.ds(128 * j, 128))
                o_s[dst] = pack(acc * ei[W])
                token(due, lambda: o_s[dst])

            def e_task(b, lo, hi, due):
                r0, n = b * T + lo, hi - lo
                if st["wr"] is None:
                    st["wr"] = wr_s[...].astype(F32).reshape(1, D)
                h = jnp.concatenate([jnp.concatenate([hh.pop((r0 + r, j)) for r in range(0, n, 8)], axis=0)
                                     for j in range(NT)], axis=1)
                m = jnp.sum(h, axis=-1, keepdims=True) * (1.0 / D)
                c = h - m
                v = jnp.sum(c * c, axis=-1, keepdims=True) * (1.0 / D)
                cw = jnp.sum(c * st["wr"], axis=-1, keepdims=True)
                rstd = rsqrt(v + EPS)
                hn = c * rstd
                out_s[pl.ds(pl.multiple_of(step * 16 + r0, 16), n), :] = (h + hn).astype(BF16)
                hn_s[pl.ds(r0 // 2, n // 2), :] = pack(hn)
                r = jnp.broadcast_to(cw * rstd, (n, 128))
                best = st["best"]
                for i in range(n // 8):
                    ri = r[8 * i:8 * i + 8]
                    rows = lax.broadcasted_iota(jnp.int32, (8, 128), 0) + (r0 + 8 * i)
                    if best is None:
                        best = (jnp.where(ri > -jnp.inf, ri, -jnp.inf), rows)
                    else:
                        upd = ri > best[0]
                        best = (jnp.where(upd, ri, best[0]), jnp.where(upd, rows, best[1]))
                st["best"] = best
                if b == NS - 1:
                    ocp(r0, r0 + n).start()
                elif hi == T:
                    ocp(b * T, (b + 1) * T).start()
                token(due, lambda: (pltpu.bitcast(best[0], U32) | pltpu.bitcast(best[1], U32)
                                    | hn_s[pl.ds(pl.multiple_of(step * 8, 8), 8), 0:128]
                                    | pltpu.bitcast(out_s[0:16, 0:128], U32)))

            def spec_task(due):
                st["xs"] = load_chunk(argmax(st["best"])[1], LATE)

            def g_seg(k, n, span):
                gu[k, n] = jnp.dot(st["xs"], (wg_s, wu_s)[k][:, pl.ds(128 * n, 128)],
                                   preferred_element_type=F32)

            def h_seg(n, span):
                if "act" not in st:
                    g = jnp.concatenate([gu[0, i] for i in range(F // 128)], axis=1)
                    u = jnp.concatenate([gu[1, i] for i in range(F // 128)], axis=1)
                    act_s[...] = pack(g * jax.nn.sigmoid(g) * u)
                    st["act"] = True
                y_s[:, pl.ds(128 * n, 128)] = mm(act_s[...], wd_s[:, pl.ds(128 * n, 128)], span)

            def do_wait(nm):
                st["toks"] = []
                for c in cp[nm]:
                    wait(c, nm)

            fns = dict(A=a_task, M=m_seg, Q=q_seg, L=l_task, S=s_task, P=p_task, E=e_task, wait=do_wait,
                       perm=permute_w, permo=permute_wo, spec=spec_task, G=g_seg, H=h_seg)
            for item in prog:
                fns[item[0]](*item[1:])
            return st["best"]

        def argmax(best):
            bv, bi = best
            mx = jnp.max(bv, axis=0, keepdims=True)
            idx = jnp.min(jnp.where(bv >= mx, bi, S - 1), axis=0, keepdims=True)
            return mx[:, 0:1], jnp.clip(idx[0, 0], 0, S - 1)

        def load_chunk(idx, nrows):
            blk = jnp.clip(idx >> 4, 0, nrows // 16 - 1)
            return pltpu.bitcast(hn_s[pl.ds(pl.multiple_of(blk * 8, 8), 8), :], BF16)

        def fix_row(mx, idx, nrows):
            base = pl.multiple_of(jnp.clip(idx >> 4, 0, nrows // 16 - 1) * 16, 16)
            y = y_s[...] * jax.nn.sigmoid(mx)
            cur = out_s[pl.ds(base, 16), :].astype(F32)
            rows = lax.broadcasted_iota(jnp.int32, (16, D), 0) + base
            out_s[pl.ds(base, 16), :] = jnp.where(rows == idx, cur + y, cur).astype(BF16)
            fix = pltpu.make_async_copy(out_s.at[pl.ds(base, 16)], out_hbm.at[pl.ds(base, 16)], sem_out.at[2])
            fix.start()
            return fix

        def tail(best):
            mx, idx = argmax(best)
            wait(ocp(0, LATE), "out0")

            def early():
                fix = fix_row(mx, idx, LATE)
                wait(ocp(LATE, S), "out1")
                wait(fix, "fix")

            def late():
                xs = load_chunk(idx, S)
                g = jnp.dot(xs, wg_s[...], preferred_element_type=F32)
                u = jnp.dot(xs, wu_s[...], preferred_element_type=F32)
                act = (g * jax.nn.sigmoid(g) * u).astype(BF16)
                y_s[...] = jnp.dot(act, wd_s[...], preferred_element_type=F32)
                wait(ocp(LATE, S), "out1")
                wait(fix_row(mx, idx, S), "fix")

            lax.cond(idx < LATE, early, late)

        pl.when(pid == 0)(start_all)

        @pl.when(pid == 1)
        def _():
            tail(main())

    @jax.jit
    def fn(A_x, A_wqkv, A_wo, B_x, B_w_r, B_w_gate, B_w_up, B_w_down):
        any_spec = pl.BlockSpec(memory_space=pl.ANY)
        out = pl.pallas_call(
            kernel,
            grid=(2,),
            out_shape=jax.ShapeDtypeStruct((S, D), BF16),
            in_specs=[any_spec] * 7,
            out_specs=any_spec,
            scratch_shapes=[
                pltpu.VMEM((S, D), BF16),
                pltpu.VMEM((D, 3 * D), BF16),
                pltpu.VMEM((NT, D // 2 + 32, 128), U32),
                pltpu.VMEM((D, D), BF16),
                pltpu.VMEM((D,), BF16),
                pltpu.VMEM((D, F), BF16),
                pltpu.VMEM((D, F), BF16),
                pltpu.VMEM((F, D), BF16),
                pltpu.VMEM((D // 2, 4 * D), U32),
                pltpu.VMEM((NT, S + HALO, 128), F32),
                pltpu.VMEM((NT, S + HALO, 128), F32),
                pltpu.VMEM((S // 2, D), U32),
                pltpu.VMEM((S // 2, D), U32),
                pltpu.VMEM((S // 2, D), U32),
                pltpu.VMEM((S + 16, D), BF16),
                pltpu.VMEM((16, D), F32),
                pltpu.VMEM((8, F), U32),
                pltpu.SemaphoreType.DMA((7,)),
                pltpu.SemaphoreType.DMA((3,)),
            ],
            compiler_params=pltpu.CompilerParams(vmem_limit_bytes=100 << 20,
                                                 dimension_semantics=("arbitrary",),
                                                 disable_bounds_checks=True,
                                                 disable_semaphore_checks=True),
            name="fused",
        )(A_x.reshape(S, D), A_wqkv, A_wo, B_w_r, B_w_gate, B_w_up, B_w_down)
        return out.reshape(1, S, D)

    return fn


pallas_sequential_preLN__sliding_local_dilated__moe_arch_mod__prompt_kernel = make_kernel()
```

```python
import functools
import math
import jax
import jax.numpy as jnp
from jax import lax
import jax.experimental.pallas as pl
import jax.experimental.pallas.tpu as pltpu

S, D, F = 2048, 640, 1536
H, DH, W, DIL = 32, 20, 8, 2
NT = D // 128
HALO = 16
EPS = 1e-5
F32, BF16, U32 = jnp.float32, jnp.bfloat16, jnp.uint32
QSCALE = DH ** -0.5 * math.log2(math.e)
R = 16
T = 128
NS = S // T
NC = T // R
KA = 384
LATE = (NS - 2) * T
XB = 7


def _fold(f, x):
    while x.shape[0] > 1:
        x = f(x[:x.shape[0] // 2], x[x.shape[0] // 2:])
    return x


def _or_all(u):
    u = pltpu.bitcast(u, U32)
    t = None
    for i in range(u.shape[0] // 8):
        for j in range(u.shape[1] // 128):
            p = u[8 * i:8 * i + 8, 128 * j:128 * (j + 1)]
            t = p if t is None else t | p
    return t


def _opts(s):
    if not isinstance(s, str):
        return dict(s)
    out = {}
    for kv in s.split(","):
        k, v = kv.split(":")
        v = [float(x) if "." in x else int(x) for x in v.split("/") if x]
        out[k] = v[0] if len(v) == 1 and not kv.endswith("/") else tuple(v)
    return out


def _rows(lo, hi):
    return range(lo, hi, R)


def _io(it):
    k = it[0]
    lhs = lambda g, b, lo=0, hi=T: [("o" if g == 3 else "xn", b, r, j) for r in _rows(lo, hi) for j in range(NT)]
    out = lambda g, b, n, lo=0, hi=T: [("y", g, b, n, r) for r in _rows(lo, hi)]
    if k == "A":
        return [], lhs(0, *it[1:4])
    if k == "M":
        _, g, b, n, lo, hi = it
        return lhs(g, b, lo, hi) + [("w", g, n, 0), ("w", g, n, 1)], out(g, b, n, lo, hi)
    if k == "Q":
        _, b, n, part = it
        return lhs(0, b) + [("w", 0, n, part)], (out(0, b, n) if part else [])
    if k == "perm":
        _, g, k0, k1, js = it
        return [], [("w", g, j, p) for j in js for p in (0, 1) if (k0, k1)[p] == (0, D)[p]]
    if k == "permo":
        return [], [("w", 3, it[1], 0), ("w", 3, it[1], 1)]
    if k == "S":
        _, r0, n = it
        b, r = divmod(r0, T)
        return ([("y", g, b, j, r // R * R) for g in (0, 1) for j in range(NT)],
                [("sm", r0 + i) for i in range(0, n, 8)])
    if k == "P":
        _, b, c, j = it
        return ([("sm", b * T + c * R + r) for r in range(0, R, 8)] + [("y", 2, b, jj, c * R) for jj in range(NT)],
                [("o", b, c * R, j)])
    if k == "E":
        _, b, lo, hi = it
        prev = [("e", b * T + lo - R)] if b * T + lo else []
        return ([("y", 3, b, n, r) for n in range(NT) for r in _rows(lo, hi)] + prev,
                [("e", b * T + r) for r in _rows(lo, hi)])
    if k == "spec":
        return [("e", LATE - R)], [("spec",)]
    if k == "G":
        return [("spec",)], [("g",) + it[1:]]
    if k == "H":
        return [("g", kk, n) for kk in range(2) for n in range(F // 128)], []
    return [], []


def _slots(it):
    k = it[0]
    if k == "M":
        return (it[5] - it[4]) / 16
    if k == "Q":
        return 1.6 * (3, 2)[it[3]]
    return {"G": 0.0, "H": 1.0}[k]


class Plan:
    def __init__(self):
        self.prog, self.pos, self.have, self.todo = [], 0.0, set(), []

    def _put(self, it, extra):
        self.prog.append(it + (extra,))
        self.have.update(_io(it)[1])

    def _emit_task(self, t, force=False):
        due, it = t
        for key in _io(it)[0]:
            if key not in self.have:
                src = [u for u in self.todo if key in _io(u[1])[1]]
                if not src or not self._emit_task(src[0], force):
                    assert not force, ("unsatisfied", it, key)
                    return False
        self.todo.remove(t)
        self._put(it, due)
        return True

    def tasks(self, ts):
        self.todo += [(None if d is None or d > 500 else self.pos + d, it) for d, it in ts]

    def mxu(self, segs):
        for sg in segs:
            end = self.pos + _slots(sg)
            for t in sorted([t for t in self.todo if t[0] is not None and t[0] < end], key=lambda t: t[0]):
                if t in self.todo:
                    self._emit_task(t)
            for key in _io(sg)[0]:
                if key not in self.have:
                    src = [u for u in self.todo if key in _io(u[1])[1]]
                    assert src, ("unsatisfied", sg, key)
                    self._emit_task(src[0], True)
            self._put(sg, (self.pos, end))
            self.pos = end

    def flush(self, pred=lambda it: True):
        for t in [t for t in self.todo if pred(t[1])]:
            if t in self.todo:
                self._emit_task(t, True)

    def wait(self, *names):
        self.prog += [("wait", n) for n in names]


def build_program(o):
    M = lambda g, b, lo=0, hi=T: [("M", g, b, n, lo, hi) for n in range(NT)]
    Q = lambda b, part: [("Q", b, n, part) for n in range(NT)]

    def parts(kind, b, dls):
        n = T // len(dls)
        return [(dl, (kind, b, i * n, (i + 1) * n)) for i, dl in enumerate(dls)]

    def LS(b, c0, cp, rl=R):
        t = []
        for c in range(NC):
            for h in range(0, R, rl):
                r0 = b * T + c * R + h
                t += [(None if c0 is None else c0 + cp * c - (R - rl - h) * cp / R, ("S", r0, rl))]
        return t

    def Pt(b, c0, cp):
        return [(None if c0 is None else c0 + cp * c + o["ps"] * j, ("P", b, c, j))
                for c in range(NC) for j in range(NT)]

    def C(b, c0, cp):
        return LS(b, c0, cp, o["rl"]) + Pt(b, c0 + o["po"], cp)

    allj = tuple(range(NT))
    p = Plan()
    p.wait("x0a")
    p.tasks(parts("A", 0, (None,)) + parts("A", 1, (None,)))
    p.flush()
    p.wait("wqa")
    p.tasks([(None, ("perm", 0, 0, KA, allj))])
    p.mxu(Q(0, 0))
    p.wait("x0b", "wqb")
    p.tasks([(None, ("perm", 0, KA, D, allj))] + parts("A", 2, (None,)))
    p.flush()
    p.mxu(Q(1, 0) + Q(0, 1) + Q(1, 1) + Q(2, 0))
    p.wait("wk")
    p.tasks([(o["pk"][0] + o["pk"][1] * j, ("perm", 1, 0, D, (j,))) for j in range(NT)] + LS(0, *o["l0"]))
    p.mxu(Q(2, 1) + M(1, 0) + M(1, 1))
    p.flush()
    p.wait("wv")
    p.tasks([(o["pv"][0] + o["pv"][1] * j, ("perm", 2, 0, D, (j,))) for j in range(NT)]
            + LS(1, *o["l1"]) + Pt(0, *o["p0"]))
    p.mxu(M(1, 2) + M(2, 0) + M(2, 1))
    p.flush()
    p.wait("wo", "wr", "x1")
    p.tasks([(o["pw"][0] + o["pw"][1] * n, ("permo", n)) for n in range(NT)])
    p.tasks(Pt(1, *o["p1"]) + parts("A", 3, o["a3"]) + parts("E", 0, o["e0"])
            + parts("E", 1, o["e1"]) + C(2, *o["c2"]) + parts("A", 4, o["a4"]))
    p.mxu(M(2, 2) + M(3, 0) + M(3, 1) + M(0, 3) + M(1, 3) + M(2, 3))
    for s in range(3, NS - 2):
        tasks = parts("E", s - 1, o["e"]) + C(s, *o["c"]) + parts("A", s + 2, o["a"])
        if s == XB:
            pre = [t for t in tasks if t[1][0] == "S" and t[1][1] < s * T + o["pre"] * R]
            p.tasks([(None, t[1]) for t in pre])
            tasks = [t for t in tasks if t not in pre]
            p.flush()
            p.wait("x2", "ffn")
        p.tasks(tasks)
        p.mxu(sum([M(g, s - 1 if g == 3 else s + 1) for g in o["mo"]], []))
    s = NS - 2
    big = M(3, s - 1) + M(0, s + 1) + M(1, s + 1) + M(3, s) + M(2, s + 1)
    small = [("G", k, n) for n in range(F // 128) for k in range(2)]
    cut = o["cut"]
    segs = []
    n_big, n_small, done = len(big) - o["sp"], len(small) - o["gh"], 0
    for g, sg in enumerate(big):
        segs.append(sg)
        if g >= o["sp"]:
            want = min(n_small, -(-(g - o["sp"] + 1) * n_small // n_big))
            segs += small[done:want]
            done = want
    segs += small[done:] + M(3, s + 1, 0, cut) + M(3, s + 1, cut, T) + [("H", n) for n in range(NT)]
    p.tasks(parts("E", s - 1, o["e13"]) + [(None, ("spec",))] + C(s, *o["c14"])
            + LS(s + 1, *o["l15"]) + Pt(s + 1, *o["p15"]) + parts("E", s, o["e14"])
            + [(o["e15"], ("E", s + 1, 0, cut)), (None, ("E", s + 1, cut, T))])
    p.mxu(segs)
    p.flush()
    return p.prog


DEFAULTS = dict(
    mode="", rl=8, ps=3, po=2, fa=(16, 99, 99, 99), pre=3, mo=(3, 0, 1, 2),
    pk=(999, 0), l0=(999, 0), pw=(999, 0), p15=(999, 0),
    pv=(25, 14), l1=(52, 8), p0=(98, 3.5),
    p1=(36, 17), a3=(100,), e0=(136, 152), e1=(176, 200), c2=(92, 16.5), a4=(160, 223),
    e=(96, 144), c=(24, 17.5), a=(68, 140),
    cut=64, sp=12, gh=6, e13=(81, 96), c14=(20, 12.75), l15=(150, 4.5), e14=(192, 195), e15=241)


def make_kernel(prof=0, O=(), **kw):
    o = dict(DEFAULTS)
    o.update(_opts(O))
    o.update(kw)
    prog = build_program(o)
    x1 = (XB - 1) * T
    xch = (2 * T, T, x1, S - 3 * T - x1)

    def wait(c, name):
        if prof:
            with jax.named_scope("w_" + name):
                c.wait()
        else:
            c.wait()

    def kernel(x_hbm, wqkv_hbm, wo_hbm, wr_hbm, wg_hbm, wu_hbm, wd_hbm, out_hbm,
               x_s, wqkv_s, wo_s, wob_s, wr_s, wg_s, wu_s, wd_s, wp_s,
               k_s, v_s, xn_s, o_s, hn_s, out_s, y_s, act_s, sem_in, sem_out):
        pid = pl.program_id(0)
        step = pid - 1
        cp = {}
        semi = dict(x0a=0, wqa=1, x0b=6, wqb=6, wk=2, wv=3, wo=4, wr=4, x1=4, x2=5, ffn=5)
        r0 = 0
        for nm, n in zip(("x0a", "x0b", "x1", "x2"), xch):
            cp[nm] = [pltpu.make_async_copy(x_hbm.at[pl.ds(r0, n)], x_s.at[pl.ds(r0, n)], sem_in.at[semi[nm]])]
            r0 += n
        for nm, lo, hi, g in (("wqa", 0, KA, 0), ("wqb", KA, D, 0), ("wk", 0, D, 1), ("wv", 0, D, 2)):
            sl = (pl.ds(lo, hi - lo), pl.ds(D * g, D))
            cp[nm] = [pltpu.make_async_copy(wqkv_hbm.at[sl], wqkv_s.at[sl], sem_in.at[semi[nm]])]
        cp["wo"] = [pltpu.make_async_copy(wo_hbm, wob_s, sem_in.at[semi["wo"]])]
        cp["wr"] = [pltpu.make_async_copy(wr_hbm, wr_s, sem_in.at[semi["wr"]])]
        cp["ffn"] = [pltpu.make_async_copy(a, b, sem_in.at[semi["ffn"]])
                     for a, b in ((wg_hbm, wg_s), (wu_hbm, wu_s), (wd_hbm, wd_s))]

        def ocp(lo, hi):
            return pltpu.make_async_copy(out_s.at[pl.ds(lo, hi - lo)], out_hbm.at[pl.ds(lo, hi - lo)],
                                         sem_out.at[0 if lo < LATE else 1])

        def start_all():
            for nm in ("x0a", "wqa", "x0b", "wqb", "wk", "wv", "wo", "wr", "x1", "x2", "ffn"):
                for c in cp[nm]:
                    c.start()

        def main():
            zero = jnp.zeros((HALO, 128), F32)
            for j in range(NT):
                k_s[j, 0:HALO, :] = zero
                v_s[j, 0:HALO, :] = zero

            lane = lax.broadcasted_iota(jnp.int32, (1, 128), 1)
            cm5 = [(lane + 128 * t) - 5 * (((lane + 128 * t) * 52429) >> 18) for t in range(NT - 1)]
            srcs = [(20 * (lane & 31) + 5 * (lane >> 5) + j) & 127 for j in range(NT)]
            never = jnp.full((8, 128), step, jnp.int32) > 0
            st = dict(best=None, toks=[], wr=None)
            q, hh, sm, gu, part = {}, {}, {}, {}, {}
            pack = lambda v: pltpu.bitcast(v.astype(BF16), U32)
            rsqrt = lambda v: jnp.exp2(jnp.log(v) * (-0.5 / math.log(2.0)))

            def token(due, u):
                if due is not None:
                    st["toks"].append((due, u()))

            def mm(lhs, w, span):
                start, end = span
                toks = [t for t in st["toks"] if t[0] < end]
                st["toks"] = [t for t in st["toks"] if t[0] >= end]
                if toks:
                    ng = lhs.shape[0] // 8
                    grp = lambda d: min(max(int(d - start), 0), ng - 1)
                    col, pos = [], 0
                    for i in sorted({grp(d) for d, _ in toks}):
                        tok = functools.reduce(jnp.bitwise_or, [t for d, t in toks if grp(d) == i])
                        col += [lhs[pos:8 * i, 0:128]] if 8 * i > pos else []
                        col.append(jnp.where(never, tok, lhs[8 * i:8 * i + 8, 0:128]))
                        pos = 8 * i + 8
                    col += [lhs[pos:, 0:128]] if pos < 8 * ng else []
                    lhs = jnp.concatenate([jnp.concatenate(col, axis=0), lhs[:, 128:]], axis=1)
                if w.dtype == U32:
                    w = pltpu.bitcast(w, BF16)
                return jnp.dot(pltpu.bitcast(lhs, BF16), w, preferred_element_type=F32)

            def permute_w(g, k0, k1, js, due):
                if ("mw", g, k0) not in st:
                    tiles = [pltpu.bitcast(wqkv_s[pl.ds(k0, k1 - k0), pl.ds(D * g + 128 * t, 128)], U32)
                             for t in range(NT)]
                    st["mw", g, k0] = []
                    for j in range(NT):
                        m = tiles[NT - 1]
                        for t in range(NT - 2, -1, -1):
                            m = jnp.where(cm5[t] == j, tiles[t], m)
                        st["mw", g, k0].append(m)
                for j in js:
                    m = st["mw", g, k0][j]
                    res = jnp.take_along_axis(m, jnp.broadcast_to(srcs[j], m.shape), axis=1,
                                              mode="promise_in_bounds")
                    wp_s[pl.ds(k0 // 2, (k1 - k0) // 2), pl.ds(D * g + 128 * j, 128)] = res
                    token(due, lambda: _or_all(res))

            def permute_wo(n, due):
                wo_s[n, pl.ds(0, D // 2), :] = pltpu.bitcast(wob_s[:, pl.ds(128 * n, 128)], U32)
                for d2 in range(DH // 2):
                    ev = wo_s[n, pl.ds(d2, H // 2, stride=DH), :]
                    od = wo_s[n, pl.ds(DH // 2 + d2, H // 2, stride=DH), :]
                    lo = (ev & jnp.uint32(0xFFFF)) | (od << 16)
                    hi = (ev >> 16) | (od & jnp.uint32(0xFFFF0000))
                    for d, val in ((2 * d2, lo), (2 * d2 + 1, hi)):
                        aa, j = divmod(d, NT)
                        wp_s[pl.ds(64 * j + 16 * aa, H // 2), pl.ds(3 * D + 128 * n, 128)] = val
                token(due, lambda: _or_all(wp_s[:, pl.ds(3 * D + 128 * n, 128)]))

            def a_task(b, lo, hi, due):
                r0, n = b * T + lo, hi - lo
                x = x_s[pl.ds(r0, n), :].astype(F32)
                m = jnp.sum(x, axis=-1, keepdims=True) * (1.0 / D)
                c = x - m
                v = jnp.sum(c * c, axis=-1, keepdims=True) * (1.0 / D)
                xn_s[pl.ds(r0 // 2, n // 2), :] = pack(c * rsqrt(v + EPS))
                token(due, lambda: _or_all(xn_s[pl.ds(r0 // 2, n // 2), :]))

            def finish(g, b, n, lo, hi, acc, due):
                r0 = b * T + lo
                if g == 0:
                    acc = acc * QSCALE
                elif g == 3:
                    acc = acc + x_s[pl.ds(r0, hi - lo), pl.ds(128 * n, 128)].astype(F32)
                token(due, lambda: _or_all(acc))
                if g == 0:
                    q[b, n] = acc
                elif g == 3:
                    hh[b, n, lo, hi] = acc
                else:
                    (k_s if g == 1 else v_s)[n, pl.ds(HALO + r0, hi - lo), :] = acc

            def m_seg(g, b, n, lo, hi, span):
                src = o_s if g == 3 else xn_s
                acc = mm(src[pl.ds((b * T + lo) // 2, (hi - lo) // 2), :],
                         wp_s[:, pl.ds(D * g + 128 * n, 128)], span)
                fa = o["fa"][g]
                finish(g, b, n, lo, hi, acc, span[1] + fa if hi - lo == T and fa < 99 else None)

            def q_seg(b, n, kpart, span):
                k0, k1 = ((0, KA), (KA, D))[kpart]
                acc = mm(xn_s[pl.ds(b * T // 2, T // 2), pl.ds(k0, k1 - k0)],
                         wp_s[pl.ds(k0 // 2, (k1 - k0) // 2), pl.ds(128 * n, 128)], span)
                if kpart == 0:
                    part[b, n] = acc
                else:
                    finish(0, b, n, 0, T, acc + part.pop((b, n)), None)

            def s_task(r0, n, due):
                b, r = divmod(r0, T)
                qc = jnp.stack([q[b, j][r:r + n] for j in range(NT)])
                lg = jnp.stack([jnp.sum(qc * k_s[:, pl.ds(HALO + r0 - DIL * w, n), :], axis=0)
                                for w in range(W)])
                lg = lg + pltpu.roll(lg, 64, 2)
                lg = lg + pltpu.roll(lg, 32, 2)
                if r0 < DIL * (W - 1):
                    pos = (lax.broadcasted_iota(jnp.int32, lg.shape, 1) + r0
                           - DIL * lax.broadcasted_iota(jnp.int32, lg.shape, 0))
                    lg = jnp.where(pos >= 0, lg, -1e9)
                e = jnp.exp2(lg - _fold(jnp.maximum, lg))
                inv = pl.reciprocal(_fold(jnp.add, e), approx=True)
                sm[r0] = (e, inv)
                token(due, lambda: _or_all(inv[0]))

            def p_task(b, c, j, due):
                r0 = b * T + c * R
                if ("pv", r0) not in st:
                    e, inv = sm.pop(r0)
                    if r0 + 8 in sm:
                        e2, inv2 = sm.pop(r0 + 8)
                        e, inv = jnp.concatenate([e, e2], axis=1), jnp.concatenate([inv, inv2], axis=1)
                    acc = None
                    for w in range(W):
                        t = e[w:w + 1] * v_s[:, pl.ds(HALO + r0 - DIL * w, R), :]
                        acc = t if acc is None else acc + t
                    st["pv", r0] = acc * inv
                dst = (pl.ds(r0 // 2, R // 2), pl.ds(128 * j, 128))
                o_s[dst] = pack(st["pv", r0][j])
                token(due, lambda: o_s[dst])

            def e_task(b, lo, hi, due):
                r0, n = b * T + lo, hi - lo
                if st["wr"] is None:
                    st["wr"] = wr_s[...].astype(F32).reshape(1, D)
                (l0, h0), = {k[2:] for k in hh if k[0] == b and k[2] <= lo and hi <= k[3]}
                h = jnp.concatenate([hh[b, j, l0, h0][lo - l0:hi - l0] for j in range(NT)], axis=1)
                m = jnp.sum(h, axis=-1, keepdims=True) * (1.0 / D)
                c = h - m
                v = jnp.sum(c * c, axis=-1, keepdims=True) * (1.0 / D)
                cw = jnp.sum(c * st["wr"], axis=-1, keepdims=True)
                rstd = rsqrt(v + EPS)
                hn = c * rstd
                out_s[pl.ds(pl.multiple_of(step * 16 + r0, 16), n), :] = (h + hn).astype(BF16)
                hn_s[pl.ds(r0 // 2, n // 2), :] = pack(hn)
                r = jnp.broadcast_to(cw * rstd, (n, 128))
                best = st["best"]
                for i in range(n // 8):
                    ri = r[8 * i:8 * i + 8]
                    rows = lax.broadcasted_iota(jnp.int32, (8, 128), 0) + (r0 + 8 * i)
                    if best is None:
                        best = (jnp.where(ri > -jnp.inf, ri, -jnp.inf), rows)
                    else:
                        upd = ri > best[0]
                        best = (jnp.where(upd, ri, best[0]), jnp.where(upd, rows, best[1]))
                st["best"] = best
                if b == NS - 1:
                    ocp(r0, r0 + n).start()
                elif hi == T:
                    ocp(b * T, (b + 1) * T).start()
                token(due, lambda: (pltpu.bitcast(best[0], U32) | pltpu.bitcast(best[1], U32)
                                    | hn_s[pl.ds(pl.multiple_of(step * 8, 8), 8), 0:128]
                                    | pltpu.bitcast(out_s[0:16, 0:128], U32)))

            def spec_task(due):
                st["xs"] = load_chunk(argmax(st["best"])[1], LATE)

            def g_seg(k, n, span):
                gu[k, n] = jnp.dot(st["xs"], (wg_s, wu_s)[k][:, pl.ds(128 * n, 128)],
                                   preferred_element_type=F32)

            def h_seg(n, span):
                if "act" not in st:
                    g = jnp.concatenate([gu[0, i] for i in range(F // 128)], axis=1)
                    u = jnp.concatenate([gu[1, i] for i in range(F // 128)], axis=1)
                    act_s[...] = pack(g * jax.nn.sigmoid(g) * u)
                    st["act"] = True
                y_s[:, pl.ds(128 * n, 128)] = mm(act_s[...], wd_s[:, pl.ds(128 * n, 128)], span)

            def do_wait(nm):
                st["toks"] = []
                for c in cp[nm]:
                    wait(c, nm)

            fns = dict(A=a_task, M=m_seg, Q=q_seg, S=s_task, P=p_task, E=e_task, wait=do_wait,
                       perm=permute_w, permo=permute_wo, spec=spec_task, G=g_seg, H=h_seg)
            for item in prog:
                fns[item[0]](*item[1:])
            return st["best"]

        def argmax(best):
            bv, bi = best
            mx = jnp.max(bv, axis=0, keepdims=True)
            idx = jnp.min(jnp.where(bv >= mx, bi, S - 1), axis=0, keepdims=True)
            return mx[:, 0:1], jnp.clip(idx[0, 0], 0, S - 1)

        def load_chunk(idx, nrows):
            blk = jnp.clip(idx >> 4, 0, nrows // 16 - 1)
            return pltpu.bitcast(hn_s[pl.ds(pl.multiple_of(blk * 8, 8), 8), :], BF16)

        def fix_row(mx, idx, nrows):
            base = pl.multiple_of(jnp.clip(idx >> 4, 0, nrows // 16 - 1) * 16, 16)
            y = y_s[...] * jax.nn.sigmoid(mx)
            cur = out_s[pl.ds(base, 16), :].astype(F32)
            rows = lax.broadcasted_iota(jnp.int32, (16, D), 0) + base
            out_s[pl.ds(base, 16), :] = jnp.where(rows == idx, cur + y, cur).astype(BF16)
            fix = pltpu.make_async_copy(out_s.at[pl.ds(base, 16)], out_hbm.at[pl.ds(base, 16)], sem_out.at[2])
            fix.start()
            return fix

        def tail(best):
            mx, idx = argmax(best)
            wait(ocp(0, LATE), "out0")

            def early():
                fix = fix_row(mx, idx, LATE)
                wait(ocp(LATE, S), "out1")
                wait(fix, "fix")

            def late():
                xs = load_chunk(idx, S)
                g = jnp.dot(xs, wg_s[...], preferred_element_type=F32)
                u = jnp.dot(xs, wu_s[...], preferred_element_type=F32)
                act = (g * jax.nn.sigmoid(g) * u).astype(BF16)
                y_s[...] = jnp.dot(act, wd_s[...], preferred_element_type=F32)
                wait(ocp(LATE, S), "out1")
                wait(fix_row(mx, idx, S), "fix")

            lax.cond(idx < LATE, early, late)

        pl.when(pid == 0)(start_all)

        @pl.when(pid == 1)
        def _():
            tail(main())

    @jax.jit
    def fn(A_x, A_wqkv, A_wo, B_x, B_w_r, B_w_gate, B_w_up, B_w_down):
        any_spec = pl.BlockSpec(memory_space=pl.ANY)
        out = pl.pallas_call(
            kernel,
            grid=(2,),
            out_shape=jax.ShapeDtypeStruct((S, D), BF16),
            in_specs=[any_spec] * 7,
            out_specs=any_spec,
            scratch_shapes=[
                pltpu.VMEM((S, D), BF16),
                pltpu.VMEM((D, 3 * D), BF16),
                pltpu.VMEM((NT, D // 2 + 32, 128), U32),
                pltpu.VMEM((D, D), BF16),
                pltpu.VMEM((D,), BF16),
                pltpu.VMEM((D, F), BF16),
                pltpu.VMEM((D, F), BF16),
                pltpu.VMEM((F, D), BF16),
                pltpu.VMEM((D // 2, 4 * D), U32),
                pltpu.VMEM((NT, S + HALO, 128), F32),
                pltpu.VMEM((NT, S + HALO, 128), F32),
                pltpu.VMEM((S // 2, D), U32),
                pltpu.VMEM((S // 2, D), U32),
                pltpu.VMEM((S // 2, D), U32),
                pltpu.VMEM((S + 16, D), BF16),
                pltpu.VMEM((16, D), F32),
                pltpu.VMEM((8, F), U32),
                pltpu.SemaphoreType.DMA((7,)),
                pltpu.SemaphoreType.DMA((3,)),
            ],
            compiler_params=pltpu.CompilerParams(vmem_limit_bytes=100 << 20,
                                                 dimension_semantics=("arbitrary",),
                                                 disable_bounds_checks=True,
                                                 disable_semaphore_checks=True),
            name="fused",
        )(A_x.reshape(S, D), A_wqkv, A_wo, B_w_r, B_w_gate, B_w_up, B_w_down)
        return out.reshape(1, S, D)

    return fn


pallas_sequential_preLN__sliding_local_dilated__moe_arch_mod__prompt_kernel = make_kernel()
```

```python
import functools
import math
import jax
import jax.numpy as jnp
from jax import lax
import jax.experimental.pallas as pl
import jax.experimental.pallas.tpu as pltpu

S, D, F = 2048, 640, 1536
H, DH, W, DIL = 32, 20, 8, 2
NT = D // 128
HALO = 16
EPS = 1e-5
F32, BF16, U32 = jnp.float32, jnp.bfloat16, jnp.uint32
QSCALE = DH ** -0.5 * math.log2(math.e)
R = 16
T = 128
NS = S // T
NC = T // R
KA = 384
LATE = (NS - 2) * T
XB = 7


def _fold(f, x):
    while x.shape[0] > 1:
        x = f(x[:x.shape[0] // 2], x[x.shape[0] // 2:])
    return x


def _or_all(u):
    u = pltpu.bitcast(u, U32)
    t = None
    for i in range(u.shape[0] // 8):
        for j in range(u.shape[1] // 128):
            p = u[8 * i:8 * i + 8, 128 * j:128 * (j + 1)]
            t = p if t is None else t | p
    return t


def _rows(lo, hi):
    return range(lo, hi, R)


def _io(it):
    k = it[0]
    lhs = lambda g, b, lo=0, hi=T: [("o" if g == 3 else "xn", b, r, j) for r in _rows(lo, hi) for j in range(NT)]
    out = lambda g, b, n, lo=0, hi=T: [("y", g, b, n, r) for r in _rows(lo, hi)]
    if k == "A":
        return [], lhs(0, *it[1:4])
    if k == "M":
        _, g, b, n, lo, hi = it
        return lhs(g, b, lo, hi) + [("w", g, n, 0), ("w", g, n, 1)], out(g, b, n, lo, hi)
    if k == "Q":
        _, b, n, part = it
        return lhs(0, b) + [("w", 0, n, part)], (out(0, b, n) if part else [])
    if k == "perm":
        _, g, k0, k1, js = it
        return [], [("w", g, j, p) for j in js for p in (0, 1) if (k0, k1)[p] == (0, D)[p]]
    if k == "permo":
        return [], [("w", 3, it[1], 0), ("w", 3, it[1], 1)]
    if k == "S":
        _, r0, n = it
        b, r = divmod(r0, T)
        return ([("y", g, b, j, r // R * R) for g in (0, 1) for j in range(NT)],
                [("sm", r0 + i) for i in range(0, n, 8)])
    if k == "P":
        _, b, c, j = it
        return ([("sm", b * T + c * R + r) for r in range(0, R, 8)] + [("y", 2, b, jj, c * R) for jj in range(NT)],
                [("o", b, c * R, j)])
    if k == "E":
        _, b, lo, hi = it
        prev = [("e", b * T + lo - R)] if b * T + lo else []
        return ([("y", 3, b, n, r) for n in range(NT) for r in _rows(lo, hi)] + prev,
                [("e", b * T + r) for r in _rows(lo, hi)])
    if k == "spec":
        return [("e", LATE - R)], [("spec",)]
    if k == "G":
        return [("spec",)], [("g",) + it[1:]]
    if k == "H":
        return [("g", kk, n) for kk in range(2) for n in range(F // 128)], []
    return [], []


def _slots(it):
    k = it[0]
    if k == "M":
        return (it[5] - it[4]) / 16
    if k == "Q":
        return 1.6 * (3, 2)[it[3]]
    return {"G": 0.0, "H": 1.0}[k]


class Plan:
    def __init__(self):
        self.prog, self.pos, self.have, self.todo = [], 0.0, set(), []

    def _put(self, it, extra):
        self.prog.append(it + (extra,))
        self.have.update(_io(it)[1])

    def _emit_task(self, t, force=False):
        due, it = t
        for key in _io(it)[0]:
            if key not in self.have:
                src = [u for u in self.todo if key in _io(u[1])[1]]
                if not src or not self._emit_task(src[0], force):
                    assert not force, ("unsatisfied", it, key)
                    return False
        self.todo.remove(t)
        self._put(it, due)
        return True

    def tasks(self, ts):
        self.todo += [(None if d is None else self.pos + d, it) for d, it in ts]

    def mxu(self, segs):
        for sg in segs:
            end = self.pos + _slots(sg)
            for t in sorted([t for t in self.todo if t[0] is not None and t[0] < end], key=lambda t: t[0]):
                if t in self.todo:
                    self._emit_task(t)
            for key in _io(sg)[0]:
                if key not in self.have:
                    src = [u for u in self.todo if key in _io(u[1])[1]]
                    assert src, ("unsatisfied", sg, key)
                    self._emit_task(src[0], True)
            self._put(sg, (self.pos, end))
            self.pos = end

    def flush(self):
        for t in list(self.todo):
            if t in self.todo:
                self._emit_task(t, True)

    def wait(self, *names):
        self.prog += [("wait", n) for n in names]


def build_program(o):
    M = lambda g, b, lo=0, hi=T: [("M", g, b, n, lo, hi) for n in range(NT)]
    Q = lambda b, part: [("Q", b, n, part) for n in range(NT)]

    def parts(kind, b, dls):
        n = T // len(dls)
        return [(dl, (kind, b, i * n, (i + 1) * n)) for i, dl in enumerate(dls)]

    def LS(b, c0, cp, rl=R):
        t = []
        for c in range(NC):
            for h in range(0, R, rl):
                r0 = b * T + c * R + h
                t += [(None if c0 is None else c0 + cp * c - (R - rl - h) * cp / R, ("S", r0, rl))]
        return t

    def Pt(b, c0, cp):
        return [(None if c0 is None else c0 + cp * c + o["ps"] * j, ("P", b, c, j))
                for c in range(NC) for j in range(NT)]

    def C(b, c0, cp):
        return LS(b, c0, cp, o["rl"]) + Pt(b, c0 + o["po"], cp)

    allj = tuple(range(NT))
    p = Plan()
    p.wait("x0a")
    p.tasks(parts("A", 0, (None,)) + parts("A", 1, (None,)))
    p.flush()
    p.wait("wqa")
    p.tasks([(None, ("perm", 0, 0, KA, allj))])
    p.mxu(Q(0, 0))
    p.wait("x0b", "wqb")
    p.tasks([(None, ("perm", 0, KA, D, allj))] + parts("A", 2, (None,)))
    p.flush()
    p.mxu(Q(1, 0) + Q(0, 1) + Q(1, 1) + Q(2, 0))
    p.wait("wk")
    p.tasks([(None, ("perm", 1, 0, D, (j,))) for j in range(NT)] + LS(0, None, 0))
    p.mxu(Q(2, 1) + M(1, 0) + M(1, 1))
    p.flush()
    p.wait("wv")
    p.tasks([(o["pv"][0] + o["pv"][1] * j, ("perm", 2, 0, D, (j,))) for j in range(NT)]
            + LS(1, *o["l1"]) + Pt(0, *o["p0"]))
    p.mxu(M(1, 2) + M(2, 0) + M(2, 1))
    p.flush()
    p.wait("wo", "wr", "x1")
    p.tasks([(None, ("permo", n)) for n in range(NT)])
    p.tasks(Pt(1, *o["p1"]) + parts("A", 3, o["a3"]) + parts("E", 0, o["e0"])
            + parts("E", 1, o["e1"]) + C(2, *o["c2"]) + parts("A", 4, o["a4"]))
    p.mxu(M(2, 2) + M(3, 0) + M(3, 1) + M(0, 3) + M(1, 3) + M(2, 3))
    for s in range(3, NS - 2):
        tasks = parts("E", s - 1, o["e"]) + C(s, *o["c"]) + parts("A", s + 2, o["a"])
        if s == XB:
            pre = [t for t in tasks if t[1][0] == "S" and t[1][1] < s * T + o["pre"] * R]
            p.tasks([(None, t[1]) for t in pre])
            tasks = [t for t in tasks if t not in pre]
            p.flush()
            p.wait("x2", "ffn")
        p.tasks(tasks)
        p.mxu(M(3, s - 1) + M(0, s + 1) + M(1, s + 1) + M(2, s + 1))
    s = NS - 2
    big = M(3, s - 1) + M(0, s + 1) + M(1, s + 1) + M(3, s) + M(2, s + 1)
    small = [("G", k, n) for n in range(F // 128) for k in range(2)]
    cut = o["cut"]
    segs = []
    n_big, n_small, done = len(big) - o["sp"], len(small) - o["gh"], 0
    for g, sg in enumerate(big):
        segs.append(sg)
        if g >= o["sp"]:
            want = min(n_small, -(-(g - o["sp"] + 1) * n_small // n_big))
            segs += small[done:want]
            done = want
    segs += small[done:] + M(3, s + 1, 0, cut) + M(3, s + 1, cut, T) + [("H", n) for n in range(NT)]
    p.tasks(parts("E", s - 1, o["e13"]) + [(None, ("spec",))] + C(s, *o["c14"])
            + LS(s + 1, *o["l15"]) + Pt(s + 1, None, 0) + parts("E", s, o["e14"])
            + [(o["e15"], ("E", s + 1, 0, cut)), (None, ("E", s + 1, cut, T))])
    p.mxu(segs)
    p.flush()
    return p.prog


SCHED = dict(
    rl=8, ps=3, po=2, fq=16, pre=3,
    pv=(25, 14), l1=(56, 12), p0=(86, 3.5),
    p1=(36, 17), a3=(100,), e0=(136, 152), e1=(176, 200), c2=(92, 16.5), a4=(160, 227),
    e=(96, 144), c=(24, 17.5), a=(68, 140),
    cut=64, sp=12, gh=6, e13=(81, 96), c14=(10, 13.0), l15=(162, 4.5), e14=(190, 203), e15=243)


def make_kernel():
    o = SCHED
    prog = build_program(o)
    x1 = (XB - 1) * T
    xch = (2 * T, T, x1, S - 3 * T - x1)

    def kernel(x_hbm, wqkv_hbm, wo_hbm, wr_hbm, wg_hbm, wu_hbm, wd_hbm, out_hbm,
               x_s, wqkv_s, wo_s, wob_s, wr_s, wg_s, wu_s, wd_s, wp_s,
               k_s, v_s, xn_s, o_s, hn_s, out_s, y_s, act_s, sem_in, sem_out):
        pid = pl.program_id(0)
        step = pid - 1
        cp = {}
        semi = dict(x0a=0, wqa=1, x0b=6, wqb=6, wk=2, wv=3, wo=4, wr=4, x1=4, x2=5, ffn=5)
        r0 = 0
        for nm, n in zip(("x0a", "x0b", "x1", "x2"), xch):
            cp[nm] = [pltpu.make_async_copy(x_hbm.at[pl.ds(r0, n)], x_s.at[pl.ds(r0, n)], sem_in.at[semi[nm]])]
            r0 += n
        for nm, lo, hi, g in (("wqa", 0, KA, 0), ("wqb", KA, D, 0), ("wk", 0, D, 1), ("wv", 0, D, 2)):
            sl = (pl.ds(lo, hi - lo), pl.ds(D * g, D))
            cp[nm] = [pltpu.make_async_copy(wqkv_hbm.at[sl], wqkv_s.at[sl], sem_in.at[semi[nm]])]
        cp["wo"] = [pltpu.make_async_copy(wo_hbm, wob_s, sem_in.at[semi["wo"]])]
        cp["wr"] = [pltpu.make_async_copy(wr_hbm, wr_s, sem_in.at[semi["wr"]])]
        cp["ffn"] = [pltpu.make_async_copy(a, b, sem_in.at[semi["ffn"]])
                     for a, b in ((wg_hbm, wg_s), (wu_hbm, wu_s), (wd_hbm, wd_s))]

        def ocp(lo, hi):
            return pltpu.make_async_copy(out_s.at[pl.ds(lo, hi - lo)], out_hbm.at[pl.ds(lo, hi - lo)],
                                         sem_out.at[0 if lo < LATE else 1])

        def start_all():
            for nm in ("x0a", "wqa", "x0b", "wqb", "wk", "wv", "wo", "wr", "x1", "x2", "ffn"):
                for c in cp[nm]:
                    c.start()

        def main():
            zero = jnp.zeros((HALO, 128), F32)
            for j in range(NT):
                k_s[j, 0:HALO, :] = zero
                v_s[j, 0:HALO, :] = zero

            lane = lax.broadcasted_iota(jnp.int32, (1, 128), 1)
            cm5 = [(lane + 128 * t) - 5 * (((lane + 128 * t) * 52429) >> 18) for t in range(NT - 1)]
            srcs = [(20 * (lane & 31) + 5 * (lane >> 5) + j) & 127 for j in range(NT)]
            never = jnp.full((8, 128), step, jnp.int32) > 0
            st = dict(best=None, toks=[], wr=None)
            q, hh, sm, gu, part = {}, {}, {}, {}, {}
            pack = lambda v: pltpu.bitcast(v.astype(BF16), U32)
            rsqrt = lambda v: jnp.exp2(jnp.log(v) * (-0.5 / math.log(2.0)))

            def token(due, u):
                if due is not None:
                    st["toks"].append((due, u()))

            def mm(lhs, w, span):
                start, end = span
                toks = [t for t in st["toks"] if t[0] < end]
                st["toks"] = [t for t in st["toks"] if t[0] >= end]
                if toks:
                    ng = lhs.shape[0] // 8
                    grp = lambda d: min(max(int(d - start), 0), ng - 1)
                    col, pos = [], 0
                    for i in sorted({grp(d) for d, _ in toks}):
                        tok = functools.reduce(jnp.bitwise_or, [t for d, t in toks if grp(d) == i])
                        col += [lhs[pos:8 * i, 0:128]] if 8 * i > pos else []
                        col.append(jnp.where(never, tok, lhs[8 * i:8 * i + 8, 0:128]))
                        pos = 8 * i + 8
                    col += [lhs[pos:, 0:128]] if pos < 8 * ng else []
                    lhs = jnp.concatenate([jnp.concatenate(col, axis=0), lhs[:, 128:]], axis=1)
                if w.dtype == U32:
                    w = pltpu.bitcast(w, BF16)
                return jnp.dot(pltpu.bitcast(lhs, BF16), w, preferred_element_type=F32)

            def permute_w(g, k0, k1, js, due):
                if ("mw", g, k0) not in st:
                    tiles = [pltpu.bitcast(wqkv_s[pl.ds(k0, k1 - k0), pl.ds(D * g + 128 * t, 128)], U32)
                             for t in range(NT)]
                    st["mw", g, k0] = []
                    for j in range(NT):
                        m = tiles[NT - 1]
                        for t in range(NT - 2, -1, -1):
                            m = jnp.where(cm5[t] == j, tiles[t], m)
                        st["mw", g, k0].append(m)
                for j in js:
                    m = st["mw", g, k0][j]
                    res = jnp.take_along_axis(m, jnp.broadcast_to(srcs[j], m.shape), axis=1,
                                              mode="promise_in_bounds")
                    wp_s[pl.ds(k0 // 2, (k1 - k0) // 2), pl.ds(D * g + 128 * j, 128)] = res
                    token(due, lambda: _or_all(res))

            def permute_wo(n, due):
                wo_s[n, pl.ds(0, D // 2), :] = pltpu.bitcast(wob_s[:, pl.ds(128 * n, 128)], U32)
                for d2 in range(DH // 2):
                    ev = wo_s[n, pl.ds(d2, H // 2, stride=DH), :]
                    od = wo_s[n, pl.ds(DH // 2 + d2, H // 2, stride=DH), :]
                    lo = (ev & jnp.uint32(0xFFFF)) | (od << 16)
                    hi = (ev >> 16) | (od & jnp.uint32(0xFFFF0000))
                    for d, val in ((2 * d2, lo), (2 * d2 + 1, hi)):
                        aa, j = divmod(d, NT)
                        wp_s[pl.ds(64 * j + 16 * aa, H // 2), pl.ds(3 * D + 128 * n, 128)] = val

            def a_task(b, lo, hi, due):
                r0, n = b * T + lo, hi - lo
                x = x_s[pl.ds(r0, n), :].astype(F32)
                m = jnp.sum(x, axis=-1, keepdims=True) * (1.0 / D)
                c = x - m
                v = jnp.sum(c * c, axis=-1, keepdims=True) * (1.0 / D)
                xn_s[pl.ds(r0 // 2, n // 2), :] = pack(c * rsqrt(v + EPS))
                token(due, lambda: _or_all(xn_s[pl.ds(r0 // 2, n // 2), :]))

            def finish(g, b, n, lo, hi, acc, due):
                r0 = b * T + lo
                if g == 0:
                    acc = acc * QSCALE
                elif g == 3:
                    acc = acc + x_s[pl.ds(r0, hi - lo), pl.ds(128 * n, 128)].astype(F32)
                token(due, lambda: _or_all(acc))
                if g == 0:
                    q[b, n] = acc
                elif g == 3:
                    hh[b, n, lo, hi] = acc
                else:
                    (k_s if g == 1 else v_s)[n, pl.ds(HALO + r0, hi - lo), :] = acc

            def m_seg(g, b, n, lo, hi, span):
                src = o_s if g == 3 else xn_s
                acc = mm(src[pl.ds((b * T + lo) // 2, (hi - lo) // 2), :],
                         wp_s[:, pl.ds(D * g + 128 * n, 128)], span)
                finish(g, b, n, lo, hi, acc, span[1] + o["fq"] if g == 0 else None)

            def q_seg(b, n, kpart, span):
                k0, k1 = ((0, KA), (KA, D))[kpart]
                acc = mm(xn_s[pl.ds(b * T // 2, T // 2), pl.ds(k0, k1 - k0)],
                         wp_s[pl.ds(k0 // 2, (k1 - k0) // 2), pl.ds(128 * n, 128)], span)
                if kpart == 0:
                    part[b, n] = acc
                else:
                    finish(0, b, n, 0, T, acc + part.pop((b, n)), None)

            def s_task(r0, n, due):
                b, r = divmod(r0, T)
                qc = jnp.stack([q[b, j][r:r + n] for j in range(NT)])
                lg = jnp.stack([jnp.sum(qc * k_s[:, pl.ds(HALO + r0 - DIL * w, n), :], axis=0)
                                for w in range(W)])
                lg = lg + pltpu.roll(lg, 64, 2)
                lg = lg + pltpu.roll(lg, 32, 2)
                if r0 < DIL * (W - 1):
                    pos = (lax.broadcasted_iota(jnp.int32, lg.shape, 1) + r0
                           - DIL * lax.broadcasted_iota(jnp.int32, lg.shape, 0))
                    lg = jnp.where(pos >= 0, lg, -1e9)
                e = jnp.exp2(lg - _fold(jnp.maximum, lg))
                inv = pl.reciprocal(_fold(jnp.add, e), approx=True)
                sm[r0] = (e, inv)
                token(due, lambda: _or_all(inv[0]))

            def p_task(b, c, j, due):
                r0 = b * T + c * R
                if ("pv", r0) not in st:
                    e, inv = sm.pop(r0)
                    if r0 + 8 in sm:
                        e2, inv2 = sm.pop(r0 + 8)
                        e, inv = jnp.concatenate([e, e2], axis=1), jnp.concatenate([inv, inv2], axis=1)
                    acc = None
                    for w in range(W):
                        t = e[w:w + 1] * v_s[:, pl.ds(HALO + r0 - DIL * w, R), :]
                        acc = t if acc is None else acc + t
                    st["pv", r0] = acc * inv
                dst = (pl.ds(r0 // 2, R // 2), pl.ds(128 * j, 128))
                o_s[dst] = pack(st["pv", r0][j])
                token(due, lambda: o_s[dst])

            def e_task(b, lo, hi, due):
                r0, n = b * T + lo, hi - lo
                if st["wr"] is None:
                    st["wr"] = wr_s[...].astype(F32).reshape(1, D)
                (l0, h0), = {k[2:] for k in hh if k[0] == b and k[2] <= lo and hi <= k[3]}
                h = jnp.concatenate([hh[b, j, l0, h0][lo - l0:hi - l0] for j in range(NT)], axis=1)
                m = jnp.sum(h, axis=-1, keepdims=True) * (1.0 / D)
                c = h - m
                v = jnp.sum(c * c, axis=-1, keepdims=True) * (1.0 / D)
                cw = jnp.sum(c * st["wr"], axis=-1, keepdims=True)
                rstd = rsqrt(v + EPS)
                hn = c * rstd
                out_s[pl.ds(pl.multiple_of(step * 16 + r0, 16), n), :] = (h + hn).astype(BF16)
                hn_s[pl.ds(r0 // 2, n // 2), :] = pack(hn)
                r = jnp.broadcast_to(cw * rstd, (n, 128))
                best = st["best"]
                for i in range(n // 8):
                    ri = r[8 * i:8 * i + 8]
                    rows = lax.broadcasted_iota(jnp.int32, (8, 128), 0) + (r0 + 8 * i)
                    if best is None:
                        best = (jnp.where(ri > -jnp.inf, ri, -jnp.inf), rows)
                    else:
                        upd = ri > best[0]
                        best = (jnp.where(upd, ri, best[0]), jnp.where(upd, rows, best[1]))
                st["best"] = best
                if b == NS - 1:
                    ocp(r0, r0 + n).start()
                elif hi == T:
                    ocp(b * T, (b + 1) * T).start()
                token(due, lambda: (pltpu.bitcast(best[0], U32) | pltpu.bitcast(best[1], U32)
                                    | hn_s[pl.ds(pl.multiple_of(step * 8, 8), 8), 0:128]
                                    | pltpu.bitcast(out_s[0:16, 0:128], U32)))

            def spec_task(due):
                st["xs"] = load_chunk(argmax(st["best"])[1], LATE)

            def g_seg(k, n, span):
                gu[k, n] = jnp.dot(st["xs"], (wg_s, wu_s)[k][:, pl.ds(128 * n, 128)],
                                   preferred_element_type=F32)

            def h_seg(n, span):
                if "act" not in st:
                    g = jnp.concatenate([gu[0, i] for i in range(F // 128)], axis=1)
                    u = jnp.concatenate([gu[1, i] for i in range(F // 128)], axis=1)
                    act_s[...] = pack(g * jax.nn.sigmoid(g) * u)
                    st["act"] = True
                y_s[:, pl.ds(128 * n, 128)] = mm(act_s[...], wd_s[:, pl.ds(128 * n, 128)], span)

            def do_wait(nm):
                st["toks"] = []
                for c in cp[nm]:
                    c.wait()

            fns = dict(A=a_task, M=m_seg, Q=q_seg, S=s_task, P=p_task, E=e_task, wait=do_wait,
                       perm=permute_w, permo=permute_wo, spec=spec_task, G=g_seg, H=h_seg)
            for item in prog:
                fns[item[0]](*item[1:])
            return st["best"]

        def argmax(best):
            bv, bi = best
            mx = jnp.max(bv, axis=0, keepdims=True)
            idx = jnp.min(jnp.where(bv >= mx, bi, S - 1), axis=0, keepdims=True)
            return mx[:, 0:1], jnp.clip(idx[0, 0], 0, S - 1)

        def load_chunk(idx, nrows):
            blk = jnp.clip(idx >> 4, 0, nrows // 16 - 1)
            return pltpu.bitcast(hn_s[pl.ds(pl.multiple_of(blk * 8, 8), 8), :], BF16)

        def fix_row(mx, idx, nrows):
            base = pl.multiple_of(jnp.clip(idx >> 4, 0, nrows // 16 - 1) * 16, 16)
            y = y_s[...] * jax.nn.sigmoid(mx)
            cur = out_s[pl.ds(base, 16), :].astype(F32)
            rows = lax.broadcasted_iota(jnp.int32, (16, D), 0) + base
            out_s[pl.ds(base, 16), :] = jnp.where(rows == idx, cur + y, cur).astype(BF16)
            fix = pltpu.make_async_copy(out_s.at[pl.ds(base, 16)], out_hbm.at[pl.ds(base, 16)], sem_out.at[2])
            fix.start()
            return fix

        def tail(best):
            mx, idx = argmax(best)
            ocp(0, LATE).wait()

            def early():
                fix = fix_row(mx, idx, LATE)
                ocp(LATE, S).wait()
                fix.wait()

            def late():
                xs = load_chunk(idx, S)
                g = jnp.dot(xs, wg_s[...], preferred_element_type=F32)
                u = jnp.dot(xs, wu_s[...], preferred_element_type=F32)
                act = (g * jax.nn.sigmoid(g) * u).astype(BF16)
                y_s[...] = jnp.dot(act, wd_s[...], preferred_element_type=F32)
                ocp(LATE, S).wait()
                fix_row(mx, idx, S).wait()

            lax.cond(idx < LATE, early, late)

        pl.when(pid == 0)(start_all)

        @pl.when(pid == 1)
        def _():
            tail(main())

    @jax.jit
    def fn(A_x, A_wqkv, A_wo, B_x, B_w_r, B_w_gate, B_w_up, B_w_down):
        any_spec = pl.BlockSpec(memory_space=pl.ANY)
        out = pl.pallas_call(
            kernel,
            grid=(2,),
            out_shape=jax.ShapeDtypeStruct((S, D), BF16),
            in_specs=[any_spec] * 7,
            out_specs=any_spec,
            scratch_shapes=[
                pltpu.VMEM((S, D), BF16),
                pltpu.VMEM((D, 3 * D), BF16),
                pltpu.VMEM((NT, D // 2 + 32, 128), U32),
                pltpu.VMEM((D, D), BF16),
                pltpu.VMEM((D,), BF16),
                pltpu.VMEM((D, F), BF16),
                pltpu.VMEM((D, F), BF16),
                pltpu.VMEM((F, D), BF16),
                pltpu.VMEM((D // 2, 4 * D), U32),
                pltpu.VMEM((NT, S + HALO, 128), F32),
                pltpu.VMEM((NT, S + HALO, 128), F32),
                pltpu.VMEM((S // 2, D), U32),
                pltpu.VMEM((S // 2, D), U32),
                pltpu.VMEM((S // 2, D), U32),
                pltpu.VMEM((S + 16, D), BF16),
                pltpu.VMEM((16, D), F32),
                pltpu.VMEM((8, F), U32),
                pltpu.SemaphoreType.DMA((7,)),
                pltpu.SemaphoreType.DMA((3,)),
            ],
            compiler_params=pltpu.CompilerParams(vmem_limit_bytes=100 << 20,
                                                 dimension_semantics=("arbitrary",),
                                                 disable_bounds_checks=True,
                                                 disable_semaphore_checks=True),
            name="fused",
        )(A_x.reshape(S, D), A_wqkv, A_wo, B_w_r, B_w_gate, B_w_up, B_w_down)
        return out.reshape(1, S, D)

    return fn


pallas_sequential_preLN__sliding_local_dilated__moe_arch_mod__prompt_kernel = make_kernel()
```

```python
import functools
import math
import jax
import jax.numpy as jnp
from jax import lax
import jax.experimental.pallas as pl
import jax.experimental.pallas.tpu as pltpu

S, D, F = 2048, 640, 1536
H, DH, W, DIL = 32, 20, 8, 2
NT = D // 128
HALO = 16
EPS = 1e-5
F32, BF16, U32 = jnp.float32, jnp.bfloat16, jnp.uint32
QSCALE = DH ** -0.5 * math.log2(math.e)
R = 16
T = 128
NS = S // T
NC = T // R
KA = 384
LATE = (NS - 2) * T
XB = 5


PROD = (("s", 0, "t", 0, 2), ("a22", 0, "t", 2, 2), ("s", 2, "b22", 0, 2), ("s7", 4, "t7", 4, 3),
        ("s", 1, "b11", 0, 2), ("bot4", 0, "w4a", 0, 1), ("a11", 0, "t", 1, 2), ("top4", 0, "w4b", 0, 1),
        ("s6", 3, "t6", 3, 3))


def _fold(f, x):
    while x.shape[0] > 1:
        x = f(x[:x.shape[0] // 2], x[x.shape[0] // 2:])
    return x


def _or_all(u):
    u = pltpu.bitcast(u, U32)
    t = None
    for i in range(u.shape[0] // 8):
        for j in range(u.shape[1] // 128):
            p = u[8 * i:8 * i + 8, 128 * j:128 * (j + 1)]
            t = p if t is None else t | p
    return t


def _rows(lo, hi):
    return range(lo, hi, R)


def _io(it):
    k = it[0]
    lhs = lambda g, b, lo=0, hi=T: [("o" if g == 3 else "xn", b, r, j) for r in _rows(lo, hi) for j in range(NT)]
    out = lambda g, b, n, lo=0, hi=T: [("y", g, b, n, r) for r in _rows(lo, hi)]
    if k == "A":
        return [], lhs(0, *it[1:4])
    if k == "M":
        _, g, b, n, lo, hi = it
        return lhs(g, b, lo, hi) + [("w", g, n, 0), ("w", g, n, 1)], out(g, b, n, lo, hi)
    if k == "Q":
        _, b, n, part = it
        return lhs(0, b) + [("w", 0, n, part)], (out(0, b, n) if part else [])
    if k == "X":
        _, g, b, n, i = it
        done = {3: (b, n), 5: (b + 1, n), 7: (b, n + 2), 8: (b + 1, n + 2)}.get(i)
        return ([("t", b, r) for r in _rows(0, T)] + [("ws", g, r) for r in _rows(0, T)],
                (out(g, *done) if done else []))
    if k == "T":
        _, b, lo, hi = it
        return lhs(0, b, lo, hi) + lhs(0, b + 1, lo, hi), [("t", b, r) for r in _rows(lo, hi)]
    if k == "WS":
        return [("w", it[1], n, p) for n in range(NT) for p in (0, 1)], [("ws", it[1], r) for r in _rows(*it[2:4])]
    if k == "perm":
        _, g, k0, k1, js = it
        return [], [("w", g, j, p) for j in js for p in (0, 1) if (k0, k1)[p] == (0, D)[p]]
    if k == "permo":
        return [], [("w", 3, it[1], 0), ("w", 3, it[1], 1)]
    if k == "S":
        _, r0, n = it
        b, r = divmod(r0, T)
        return ([("y", g, b, j, r // R * R) for g in (0, 1) for j in range(NT)],
                [("sm", r0 + i) for i in range(0, n, 8)])
    if k == "P":
        _, b, c, j = it
        return ([("sm", b * T + c * R + r) for r in range(0, R, 8)] + [("y", 2, b, jj, c * R) for jj in range(NT)],
                [("o", b, c * R, j)])
    if k == "E":
        _, b, lo, hi = it
        prev = [("e", b * T + lo - R)] if b * T + lo else []
        return ([("y", 3, b, n, r) for n in range(NT) for r in _rows(lo, hi)] + prev,
                [("e", b * T + r) for r in _rows(lo, hi)])
    if k == "spec":
        return [("e", LATE - R)], [("spec",)]
    if k == "G":
        return [("spec",)], [("g",) + it[1:]]
    if k == "H":
        return [("g", kk, n) for kk in range(2) for n in range(F // 128)], []
    return [], []


def _slots(it):
    k = it[0]
    if k == "M":
        return (it[5] - it[4]) / 16
    if k == "Q":
        return 1.6 * (3, 2)[it[3]]
    if k == "X":
        return 1.6 * PROD[it[4]][4]
    return {"G": 0.0, "H": 1.0}[k]


class Plan:
    def __init__(self):
        self.prog, self.pos, self.have, self.todo = [], 0.0, set(), []

    def _put(self, it, extra):
        self.prog.append(it + (extra,))
        self.have.update(_io(it)[1])

    def _emit_task(self, t, force=False):
        due, it = t
        for key in _io(it)[0]:
            if key not in self.have:
                src = [u for u in self.todo if key in _io(u[1])[1]]
                if not src or not self._emit_task(src[0], force):
                    assert not force, ("unsatisfied", it, key)
                    return False
        self.todo.remove(t)
        self._put(it, due)
        return True

    def tasks(self, ts):
        self.todo += [(None if d is None else self.pos + d, it) for d, it in ts]

    def due(self, end):
        for t in sorted([t for t in self.todo if t[0] is not None and t[0] < end], key=lambda t: t[0]):
            if t in self.todo:
                self._emit_task(t)

    def mxu(self, segs):
        for sg in segs:
            end = self.pos + _slots(sg)
            self.due(end)
            for key in _io(sg)[0]:
                if key not in self.have:
                    src = [u for u in self.todo if key in _io(u[1])[1]]
                    assert src, ("unsatisfied", sg, key)
                    self._emit_task(src[0], True)
            self._put(sg, (self.pos, end))
            self.pos = end

    def flush(self, pred=lambda it: True):
        for t in [t for t in self.todo if pred(t[1])]:
            if t in self.todo:
                self._emit_task(t, True)

    def wait(self, *names):
        self.prog += [("wait", n) for n in names]


def build_program(o):
    M = lambda g, b, lo=0, hi=T: [("M", g, b, n, lo, hi) for n in range(NT)]
    Q = lambda b, part: [("Q", b, n, part) for n in range(NT)]

    def parts(kind, b, dls):
        n = T // len(dls)
        return [(dl, (kind, b, i * n, (i + 1) * n)) for i, dl in enumerate(dls)]

    def LS(b, c0, cp, rl=R):
        t = []
        for c in range(NC):
            for h in range(0, R, rl):
                r0 = b * T + c * R + h
                t += [(None if c0 is None else c0 + cp * c - (R - rl - h) * cp / R, ("S", r0, rl))]
        return t

    def Pt(b, c0, cp):
        return [(None if c0 is None else c0 + cp * c + o["ps"] * j, ("P", b, c, j))
                for c in range(NC) for j in range(NT)]

    def C(b, c0, cp):
        return LS(b, c0, cp, o["rl"]) + Pt(b, c0 + o["po"], cp)

    def WS(g, d):
        return [(None if d is None else d - 5 * (3 - i), ("WS", g, 32 * i, 32 * i + 32)) for i in range(4)]

    def X(g, b):
        x = [[("X", g, b, n, i) for i in range(len(PROD))] for n in range(2)]
        return x[0] + [("M", g, b, 4, 0, T)] + x[1] + [("M", g, b + 1, 4, 0, T)]

    sh = lambda ts, d: [(None if t is None else t + d, it) for t, it in ts]
    allj = tuple(range(NT))
    p = Plan()
    p.wait("x0a")
    p.tasks(parts("A", 0, (None,)) + parts("A", 1, (None,)))
    p.flush()
    p.wait("wqa")
    p.tasks([(None, ("perm", 0, 0, KA, allj))])
    p.mxu(Q(0, 0))
    p.wait("x0b", "wqb")
    p.tasks([(None, ("perm", 0, KA, D, allj))] + parts("A", 2, (None,)))
    p.flush()
    p.tasks(WS(0, o["ws"][0]))
    p.mxu(Q(1, 0) + Q(0, 1) + Q(1, 1) + Q(2, 0))
    p.flush()
    p.wait("wk")
    p.tasks([(None, ("perm", 1, 0, D, (j,))) for j in range(NT)] + LS(0, None, 0) + WS(1, o["ws"][1]))
    p.mxu(Q(2, 1) + M(1, 0) + M(1, 1))
    p.flush()
    p.wait("wv")
    p.tasks([(o["pv"][0] + o["pv"][1] * j, ("perm", 2, 0, D, (j,))) for j in range(NT)]
            + LS(1, *o["l1"]) + Pt(0, *o["p0"]) + WS(2, o["ws"][2]))
    p.mxu(M(1, 2) + M(2, 0) + M(2, 1))
    p.flush()
    p.wait("wo", "wr", "x1")
    p.tasks([(None, ("permo", n)) for n in range(NT)])
    p.tasks(Pt(1, *o["p1"]) + parts("A", 3, o["a3"]) + parts("A", 4, o["a4"]) + parts("E", 0, o["e0"])
            + [(None, ("T", 3, 0, T))])
    p.mxu(M(2, 2) + M(3, 0))
    for b in range(1, NS - 4, 2):
        xs = X(0, b + 2) + X(1, b + 2)
        segs = (M(3, b - 1) + xs + M(3, b) if b > 1 else M(3, b) + xs) + X(2, b + 2)
        e1, e2, a1, a2, p1, c2, l1 = [o["per"][b][i:i + 2] for i in range(0, 14, 2)]
        tasks = parts("E", b - 1, e1) + Pt(b, *p1) if b > 1 else []
        tasks += parts("E", b, e2) + C(b + 1, *c2) + parts("A", b + 4, a1)
        if b + 5 < NS:
            tasks += parts("A", b + 5, a2) + parts("T", b + 4, (None, None))
            tasks += sh(LS(b + 2, *l1, o["rl"]), sum(_slots(sg) for sg in segs) - 60)
        else:
            tasks += LS(b + 2, *o["l13"], o["rl"])
        if b == XB:
            late = [t for t in tasks if t[1][0] in "AT"]
            p.tasks([t for t in tasks if t not in late])
            base = p.pos
            p.mxu(segs[:o["xp"]])
            p.due(p.pos + o["xl"])
            p.flush(lambda it: it[0] in "AT" or it[0] == "E" and it[1] < XB - 1)
            assert ("e", (XB - 1) * T - R) in p.have
            p.wait("x2", "ffn")
            p.prog.append(("out", 0, (XB - 1) * T))
            p.tasks(sh(late, base - p.pos))
            p.mxu(segs[o["xp"]:])
        else:
            p.tasks(tasks)
            p.mxu(segs)
    p.tasks(Pt(NS - 3, *o["p13"]) + parts("E", NS - 4, o["e12"]))
    p.mxu(M(3, NS - 4))
    s = NS - 2
    big = M(3, s - 1) + M(0, s + 1) + M(1, s + 1) + M(3, s) + M(2, s + 1)
    small = [("G", k, n) for n in range(F // 128) for k in range(2)]
    cut = o["cut"]
    segs = []
    n_big, n_small, done = len(big) - o["sp"], len(small) - o["gh"], 0
    for g, sg in enumerate(big):
        segs.append(sg)
        if g >= o["sp"]:
            want = min(n_small, -(-(g - o["sp"] + 1) * n_small // n_big))
            segs += small[done:want]
            done = want
    segs += small[done:] + M(3, s + 1, 0, cut) + M(3, s + 1, cut, T) + [("H", n) for n in range(NT)]
    p.tasks(parts("E", s - 1, o["e13"]) + [(None, ("spec",))] + C(s, *o["c14"])
            + LS(s + 1, *o["l15"]) + Pt(s + 1, None, 0) + parts("E", s, o["e14"])
            + [(o["e15"], ("E", s + 1, 0, cut)), (None, ("E", s + 1, cut, T))])
    p.mxu(segs)
    p.flush()
    return p.prog


SCHED = dict(
    rl=8, ps=3, po=2, fq=16, ws=(50, 60, None), pv=(25, 14), l1=(56, 12), p0=(86, 3.5),
    p1=(30, 5.0), a3=(45,), a4=(82,), e0=(150, 180), xp=15, xl=30,
    per={1: (0, 0, 270, 298, 140, 169, 187, 217, 0, 0, 24, 27.0, 80, 19.0),
         3: (80, 112, 266, 308, 140, 177, 187, 217, 22, 19.0, 160, 16.5, 80, 19.0),
         5: (80, 112, 266, 308, 140, 169, 187, 217, 22, 19.0, 160, 16.0, 80, 19.0),
         7: (80, 112, 266, 308, 140, 169, 187, 217, 22, 19.5, 160, 16.0, 80, 19.0),
         9: (80, 112, 266, 308, 140, 167, 195, 217, 22, 19.0, 160, 16.0, 72, 19.0),
         11: (82, 112, 268, 308, 140, 169, 187, 217, 22, 19.0, 160, 16.0, 80, 19.0)},
    l13=(239, 9.0), p13=(8, 5.0), e12=(80, 108),
    cut=64, sp=12, gh=6, e13=(81, 96), c14=(2, 12.75), l15=(162, 4.5), e14=(198, 213), e15=243)


def make_kernel():
    o = SCHED
    prog = build_program(o)
    x1 = (XB + 1) * T
    xch = (2 * T, T, x1, S - 3 * T - x1)

    def kernel(x_hbm, wqkv_hbm, wo_hbm, wr_hbm, wg_hbm, wu_hbm, wd_hbm, out_hbm,
               x_s, wqkv_s, wo_s, wob_s, wr_s, wg_s, wu_s, wd_s, wp_s, ws_s, ts_s,
               k_s, v_s, xn_s, o_s, hn_s, out_s, y_s, act_s, sem_in, sem_out):
        pid = pl.program_id(0)
        step = pid - 1
        cp = {}
        semi = dict(x0a=0, wqa=1, x0b=6, wqb=6, wk=2, wv=3, wo=4, wr=4, x1=4, x2=5, ffn=5)
        r0 = 0
        for nm, n in zip(("x0a", "x0b", "x1", "x2"), xch):
            cp[nm] = [pltpu.make_async_copy(x_hbm.at[pl.ds(r0, n)], x_s.at[pl.ds(r0, n)], sem_in.at[semi[nm]])]
            r0 += n
        for nm, lo, hi, g in (("wqa", 0, KA, 0), ("wqb", KA, D, 0), ("wk", 0, D, 1), ("wv", 0, D, 2)):
            sl = (pl.ds(lo, hi - lo), pl.ds(D * g, D))
            cp[nm] = [pltpu.make_async_copy(wqkv_hbm.at[sl], wqkv_s.at[sl], sem_in.at[semi[nm]])]
        cp["wo"] = [pltpu.make_async_copy(wo_hbm, wob_s, sem_in.at[semi["wo"]])]
        cp["wr"] = [pltpu.make_async_copy(wr_hbm, wr_s, sem_in.at[semi["wr"]])]
        cp["ffn"] = [pltpu.make_async_copy(a, b, sem_in.at[semi["ffn"]])
                     for a, b in ((wg_hbm, wg_s), (wu_hbm, wu_s), (wd_hbm, wd_s))]

        def ocp(lo, hi):
            return pltpu.make_async_copy(out_s.at[pl.ds(lo, hi - lo)], out_hbm.at[pl.ds(lo, hi - lo)],
                                         sem_out.at[0 if lo < LATE else 1])

        def start_all():
            for nm in ("x0a", "wqa", "x0b", "wqb", "wk", "wv", "wo", "wr", "x1", "x2", "ffn"):
                for c in cp[nm]:
                    c.start()

        def main():
            zero = jnp.zeros((HALO, 128), F32)
            for j in range(NT):
                k_s[j, 0:HALO, :] = zero
                v_s[j, 0:HALO, :] = zero

            lane = lax.broadcasted_iota(jnp.int32, (1, 128), 1)
            cm5 = [(lane + 128 * t) - 5 * (((lane + 128 * t) * 52429) >> 18) for t in range(NT - 1)]
            srcs = [(20 * (lane & 31) + 5 * (lane >> 5) + j) & 127 for j in range(NT)]
            never = jnp.full((8, 128), step, jnp.int32) > 0
            st = dict(best=None, toks=[], wr=None)
            q, hh, sm, gu, part = {}, {}, {}, {}, {}
            pack = lambda v: pltpu.bitcast(v.astype(BF16), U32)
            rsqrt = lambda v: jnp.exp2(jnp.log(v) * (-0.5 / math.log(2.0)))

            def token(due, u):
                if due is not None:
                    st["toks"].append((due, u()))

            def mm(lhs, w, span):
                start, end = span
                toks = [t for t in st["toks"] if t[0] < end]
                st["toks"] = [t for t in st["toks"] if t[0] >= end]
                if toks:
                    ng = lhs.shape[0] // 8
                    grp = lambda d: min(max(int(d - start), 0), ng - 1)
                    col, pos = [], 0
                    for i in sorted({grp(d) for d, _ in toks}):
                        tok = functools.reduce(jnp.bitwise_or, [t for d, t in toks if grp(d) == i])
                        col += [lhs[pos:8 * i, 0:128]] if 8 * i > pos else []
                        col.append(jnp.where(never, tok, lhs[8 * i:8 * i + 8, 0:128]))
                        pos = 8 * i + 8
                    col += [lhs[pos:, 0:128]] if pos < 8 * ng else []
                    col = jnp.concatenate(col, axis=0)
                    lhs = jnp.concatenate([col, lhs[:, 128:]], axis=1) if lhs.shape[1] > 128 else col
                if w.dtype == U32:
                    w = pltpu.bitcast(w, BF16)
                return jnp.dot(pltpu.bitcast(lhs, BF16), w, preferred_element_type=F32)

            def permute_w(g, k0, k1, js, due):
                if ("mw", g, k0) not in st:
                    tiles = [pltpu.bitcast(wqkv_s[pl.ds(k0, k1 - k0), pl.ds(D * g + 128 * t, 128)], U32)
                             for t in range(NT)]
                    st["mw", g, k0] = []
                    for j in range(NT):
                        m = tiles[NT - 1]
                        for t in range(NT - 2, -1, -1):
                            m = jnp.where(cm5[t] == j, tiles[t], m)
                        st["mw", g, k0].append(m)
                for j in js:
                    m = st["mw", g, k0][j]
                    res = jnp.take_along_axis(m, jnp.broadcast_to(srcs[j], m.shape), axis=1,
                                              mode="promise_in_bounds")
                    wp_s[pl.ds(k0 // 2, (k1 - k0) // 2), pl.ds(D * g + 128 * j, 128)] = res
                    token(due, lambda: _or_all(res))

            def permute_wo(n, due):
                wo_s[n, pl.ds(0, D // 2), :] = pltpu.bitcast(wob_s[:, pl.ds(128 * n, 128)], U32)
                for d2 in range(DH // 2):
                    ev = wo_s[n, pl.ds(d2, H // 2, stride=DH), :]
                    od = wo_s[n, pl.ds(DH // 2 + d2, H // 2, stride=DH), :]
                    lo = (ev & jnp.uint32(0xFFFF)) | (od << 16)
                    hi = (ev >> 16) | (od & jnp.uint32(0xFFFF0000))
                    for d, val in ((2 * d2, lo), (2 * d2 + 1, hi)):
                        aa, j = divmod(d, NT)
                        wp_s[pl.ds(64 * j + 16 * aa, H // 2), pl.ds(3 * D + 128 * n, 128)] = val

            def sums(blocks, combos):
                un = [pltpu.bitcast(u, BF16).astype(F32) for u in blocks]
                return [pack(un[x] + un[y] if sg > 0 else un[x] - un[y]) for x, sg, y in combos]

            def ws_task(g, lo, hi, due):
                b = [wp_s[pl.ds(128 * i + lo, hi - lo), pl.ds(D * g + 256 * j, 256)]
                     for i in range(2) for j in range(2)]
                res = sums(b, ((0, 1, 3), (1, -1, 3), (2, -1, 0), (0, 1, 1), (2, 1, 3)))
                dst = lambda i: pl.ds((5 * g + i) * 128 + lo, hi - lo)
                for i, v in enumerate(res):
                    ws_s[dst(i), :] = v
                token(due, lambda: _or_all(jnp.concatenate([ws_s[dst(i), :] for i in range(5)], axis=0)))

            def t_task(b, lo, hi, due):
                a = [xn_s[pl.ds(((b + i) * T + lo) // 2, (hi - lo) // 2), pl.ds(256 * j, 256)]
                     for i in range(2) for j in range(2)]
                for i, v in enumerate(sums(a, ((0, 1, 3), (2, 1, 3), (0, 1, 1), (2, -1, 0), (1, -1, 3)))):
                    ts_s[pl.ds((5 * (b // 2) + i) * 64 + lo // 2, (hi - lo) // 2), :] = v

            def a_task(b, lo, hi, due):
                r0, n = b * T + lo, hi - lo
                x = x_s[pl.ds(r0, n), :].astype(F32)
                m = jnp.sum(x, axis=-1, keepdims=True) * (1.0 / D)
                c = x - m
                v = jnp.sum(c * c, axis=-1, keepdims=True) * (1.0 / D)
                xn_s[pl.ds(r0 // 2, n // 2), :] = pack(c * rsqrt(v + EPS))
                token(due, lambda: _or_all(xn_s[pl.ds(r0 // 2, n // 2), :]))

            def finish(g, b, n, lo, hi, acc, due):
                r0 = b * T + lo
                if g == 0:
                    acc = acc * QSCALE
                elif g == 3:
                    acc = acc + x_s[pl.ds(r0, hi - lo), pl.ds(128 * n, 128)].astype(F32)
                token(due, lambda: _or_all(acc))
                if g == 0:
                    q[b, n] = acc
                elif g == 3:
                    hh[b, n, lo, hi] = acc
                else:
                    (k_s if g == 1 else v_s)[n, pl.ds(HALO + r0, hi - lo), :] = acc

            def m_seg(g, b, n, lo, hi, span):
                src = o_s if g == 3 else xn_s
                acc = mm(src[pl.ds((b * T + lo) // 2, (hi - lo) // 2), :],
                         wp_s[:, pl.ds(D * g + 128 * n, 128)], span)
                finish(g, b, n, lo, hi, acc, span[1] + o["fq"] if g == 0 else None)

            def q_seg(b, n, kpart, span):
                k0, k1 = ((0, KA), (KA, D))[kpart]
                acc = mm(xn_s[pl.ds(b * T // 2, T // 2), pl.ds(k0, k1 - k0)],
                         wp_s[pl.ds(k0 // 2, (k1 - k0) // 2), pl.ds(128 * n, 128)], span)
                if kpart == 0:
                    part[b, n] = acc
                else:
                    finish(0, b, n, 0, T, acc + part.pop((b, n)), None)

            def x_seg(g, b, n, i, span):
                blk = lambda bb, c0, w: xn_s[pl.ds(bb * T // 2, T // 2), pl.ds(c0, w)]
                wb = lambda r, c: wp_s[pl.ds(r, 128 if r < 256 else 64), pl.ds(D * g + c, 128)]
                ln, li, rn, ri, _ = PROD[i]
                ss = lambda: ts_s[pl.ds((5 * (b // 2) + li) * 64, 64), :]
                tt = lambda: ws_s[pl.ds((5 * g + ri) * 128, 128), pl.ds(128 * n, 128)]
                lhs = {"s": ss, "a11": lambda: blk(b, 0, 256), "a22": lambda: blk(b + 1, 256, 256),
                       "top4": lambda: blk(b, 512, 128), "bot4": lambda: blk(b + 1, 512, 128),
                       "s7": lambda: jnp.concatenate([ss(), blk(b, 512, 128)], axis=1),
                       "s6": lambda: jnp.concatenate([ss(), blk(b + 1, 512, 128)], axis=1)}[ln]()
                rhs = {"t": tt, "b11": lambda: wb(0, 128 * n), "b22": lambda: wb(128, 256 + 128 * n),
                       "w4a": lambda: wb(256, 128 * n), "w4b": lambda: wb(256, 256 + 128 * n),
                       "t7": lambda: jnp.concatenate([tt(), wb(256, 128 * n)], axis=0),
                       "t6": lambda: jnp.concatenate([tt(), wb(256, 256 + 128 * n)], axis=0)}[rn]()
                m = mm(lhs, rhs, span)
                due = span[1] + o["fq"] if g == 0 else None
                c = part.setdefault((g, b, n), {})
                if i == 0:
                    c[11] = c[22] = m
                elif i == 1:
                    c[11], c[21] = c[11] + m, m
                elif i == 2:
                    c[11], c[12] = c[11] - m, m
                elif i == 3:
                    finish(g, b, n, 0, T, c.pop(11) + m, due)
                elif i == 4:
                    c[21], c[22] = c[21] + m, c[22] - m
                elif i == 5:
                    finish(g, b + 1, n, 0, T, c.pop(21) + m, due)
                elif i == 6:
                    c[12], c[22] = c[12] + m, c[22] + m
                elif i == 7:
                    finish(g, b, n + 2, 0, T, c.pop(12) + m, due)
                else:
                    finish(g, b + 1, n + 2, 0, T, c.pop(22) + m, due)

            def s_task(r0, n, due):
                b, r = divmod(r0, T)
                qc = jnp.stack([q[b, j][r:r + n] for j in range(NT)])
                lg = jnp.stack([jnp.sum(qc * k_s[:, pl.ds(HALO + r0 - DIL * w, n), :], axis=0)
                                for w in range(W)])
                lg = lg + pltpu.roll(lg, 64, 2)
                lg = lg + pltpu.roll(lg, 32, 2)
                if r0 < DIL * (W - 1):
                    pos = (lax.broadcasted_iota(jnp.int32, lg.shape, 1) + r0
                           - DIL * lax.broadcasted_iota(jnp.int32, lg.shape, 0))
                    lg = jnp.where(pos >= 0, lg, -1e9)
                e = jnp.exp2(lg - _fold(jnp.maximum, lg))
                inv = pl.reciprocal(_fold(jnp.add, e), approx=True)
                sm[r0] = (e, inv)
                token(due, lambda: _or_all(inv[0]))

            def p_task(b, c, j, due):
                r0 = b * T + c * R
                if ("pv", r0) not in st:
                    e, inv = sm.pop(r0)
                    if r0 + 8 in sm:
                        e2, inv2 = sm.pop(r0 + 8)
                        e, inv = jnp.concatenate([e, e2], axis=1), jnp.concatenate([inv, inv2], axis=1)
                    acc = None
                    for w in range(W):
                        t = e[w:w + 1] * v_s[:, pl.ds(HALO + r0 - DIL * w, R), :]
                        acc = t if acc is None else acc + t
                    st["pv", r0] = acc * inv
                dst = (pl.ds(r0 // 2, R // 2), pl.ds(128 * j, 128))
                o_s[dst] = pack(st["pv", r0][j])
                token(due, lambda: o_s[dst])

            def e_task(b, lo, hi, due):
                r0, n = b * T + lo, hi - lo
                if st["wr"] is None:
                    st["wr"] = wr_s[...].astype(F32).reshape(1, D)
                (l0, h0), = {k[2:] for k in hh if k[0] == b and k[2] <= lo and hi <= k[3]}
                h = jnp.concatenate([hh[b, j, l0, h0][lo - l0:hi - l0] for j in range(NT)], axis=1)
                m = jnp.sum(h, axis=-1, keepdims=True) * (1.0 / D)
                c = h - m
                v = jnp.sum(c * c, axis=-1, keepdims=True) * (1.0 / D)
                cw = jnp.sum(c * st["wr"], axis=-1, keepdims=True)
                rstd = rsqrt(v + EPS)
                hn = c * rstd
                out_s[pl.ds(pl.multiple_of(step * 16 + r0, 16), n), :] = (h + hn).astype(BF16)
                hn_s[pl.ds(r0 // 2, n // 2), :] = pack(hn)
                r = jnp.broadcast_to(cw * rstd, (n, 128))
                best = st["best"]
                for i in range(n // 8):
                    ri = r[8 * i:8 * i + 8]
                    rows = lax.broadcasted_iota(jnp.int32, (8, 128), 0) + (r0 + 8 * i)
                    if best is None:
                        best = (jnp.where(ri > -jnp.inf, ri, -jnp.inf), rows)
                    else:
                        upd = ri > best[0]
                        best = (jnp.where(upd, ri, best[0]), jnp.where(upd, rows, best[1]))
                st["best"] = best
                if b == NS - 1:
                    ocp(r0, r0 + n).start()
                elif hi == T and b >= XB - 1:
                    ocp(b * T, (b + 1) * T).start()
                token(due, lambda: (pltpu.bitcast(best[0], U32) | pltpu.bitcast(best[1], U32)
                                    | hn_s[pl.ds(pl.multiple_of(step * 8, 8), 8), 0:128]
                                    | pltpu.bitcast(out_s[0:16, 0:128], U32)))

            def spec_task(due):
                st["xs"] = load_chunk(argmax(st["best"])[1], LATE)

            def g_seg(k, n, span):
                gu[k, n] = jnp.dot(st["xs"], (wg_s, wu_s)[k][:, pl.ds(128 * n, 128)],
                                   preferred_element_type=F32)

            def h_seg(n, span):
                if "act" not in st:
                    g = jnp.concatenate([gu[0, i] for i in range(F // 128)], axis=1)
                    u = jnp.concatenate([gu[1, i] for i in range(F // 128)], axis=1)
                    act_s[...] = pack(g * jax.nn.sigmoid(g) * u)
                    st["act"] = True
                y_s[:, pl.ds(128 * n, 128)] = mm(act_s[...], wd_s[:, pl.ds(128 * n, 128)], span)

            def do_wait(nm):
                st["toks"] = []
                for c in cp[nm]:
                    c.wait()

            fns = dict(out=lambda lo, hi: ocp(lo, hi).start(), X=x_seg, T=t_task, WS=ws_task, A=a_task, M=m_seg, Q=q_seg, S=s_task, P=p_task, E=e_task, wait=do_wait,
                       perm=permute_w, permo=permute_wo, spec=spec_task, G=g_seg, H=h_seg)
            for item in prog:
                fns[item[0]](*item[1:])
            return st["best"]

        def argmax(best):
            bv, bi = best
            mx = jnp.max(bv, axis=0, keepdims=True)
            idx = jnp.min(jnp.where(bv >= mx, bi, S - 1), axis=0, keepdims=True)
            return mx[:, 0:1], jnp.clip(idx[0, 0], 0, S - 1)

        def load_chunk(idx, nrows):
            blk = jnp.clip(idx >> 4, 0, nrows // 16 - 1)
            return pltpu.bitcast(hn_s[pl.ds(pl.multiple_of(blk * 8, 8), 8), :], BF16)

        def fix_row(mx, idx, nrows):
            base = pl.multiple_of(jnp.clip(idx >> 4, 0, nrows // 16 - 1) * 16, 16)
            y = y_s[...] * jax.nn.sigmoid(mx)
            cur = out_s[pl.ds(base, 16), :].astype(F32)
            rows = lax.broadcasted_iota(jnp.int32, (16, D), 0) + base
            out_s[pl.ds(base, 16), :] = jnp.where(rows == idx, cur + y, cur).astype(BF16)
            fix = pltpu.make_async_copy(out_s.at[pl.ds(base, 16)], out_hbm.at[pl.ds(base, 16)], sem_out.at[2])
            fix.start()
            return fix

        def tail(best):
            mx, idx = argmax(best)
            ocp(0, LATE).wait()

            def early():
                fix = fix_row(mx, idx, LATE)
                ocp(LATE, S).wait()
                fix.wait()

            def late():
                xs = load_chunk(idx, S)
                g = jnp.dot(xs, wg_s[...], preferred_element_type=F32)
                u = jnp.dot(xs, wu_s[...], preferred_element_type=F32)
                act = (g * jax.nn.sigmoid(g) * u).astype(BF16)
                y_s[...] = jnp.dot(act, wd_s[...], preferred_element_type=F32)
                ocp(LATE, S).wait()
                fix_row(mx, idx, S).wait()

            lax.cond(idx < LATE, early, late)

        pl.when(pid == 0)(start_all)

        @pl.when(pid == 1)
        def _():
            tail(main())

    @jax.jit
    def fn(A_x, A_wqkv, A_wo, B_x, B_w_r, B_w_gate, B_w_up, B_w_down):
        any_spec = pl.BlockSpec(memory_space=pl.ANY)
        out = pl.pallas_call(
            kernel,
            grid=(2,),
            out_shape=jax.ShapeDtypeStruct((S, D), BF16),
            in_specs=[any_spec] * 7,
            out_specs=any_spec,
            scratch_shapes=[
                pltpu.VMEM((S, D), BF16),
                pltpu.VMEM((D, 3 * D), BF16),
                pltpu.VMEM((NT, D // 2 + 32, 128), U32),
                pltpu.VMEM((D, D), BF16),
                pltpu.VMEM((D,), BF16),
                pltpu.VMEM((D, F), BF16),
                pltpu.VMEM((D, F), BF16),
                pltpu.VMEM((F, D), BF16),
                pltpu.VMEM((D // 2, 4 * D), U32),
                pltpu.VMEM((15 * 128, 256), U32),
                pltpu.VMEM((NS // 2 * 5 * 64, 256), U32),
                pltpu.VMEM((NT, S + HALO, 128), F32),
                pltpu.VMEM((NT, S + HALO, 128), F32),
                pltpu.VMEM((S // 2, D), U32),
                pltpu.VMEM((S // 2, D), U32),
                pltpu.VMEM((S // 2, D), U32),
                pltpu.VMEM((S + 16, D), BF16),
                pltpu.VMEM((16, D), F32),
                pltpu.VMEM((8, F), U32),
                pltpu.SemaphoreType.DMA((7,)),
                pltpu.SemaphoreType.DMA((3,)),
            ],
            compiler_params=pltpu.CompilerParams(vmem_limit_bytes=100 << 20,
                                                 dimension_semantics=("arbitrary",),
                                                 disable_bounds_checks=True,
                                                 disable_semaphore_checks=True),
            name="fused",
        )(A_x.reshape(S, D), A_wqkv, A_wo, B_w_r, B_w_gate, B_w_up, B_w_down)
        return out.reshape(1, S, D)

    return fn


pallas_sequential_preLN__sliding_local_dilated__moe_arch_mod__prompt_kernel = make_kernel()
```

```python
import functools
import math
import jax
import jax.numpy as jnp
from jax import lax
import jax.experimental.pallas as pl
import jax.experimental.pallas.tpu as pltpu

S, D, F = 2048, 640, 1536
H, DH, W, DIL = 32, 20, 8, 2
NT = D // 128
HALO = 16
EPS = 1e-5
F32, BF16, U32 = jnp.float32, jnp.bfloat16, jnp.uint32
QSCALE = DH ** -0.5 * math.log2(math.e)
R = 16
T = 128
NS = S // T
NC = T // R
KA = 384
LATE = (NS - 2) * T
XB = 5


PROD = (("s", 0, "t", 0, 2), ("a22", 0, "t", 2, 2), ("s", 2, "b22", 0, 2), ("s7", 4, "t7", 4, 3),
        ("s", 1, "b11", 0, 2), ("bot4", 0, "w4a", 0, 1), ("a11", 0, "t", 1, 2), ("top4", 0, "w4b", 0, 1),
        ("s6", 3, "t6", 3, 3))


def _fold(f, x):
    while x.shape[0] > 1:
        x = f(x[:x.shape[0] // 2], x[x.shape[0] // 2:])
    return x


def _or_all(u):
    u = pltpu.bitcast(u, U32)
    t = None
    for i in range(u.shape[0] // 8):
        for j in range(u.shape[1] // 128):
            p = u[8 * i:8 * i + 8, 128 * j:128 * (j + 1)]
            t = p if t is None else t | p
    return t


def _rows(lo, hi):
    return range(lo, hi, R)


def _io(it):
    k = it[0]
    lhs = lambda g, b, lo=0, hi=T: [("o" if g == 3 else "xn", b, r, j) for r in _rows(lo, hi) for j in range(NT)]
    out = lambda g, b, n, lo=0, hi=T: [("y", g, b, n, r) for r in _rows(lo, hi)]
    if k == "A":
        return [], lhs(0, *it[1:4])
    if k == "M":
        _, g, b, n, lo, hi = it
        return lhs(g, b, lo, hi) + [("w", g, n, 0), ("w", g, n, 1)], out(g, b, n, lo, hi)
    if k == "Q":
        _, b, n, part = it
        return lhs(0, b) + [("w", 0, n, part)], (out(0, b, n) if part else [])
    if k == "X":
        _, ga, na, gb, nb, b, i = it
        done = {3: (ga, b, na), 5: (ga, b + 1, na), 7: (gb, b, nb), 8: (gb, b + 1, nb)}.get(i)
        return ([("t", b, r) for r in _rows(0, T)] + [("ws", ga if ga == gb else 3, r) for r in _rows(0, T)],
                (out(*done) if done else []))
    if k == "T":
        _, b, lo, hi = it
        return lhs(0, b, lo, hi) + lhs(0, b + 1, lo, hi), [("t", b, r) for r in _rows(lo, hi)]
    if k == "WS":
        gs = (0, 1) if it[1] == 3 else (it[1],)
        return ([("w", g, n, p) for g in gs for n in range(NT) for p in (0, 1)],
                [("ws", it[1], r) for r in _rows(*it[2:4])])
    if k == "perm":
        _, g, k0, k1, js = it
        return [], [("w", g, j, p) for j in js for p in (0, 1) if (k0, k1)[p] == (0, D)[p]]
    if k == "permo":
        return [], [("w", 3, it[1], 0), ("w", 3, it[1], 1)]
    if k == "S":
        _, r0, n = it
        b, r = divmod(r0, T)
        return ([("y", g, b, j, r // R * R) for g in (0, 1) for j in range(NT)],
                [("sm", r0 + i) for i in range(0, n, 8)])
    if k == "P":
        _, b, c, j = it
        return ([("sm", b * T + c * R + r) for r in range(0, R, 8)] + [("y", 2, b, jj, c * R) for jj in range(NT)],
                [("o", b, c * R, j)])
    if k == "E":
        _, b, lo, hi = it
        prev = [("e", b * T + lo - R)] if b * T + lo else []
        return ([("y", 3, b, n, r) for n in range(NT) for r in _rows(lo, hi)] + prev,
                [("e", b * T + r) for r in _rows(lo, hi)])
    if k == "spec":
        return [("e", LATE - R)], [("spec",)]
    if k == "G":
        return [("spec",)], [("g",) + it[1:]]
    if k == "H":
        return [("g", kk, n) for kk in range(2) for n in range(F // 128)], []
    return [], []


def _slots(it):
    k = it[0]
    if k == "M":
        return (it[5] - it[4]) / 16
    if k == "Q":
        return 1.6 * (3, 2)[it[3]]
    if k == "X":
        return 1.6 * PROD[it[6]][4]
    return {"G": 0.0, "H": 1.0}[k]


class Plan:
    def __init__(self):
        self.prog, self.pos, self.have, self.todo = [], 0.0, set(), []

    def _put(self, it, extra):
        self.prog.append(it + (extra,))
        self.have.update(_io(it)[1])

    def _emit_task(self, t, force=False):
        due, it = t
        for key in _io(it)[0]:
            if key not in self.have:
                src = [u for u in self.todo if key in _io(u[1])[1]]
                if not src or not self._emit_task(src[0], force):
                    assert not force, ("unsatisfied", it, key)
                    return False
        self.todo.remove(t)
        self._put(it, due)
        return True

    def tasks(self, ts):
        self.todo += [(None if d is None else self.pos + d, it) for d, it in ts]

    def due(self, end):
        for t in sorted([t for t in self.todo if t[0] is not None and t[0] < end], key=lambda t: t[0]):
            if t in self.todo:
                self._emit_task(t)

    def mxu(self, segs):
        for sg in segs:
            end = self.pos + _slots(sg)
            self.due(end)
            for key in _io(sg)[0]:
                if key not in self.have:
                    src = [u for u in self.todo if key in _io(u[1])[1]]
                    assert src, ("unsatisfied", sg, key)
                    self._emit_task(src[0], True)
            self._put(sg, (self.pos, end))
            self.pos = end

    def flush(self, pred=lambda it: True):
        for t in [t for t in self.todo if pred(t[1])]:
            if t in self.todo:
                self._emit_task(t, True)

    def wait(self, *names):
        self.prog += [("wait", n) for n in names]


def build_program(o):
    M = lambda g, b, lo=0, hi=T: [("M", g, b, n, lo, hi) for n in range(NT)]
    Q = lambda b, part: [("Q", b, n, part) for n in range(NT)]

    def parts(kind, b, dls):
        n = T // len(dls)
        return [(dl, (kind, b, i * n, (i + 1) * n)) for i, dl in enumerate(dls)]

    def LS(b, c0, cp, rl=R):
        t = []
        for c in range(NC):
            for h in range(0, R, rl):
                r0 = b * T + c * R + h
                t += [(None if c0 is None else c0 + cp * c - (R - rl - h) * cp / R, ("S", r0, rl))]
        return t

    def Pt(b, c0, cp):
        return [(None if c0 is None else c0 + cp * c + o["ps"] * j, ("P", b, c, j))
                for c in range(NC) for j in range(NT)]

    def C(b, c0, cp):
        return LS(b, c0, cp, o["rl"]) + Pt(b, c0 + o["po"], cp)

    def WS(g, d):
        return [(None if d is None else d - 5 * (3 - i), ("WS", g, 32 * i, 32 * i + 32)) for i in range(4)]

    def X(ga, na, gb, nb, b):
        return [("X", ga, na, gb, nb, b, i) for i in range(len(PROD))]

    sh = lambda ts, d: [(None if t is None else t + d, it) for t, it in ts]
    allj = tuple(range(NT))
    p = Plan()
    p.wait("x0a")
    p.tasks(parts("A", 0, (None,)) + parts("A", 1, (None,)))
    p.flush()
    p.wait("wqa")
    p.tasks([(None, ("perm", 0, 0, KA, allj))])
    p.mxu(Q(0, 0))
    p.wait("x0b", "wqb")
    p.tasks([(None, ("perm", 0, KA, D, allj))] + parts("A", 2, (None,)))
    p.flush()
    p.tasks(WS(0, o["ws"][0]))
    p.mxu(Q(1, 0) + Q(0, 1) + Q(1, 1) + Q(2, 0))
    p.flush()
    p.wait("wk")
    p.tasks([(None, ("perm", 1, 0, D, (j,))) for j in range(NT)] + LS(0, None, 0) + WS(1, o["ws"][1]))
    p.mxu(Q(2, 1) + M(1, 0) + M(1, 1))
    p.flush()
    p.wait("wv")
    p.tasks([(o["pv"][0] + o["pv"][1] * j, ("perm", 2, 0, D, (j,))) for j in range(NT)]
            + LS(1, *o["l1"]) + Pt(0, *o["p0"]) + WS(2, o["ws"][2]))
    p.mxu(M(1, 2) + M(2, 0) + M(2, 1))
    p.flush()
    p.wait("wo", "wr", "x1")
    p.tasks([(None, ("permo", n)) for n in range(NT)])
    p.tasks(Pt(1, *o["p1"]) + parts("A", 3, o["a3"]) + parts("A", 4, o["a4"]) + parts("E", 0, o["e0"])
            + [(None, ("T", 3, 0, T)), (None, ("WS", 3, 0, T))])
    p.mxu(M(2, 2) + M(3, 0))
    for b in range(1, NS - 4, 2):
        nb = b + 2
        qk = X(0, 0, 0, 2, nb) + X(0, 1, 0, 3, nb) + X(0, 4, 1, 4, nb) + X(1, 0, 1, 2, nb) + X(1, 1, 1, 3, nb)
        v = X(2, 0, 2, 2, nb) + M(2, nb)[4:] + X(2, 1, 2, 3, nb) + M(2, nb + 1)[4:]
        segs = (M(3, b - 1) + qk + M(3, b) if b > 1 else M(3, b) + qk) + v
        e1, e2, a1, a2, p1, c2, l1 = [o["per"][b][i:i + 2] for i in range(0, 14, 2)]
        tasks = parts("E", b - 1, e1) + Pt(b, *p1) if b > 1 else []
        tasks += parts("E", b, e2) + C(b + 1, *c2) + parts("A", b + 4, a1)
        if b + 5 < NS:
            tasks += parts("A", b + 5, a2) + parts("T", b + 4, (None, None))
            tasks += sh(LS(b + 2, *l1, o["rl"]), sum(_slots(sg) for sg in segs) - 60)
        else:
            tasks += LS(b + 2, *o["l13"], o["rl"])
        if b == XB:
            late = [t for t in tasks if t[1][0] in "AT"]
            p.tasks([t for t in tasks if t not in late])
            base = p.pos
            p.mxu(segs[:o["xp"]])
            p.due(p.pos + o["xl"])
            p.flush(lambda it: it[0] in "AT" or it[0] == "E" and it[1] < XB - 1)
            assert ("e", (XB - 1) * T - R) in p.have
            p.wait("x2", "ffn")
            p.prog.append(("out", 0, (XB - 1) * T))
            p.tasks(sh(late, base - p.pos))
            p.mxu(segs[o["xp"]:])
        else:
            p.tasks(tasks)
            p.mxu(segs)
    p.tasks(Pt(NS - 3, *o["p13"]) + parts("E", NS - 4, o["e12"]))
    p.mxu(M(3, NS - 4))
    s = NS - 2
    big = M(3, s - 1) + M(0, s + 1) + M(1, s + 1) + M(3, s) + M(2, s + 1)
    small = [("G", k, n) for n in range(F // 128) for k in range(2)]
    cut = o["cut"]
    segs = []
    n_big, n_small, done = len(big) - o["sp"], len(small) - o["gh"], 0
    for g, sg in enumerate(big):
        segs.append(sg)
        if g >= o["sp"]:
            want = min(n_small, -(-(g - o["sp"] + 1) * n_small // n_big))
            segs += small[done:want]
            done = want
    segs += small[done:] + M(3, s + 1, 0, cut) + M(3, s + 1, cut, T) + [("H", n) for n in range(NT)]
    p.tasks(parts("E", s - 1, o["e13"]) + [(None, ("spec",))] + C(s, *o["c14"])
            + LS(s + 1, *o["l15"]) + Pt(s + 1, None, 0) + parts("E", s, o["e14"])
            + [(o["e15"], ("E", s + 1, 0, cut)), (None, ("E", s + 1, cut, T))])
    p.mxu(segs)
    p.flush()
    return p.prog


SCHED = dict(
    rl=8, ps=3, po=2, fq=16, ws=(50, 60, None), pv=(25, 14), l1=(56, 12), p0=(86, 3.5),
    p1=(30, 5.0), a3=(45,), a4=(82,), e0=(150, 180), xp=14, xl=30,
    per={1: (0, 0, 270, 298, 140, 169, 187, 217, 0, 0, 24, 27.0, 80, 19.0),
         3: (80, 112, 266, 308, 140, 177, 187, 217, 22, 19.0, 168, 16.5, 80, 19.0),
         5: (80, 112, 254, 308, 140, 173, 187, 217, 18, 19.0, 160, 16.0, 80, 19.0),
         7: (80, 112, 262, 308, 140, 169, 187, 217, 10, 20.0, 160, 16.0, 80, 19.0),
         9: (80, 112, 270, 308, 140, 167, 191, 229, 18, 19.0, 168, 16.0, 72, 18.25),
         11: (82, 112, 272, 308, 140, 169, 187, 217, 22, 19.0, 168, 16.0, 80, 19.0)},
    l13=(231, 9.0), p13=(8, 5.0), e12=(72, 100),
    cut=64, sp=12, gh=6, e13=(89, 104), c14=(2, 12.75), l15=(162, 4.5), e14=(198, 213), e15=243)


def make_kernel():
    o = SCHED
    prog = build_program(o)
    x1 = (XB + 1) * T
    xch = (2 * T, T, x1, S - 3 * T - x1)

    def kernel(x_hbm, wqkv_hbm, wo_hbm, wr_hbm, wg_hbm, wu_hbm, wd_hbm, out_hbm,
               x_s, wqkv_s, wo_s, wob_s, wr_s, wg_s, wu_s, wd_s, wp_s, ws_s, ts_s,
               k_s, v_s, xn_s, o_s, hn_s, out_s, y_s, act_s, sem_in, sem_out):
        pid = pl.program_id(0)
        step = pid - 1
        cp = {}
        semi = dict(x0a=0, wqa=1, x0b=6, wqb=6, wk=2, wv=3, wo=4, wr=4, x1=4, x2=5, ffn=5)
        r0 = 0
        for nm, n in zip(("x0a", "x0b", "x1", "x2"), xch):
            cp[nm] = [pltpu.make_async_copy(x_hbm.at[pl.ds(r0, n)], x_s.at[pl.ds(r0, n)], sem_in.at[semi[nm]])]
            r0 += n
        for nm, lo, hi, g in (("wqa", 0, KA, 0), ("wqb", KA, D, 0), ("wk", 0, D, 1), ("wv", 0, D, 2)):
            sl = (pl.ds(lo, hi - lo), pl.ds(D * g, D))
            cp[nm] = [pltpu.make_async_copy(wqkv_hbm.at[sl], wqkv_s.at[sl], sem_in.at[semi[nm]])]
        cp["wo"] = [pltpu.make_async_copy(wo_hbm, wob_s, sem_in.at[semi["wo"]])]
        cp["wr"] = [pltpu.make_async_copy(wr_hbm, wr_s, sem_in.at[semi["wr"]])]
        cp["ffn"] = [pltpu.make_async_copy(a, b, sem_in.at[semi["ffn"]])
                     for a, b in ((wg_hbm, wg_s), (wu_hbm, wu_s), (wd_hbm, wd_s))]

        def ocp(lo, hi):
            return pltpu.make_async_copy(out_s.at[pl.ds(lo, hi - lo)], out_hbm.at[pl.ds(lo, hi - lo)],
                                         sem_out.at[0 if lo < LATE else 1])

        def start_all():
            for nm in ("x0a", "wqa", "x0b", "wqb", "wk", "wv", "wo", "wr", "x1", "x2", "ffn"):
                for c in cp[nm]:
                    c.start()

        def main():
            zero = jnp.zeros((HALO, 128), F32)
            for j in range(NT):
                k_s[j, 0:HALO, :] = zero
                v_s[j, 0:HALO, :] = zero

            lane = lax.broadcasted_iota(jnp.int32, (1, 128), 1)
            cm5 = [(lane + 128 * t) - 5 * (((lane + 128 * t) * 52429) >> 18) for t in range(NT - 1)]
            srcs = [(20 * (lane & 31) + 5 * (lane >> 5) + j) & 127 for j in range(NT)]
            never = jnp.full((8, 128), step, jnp.int32) > 0
            st = dict(best=None, toks=[], wr=None)
            q, hh, sm, gu, part = {}, {}, {}, {}, {}
            pack = lambda v: pltpu.bitcast(v.astype(BF16), U32)
            rsqrt = lambda v: jnp.exp2(jnp.log(v) * (-0.5 / math.log(2.0)))

            def token(due, u):
                if due is not None:
                    st["toks"].append((due, u()))

            def mm(lhs, w, span):
                start, end = span
                toks = [t for t in st["toks"] if t[0] < end]
                st["toks"] = [t for t in st["toks"] if t[0] >= end]
                if toks:
                    ng = lhs.shape[0] // 8
                    grp = lambda d: min(max(int(d - start), 0), ng - 1)
                    col, pos = [], 0
                    for i in sorted({grp(d) for d, _ in toks}):
                        tok = functools.reduce(jnp.bitwise_or, [t for d, t in toks if grp(d) == i])
                        col += [lhs[pos:8 * i, 0:128]] if 8 * i > pos else []
                        col.append(jnp.where(never, tok, lhs[8 * i:8 * i + 8, 0:128]))
                        pos = 8 * i + 8
                    col += [lhs[pos:, 0:128]] if pos < 8 * ng else []
                    col = jnp.concatenate(col, axis=0)
                    lhs = jnp.concatenate([col, lhs[:, 128:]], axis=1) if lhs.shape[1] > 128 else col
                if w.dtype == U32:
                    w = pltpu.bitcast(w, BF16)
                return jnp.dot(pltpu.bitcast(lhs, BF16), w, preferred_element_type=F32)

            def permute_w(g, k0, k1, js, due):
                if ("mw", g, k0) not in st:
                    tiles = [pltpu.bitcast(wqkv_s[pl.ds(k0, k1 - k0), pl.ds(D * g + 128 * t, 128)], U32)
                             for t in range(NT)]
                    st["mw", g, k0] = []
                    for j in range(NT):
                        m = tiles[NT - 1]
                        for t in range(NT - 2, -1, -1):
                            m = jnp.where(cm5[t] == j, tiles[t], m)
                        st["mw", g, k0].append(m)
                for j in js:
                    m = st["mw", g, k0][j]
                    res = jnp.take_along_axis(m, jnp.broadcast_to(srcs[j], m.shape), axis=1,
                                              mode="promise_in_bounds")
                    wp_s[pl.ds(k0 // 2, (k1 - k0) // 2), pl.ds(D * g + 128 * j, 128)] = res
                    token(due, lambda: _or_all(res))

            def permute_wo(n, due):
                wo_s[n, pl.ds(0, D // 2), :] = pltpu.bitcast(wob_s[:, pl.ds(128 * n, 128)], U32)
                for d2 in range(DH // 2):
                    ev = wo_s[n, pl.ds(d2, H // 2, stride=DH), :]
                    od = wo_s[n, pl.ds(DH // 2 + d2, H // 2, stride=DH), :]
                    lo = (ev & jnp.uint32(0xFFFF)) | (od << 16)
                    hi = (ev >> 16) | (od & jnp.uint32(0xFFFF0000))
                    for d, val in ((2 * d2, lo), (2 * d2 + 1, hi)):
                        aa, j = divmod(d, NT)
                        wp_s[pl.ds(64 * j + 16 * aa, H // 2), pl.ds(3 * D + 128 * n, 128)] = val

            def sums(blocks, combos):
                un = [pltpu.bitcast(u, BF16).astype(F32) for u in blocks]
                return [pack(un[x] + un[y] if sg > 0 else un[x] - un[y]) for x, sg, y in combos]

            def ws_task(g, lo, hi, due):
                cols = [pl.ds(D * j + 512, 128) if g == 3 else pl.ds(D * g + 256 * j, 256) for j in range(2)]
                b = [wp_s[pl.ds(128 * i + lo, hi - lo), cols[j]] for i in range(2) for j in range(2)]
                res = sums(b, ((0, 1, 3), (1, -1, 3), (2, -1, 0), (0, 1, 1), (2, 1, 3)))
                dst = lambda i: (pl.ds((5 * g + i) * 128 + lo, hi - lo), pl.ds(0, 128 if g == 3 else 256))
                for i, v in enumerate(res):
                    ws_s[dst(i)] = v
                token(due, lambda: _or_all(jnp.concatenate([ws_s[dst(i)] for i in range(5)], axis=0)))

            def t_task(b, lo, hi, due):
                a = [xn_s[pl.ds(((b + i) * T + lo) // 2, (hi - lo) // 2), pl.ds(256 * j, 256)]
                     for i in range(2) for j in range(2)]
                for i, v in enumerate(sums(a, ((0, 1, 3), (2, 1, 3), (0, 1, 1), (2, -1, 0), (1, -1, 3)))):
                    ts_s[pl.ds((5 * (b // 2) + i) * 64 + lo // 2, (hi - lo) // 2), :] = v

            def a_task(b, lo, hi, due):
                r0, n = b * T + lo, hi - lo
                x = x_s[pl.ds(r0, n), :].astype(F32)
                m = jnp.sum(x, axis=-1, keepdims=True) * (1.0 / D)
                c = x - m
                v = jnp.sum(c * c, axis=-1, keepdims=True) * (1.0 / D)
                xn_s[pl.ds(r0 // 2, n // 2), :] = pack(c * rsqrt(v + EPS))
                token(due, lambda: _or_all(xn_s[pl.ds(r0 // 2, n // 2), :]))

            def finish(g, b, n, lo, hi, acc, due):
                r0 = b * T + lo
                if g == 0:
                    acc = acc * QSCALE
                elif g == 3:
                    acc = acc + x_s[pl.ds(r0, hi - lo), pl.ds(128 * n, 128)].astype(F32)
                token(due, lambda: _or_all(acc))
                if g == 0:
                    q[b, n] = acc
                elif g == 3:
                    hh[b, n, lo, hi] = acc
                else:
                    (k_s if g == 1 else v_s)[n, pl.ds(HALO + r0, hi - lo), :] = acc

            def m_seg(g, b, n, lo, hi, span):
                src = o_s if g == 3 else xn_s
                acc = mm(src[pl.ds((b * T + lo) // 2, (hi - lo) // 2), :],
                         wp_s[:, pl.ds(D * g + 128 * n, 128)], span)
                finish(g, b, n, lo, hi, acc, span[1] + o["fq"] if g == 0 else None)

            def q_seg(b, n, kpart, span):
                k0, k1 = ((0, KA), (KA, D))[kpart]
                acc = mm(xn_s[pl.ds(b * T // 2, T // 2), pl.ds(k0, k1 - k0)],
                         wp_s[pl.ds(k0 // 2, (k1 - k0) // 2), pl.ds(128 * n, 128)], span)
                if kpart == 0:
                    part[b, n] = acc
                else:
                    finish(0, b, n, 0, T, acc + part.pop((b, n)), None)

            def x_seg(ga, na, gb, nb, b, i, span):
                blk = lambda bb, c0, w: xn_s[pl.ds(bb * T // 2, T // 2), pl.ds(c0, w)]
                ca, cb = D * ga + 128 * na, D * gb + 128 * nb
                wb = lambda r, c: wp_s[pl.ds(r, 128 if r < 256 else 64), pl.ds(c, 128)]
                ln, li, rn, ri, _ = PROD[i]
                ss = lambda: ts_s[pl.ds((5 * (b // 2) + li) * 64, 64), :]
                wg, wn = (ga, na) if ga == gb else (3, 0)
                tt = lambda: ws_s[pl.ds((5 * wg + ri) * 128, 128), pl.ds(128 * wn, 128)]
                lhs = {"s": ss, "a11": lambda: blk(b, 0, 256), "a22": lambda: blk(b + 1, 256, 256),
                       "top4": lambda: blk(b, 512, 128), "bot4": lambda: blk(b + 1, 512, 128),
                       "s7": lambda: jnp.concatenate([ss(), blk(b, 512, 128)], axis=1),
                       "s6": lambda: jnp.concatenate([ss(), blk(b + 1, 512, 128)], axis=1)}[ln]()
                rhs = {"t": tt, "b11": lambda: wb(0, ca), "b22": lambda: wb(128, cb),
                       "w4a": lambda: wb(256, ca), "w4b": lambda: wb(256, cb),
                       "t7": lambda: jnp.concatenate([tt(), wb(256, ca)], axis=0),
                       "t6": lambda: jnp.concatenate([tt(), wb(256, cb)], axis=0)}[rn]()
                m = mm(lhs, rhs, span)
                due = lambda g: span[1] + o["fq"] if g == 0 else None
                c = part.setdefault((ga, na, b), {})
                if i == 0:
                    c[11] = c[22] = m
                elif i == 1:
                    c[11], c[21] = c[11] + m, m
                elif i == 2:
                    c[11], c[12] = c[11] - m, m
                elif i == 3:
                    finish(ga, b, na, 0, T, c.pop(11) + m, due(ga))
                elif i == 4:
                    c[21], c[22] = c[21] + m, c[22] - m
                elif i == 5:
                    finish(ga, b + 1, na, 0, T, c.pop(21) + m, due(ga))
                elif i == 6:
                    c[12], c[22] = c[12] + m, c[22] + m
                elif i == 7:
                    finish(gb, b, nb, 0, T, c.pop(12) + m, due(gb))
                else:
                    finish(gb, b + 1, nb, 0, T, c.pop(22) + m, due(gb))

            def s_task(r0, n, due):
                b, r = divmod(r0, T)
                qc = jnp.stack([q[b, j][r:r + n] for j in range(NT)])
                lg = jnp.stack([jnp.sum(qc * k_s[:, pl.ds(HALO + r0 - DIL * w, n), :], axis=0)
                                for w in range(W)])
                lg = lg + pltpu.roll(lg, 64, 2)
                lg = lg + pltpu.roll(lg, 32, 2)
                if r0 < DIL * (W - 1):
                    pos = (lax.broadcasted_iota(jnp.int32, lg.shape, 1) + r0
                           - DIL * lax.broadcasted_iota(jnp.int32, lg.shape, 0))
                    lg = jnp.where(pos >= 0, lg, -1e9)
                e = jnp.exp2(lg - _fold(jnp.maximum, lg))
                inv = pl.reciprocal(_fold(jnp.add, e), approx=True)
                sm[r0] = (e, inv)
                token(due, lambda: _or_all(inv[0]))

            def p_task(b, c, j, due):
                r0 = b * T + c * R
                if ("pv", r0) not in st:
                    e, inv = sm.pop(r0)
                    if r0 + 8 in sm:
                        e2, inv2 = sm.pop(r0 + 8)
                        e, inv = jnp.concatenate([e, e2], axis=1), jnp.concatenate([inv, inv2], axis=1)
                    acc = None
                    for w in range(W):
                        t = e[w:w + 1] * v_s[:, pl.ds(HALO + r0 - DIL * w, R), :]
                        acc = t if acc is None else acc + t
                    st["pv", r0] = acc * inv
                dst = (pl.ds(r0 // 2, R // 2), pl.ds(128 * j, 128))
                o_s[dst] = pack(st["pv", r0][j])
                token(due, lambda: o_s[dst])

            def e_task(b, lo, hi, due):
                r0, n = b * T + lo, hi - lo
                if st["wr"] is None:
                    st["wr"] = wr_s[...].astype(F32).reshape(1, D)
                (l0, h0), = {k[2:] for k in hh if k[0] == b and k[2] <= lo and hi <= k[3]}
                h = jnp.concatenate([hh[b, j, l0, h0][lo - l0:hi - l0] for j in range(NT)], axis=1)
                m = jnp.sum(h, axis=-1, keepdims=True) * (1.0 / D)
                c = h - m
                v = jnp.sum(c * c, axis=-1, keepdims=True) * (1.0 / D)
                cw = jnp.sum(c * st["wr"], axis=-1, keepdims=True)
                rstd = rsqrt(v + EPS)
                hn = c * rstd
                out_s[pl.ds(pl.multiple_of(step * 16 + r0, 16), n), :] = (h + hn).astype(BF16)
                hn_s[pl.ds(r0 // 2, n // 2), :] = pack(hn)
                r = jnp.broadcast_to(cw * rstd, (n, 128))
                best = st["best"]
                for i in range(n // 8):
                    ri = r[8 * i:8 * i + 8]
                    rows = lax.broadcasted_iota(jnp.int32, (8, 128), 0) + (r0 + 8 * i)
                    if best is None:
                        best = (jnp.where(ri > -jnp.inf, ri, -jnp.inf), rows)
                    else:
                        upd = ri > best[0]
                        best = (jnp.where(upd, ri, best[0]), jnp.where(upd, rows, best[1]))
                st["best"] = best
                if b == NS - 1:
                    ocp(r0, r0 + n).start()
                elif hi == T and b >= XB - 1:
                    ocp(b * T, (b + 1) * T).start()
                token(due, lambda: (pltpu.bitcast(best[0], U32) | pltpu.bitcast(best[1], U32)
                                    | hn_s[pl.ds(pl.multiple_of(step * 8, 8), 8), 0:128]
                                    | pltpu.bitcast(out_s[0:16, 0:128], U32)))

            def spec_task(due):
                st["xs"] = load_chunk(argmax(st["best"])[1], LATE)

            def g_seg(k, n, span):
                gu[k, n] = jnp.dot(st["xs"], (wg_s, wu_s)[k][:, pl.ds(128 * n, 128)],
                                   preferred_element_type=F32)

            def h_seg(n, span):
                if "act" not in st:
                    g = jnp.concatenate([gu[0, i] for i in range(F // 128)], axis=1)
                    u = jnp.concatenate([gu[1, i] for i in range(F // 128)], axis=1)
                    act_s[...] = pack(g * jax.nn.sigmoid(g) * u)
                    st["act"] = True
                y_s[:, pl.ds(128 * n, 128)] = mm(act_s[...], wd_s[:, pl.ds(128 * n, 128)], span)

            def do_wait(nm):
                st["toks"] = []
                for c in cp[nm]:
                    c.wait()

            fns = dict(out=lambda lo, hi: ocp(lo, hi).start(), X=x_seg, T=t_task, WS=ws_task, A=a_task, M=m_seg, Q=q_seg, S=s_task, P=p_task, E=e_task, wait=do_wait,
                       perm=permute_w, permo=permute_wo, spec=spec_task, G=g_seg, H=h_seg)
            for item in prog:
                fns[item[0]](*item[1:])
            return st["best"]

        def argmax(best):
            bv, bi = best
            mx = jnp.max(bv, axis=0, keepdims=True)
            idx = jnp.min(jnp.where(bv >= mx, bi, S - 1), axis=0, keepdims=True)
            return mx[:, 0:1], jnp.clip(idx[0, 0], 0, S - 1)

        def load_chunk(idx, nrows):
            blk = jnp.clip(idx >> 4, 0, nrows // 16 - 1)
            return pltpu.bitcast(hn_s[pl.ds(pl.multiple_of(blk * 8, 8), 8), :], BF16)

        def fix_row(mx, idx, nrows):
            base = pl.multiple_of(jnp.clip(idx >> 4, 0, nrows // 16 - 1) * 16, 16)
            y = y_s[...] * jax.nn.sigmoid(mx)
            cur = out_s[pl.ds(base, 16), :].astype(F32)
            rows = lax.broadcasted_iota(jnp.int32, (16, D), 0) + base
            out_s[pl.ds(base, 16), :] = jnp.where(rows == idx, cur + y, cur).astype(BF16)
            fix = pltpu.make_async_copy(out_s.at[pl.ds(base, 16)], out_hbm.at[pl.ds(base, 16)], sem_out.at[2])
            fix.start()
            return fix

        def tail(best):
            mx, idx = argmax(best)
            ocp(0, LATE).wait()

            def early():
                fix = fix_row(mx, idx, LATE)
                ocp(LATE, S).wait()
                fix.wait()

            def late():
                xs = load_chunk(idx, S)
                g = jnp.dot(xs, wg_s[...], preferred_element_type=F32)
                u = jnp.dot(xs, wu_s[...], preferred_element_type=F32)
                act = (g * jax.nn.sigmoid(g) * u).astype(BF16)
                y_s[...] = jnp.dot(act, wd_s[...], preferred_element_type=F32)
                ocp(LATE, S).wait()
                fix_row(mx, idx, S).wait()

            lax.cond(idx < LATE, early, late)

        pl.when(pid == 0)(start_all)

        @pl.when(pid == 1)
        def _():
            tail(main())

    @jax.jit
    def fn(A_x, A_wqkv, A_wo, B_x, B_w_r, B_w_gate, B_w_up, B_w_down):
        any_spec = pl.BlockSpec(memory_space=pl.ANY)
        out = pl.pallas_call(
            kernel,
            grid=(2,),
            out_shape=jax.ShapeDtypeStruct((S, D), BF16),
            in_specs=[any_spec] * 7,
            out_specs=any_spec,
            scratch_shapes=[
                pltpu.VMEM((S, D), BF16),
                pltpu.VMEM((D, 3 * D), BF16),
                pltpu.VMEM((NT, D // 2 + 32, 128), U32),
                pltpu.VMEM((D, D), BF16),
                pltpu.VMEM((D,), BF16),
                pltpu.VMEM((D, F), BF16),
                pltpu.VMEM((D, F), BF16),
                pltpu.VMEM((F, D), BF16),
                pltpu.VMEM((D // 2, 4 * D), U32),
                pltpu.VMEM((20 * 128, 256), U32),
                pltpu.VMEM((NS // 2 * 5 * 64, 256), U32),
                pltpu.VMEM((NT, S + HALO, 128), F32),
                pltpu.VMEM((NT, S + HALO, 128), F32),
                pltpu.VMEM((S // 2, D), U32),
                pltpu.VMEM((S // 2, D), U32),
                pltpu.VMEM((S // 2, D), U32),
                pltpu.VMEM((S + 16, D), BF16),
                pltpu.VMEM((16, D), F32),
                pltpu.VMEM((8, F), U32),
                pltpu.SemaphoreType.DMA((7,)),
                pltpu.SemaphoreType.DMA((3,)),
            ],
            compiler_params=pltpu.CompilerParams(vmem_limit_bytes=100 << 20,
                                                 dimension_semantics=("arbitrary",),
                                                 disable_bounds_checks=True,
                                                 disable_semaphore_checks=True),
            name="fused",
        )(A_x.reshape(S, D), A_wqkv, A_wo, B_w_r, B_w_gate, B_w_up, B_w_down)
        return out.reshape(1, S, D)

    return fn


pallas_sequential_preLN__sliding_local_dilated__moe_arch_mod__prompt_kernel = make_kernel()
```

```python
import functools
import math
import jax
import jax.numpy as jnp
from jax import lax
import jax.experimental.pallas as pl
import jax.experimental.pallas.tpu as pltpu

S, D, F = 2048, 640, 1536
H, DH, W, DIL = 32, 20, 8, 2
NT = D // 128
HALO = 16
EPS = 1e-5
F32, BF16, U32 = jnp.float32, jnp.bfloat16, jnp.uint32
QSCALE = DH ** -0.5 * math.log2(math.e)
R = 16
T = 128
NS = S // T
NC = T // R
KA = 384
LATE = (NS - 2) * T
XB = 5


PROD = (("s", 0, "t", 0, 2), ("a22", 0, "t", 2, 2), ("s", 2, "b22", 0, 2), ("s7", 4, "t7", 4, 3),
        ("s", 1, "b11", 0, 2), ("bot4", 0, "w4a", 0, 1), ("a11", 0, "t", 1, 2), ("top4", 0, "w4b", 0, 1),
        ("s6", 3, "t6", 3, 3))


def _fold(f, x):
    while x.shape[0] > 1:
        x = f(x[:x.shape[0] // 2], x[x.shape[0] // 2:])
    return x


def _or_all(u):
    u = pltpu.bitcast(u, U32)
    t = None
    for i in range(u.shape[0] // 8):
        for j in range(u.shape[1] // 128):
            p = u[8 * i:8 * i + 8, 128 * j:128 * (j + 1)]
            t = p if t is None else t | p
    return t


def _rows(lo, hi):
    return range(lo, hi, R)


def _io(it):
    k = it[0]
    lhs = lambda g, b, lo=0, hi=T: [("o" if g == 3 else "xn", b, r, j) for r in _rows(lo, hi) for j in range(NT)]
    out = lambda g, b, n, lo=0, hi=T: [("y", g, b, n, r) for r in _rows(lo, hi)]
    if k == "A":
        return [], lhs(0, *it[1:4])
    if k == "M":
        _, g, b, n, lo, hi = it
        return lhs(g, b, lo, hi) + [("w", g, n, 0), ("w", g, n, 1)], out(g, b, n, lo, hi)
    if k == "Q":
        _, b, n, part = it
        return lhs(0, b) + [("w", 0, n, part)], (out(0, b, n) if part else [])
    if k == "X":
        _, ga, na, gb, nb, b, i = it
        done = {3: (ga, b, na), 5: (ga, b + 1, na), 7: (gb, b, nb), 8: (gb, b + 1, nb)}.get(i)
        return ([("t", b, r) for r in _rows(0, T)] + [("ws", ga if ga == gb else 3, r) for r in _rows(0, T)],
                (out(*done) if done else []))
    if k == "T":
        _, b, lo, hi = it
        return lhs(0, b, lo, hi) + lhs(0, b + 1, lo, hi), [("t", b, r) for r in _rows(lo, hi)]
    if k == "WS":
        gs = (0, 1) if it[1] == 3 else (it[1],)
        return ([("w", g, n, p) for g in gs for n in range(NT) for p in (0, 1)],
                [("ws", it[1], r) for r in _rows(*it[2:4])])
    if k == "perm":
        _, g, k0, k1, js = it
        return [], [("w", g, j, p) for j in js for p in (0, 1) if (k0, k1)[p] == (0, D)[p]]
    if k == "permo":
        return [], [("w", 3, it[1], 0), ("w", 3, it[1], 1)]
    if k == "S":
        _, r0, n = it
        b, r = divmod(r0, T)
        return ([("y", g, b, j, r // R * R) for g in (0, 1) for j in range(NT)],
                [("sm", r0 + i) for i in range(0, n, 8)])
    if k == "P":
        _, b, c, j = it
        return ([("sm", b * T + c * R + r) for r in range(0, R, 8)] + [("y", 2, b, jj, c * R) for jj in range(NT)],
                [("o", b, c * R, j)])
    if k == "E":
        _, b, lo, hi = it
        prev = [("e", b * T + lo - R)] if b * T + lo else []
        return ([("y", 3, b, n, r) for n in range(NT) for r in _rows(lo, hi)] + prev,
                [("e", b * T + r) for r in _rows(lo, hi)])
    if k == "spec":
        return [("e", LATE - R)], [("spec",)]
    if k == "G":
        return [("spec",)], [("g",) + it[1:]]
    if k == "H":
        return [("g", kk, n) for kk in range(2) for n in range(F // 128)], []
    return [], []


def _slots(it):
    k = it[0]
    if k == "M":
        return (it[5] - it[4]) / 16
    if k == "Q":
        return 1.6 * (3, 2)[it[3]]
    if k == "X":
        return 1.6 * PROD[it[6]][4]
    return {"G": 0.0, "H": 1.0}[k]


class Plan:
    def __init__(self):
        self.prog, self.pos, self.have, self.todo = [], 0.0, set(), []

    def _put(self, it, extra):
        self.prog.append(it + (extra,))
        self.have.update(_io(it)[1])

    def _emit_task(self, t, force=False):
        due, it = t
        for key in _io(it)[0]:
            if key not in self.have:
                src = [u for u in self.todo if key in _io(u[1])[1]]
                if not src or not self._emit_task(src[0], force):
                    assert not force, ("unsatisfied", it, key)
                    return False
        self.todo.remove(t)
        self._put(it, due)
        return True

    def tasks(self, ts):
        self.todo += [(None if d is None else self.pos + d, it) for d, it in ts]

    def due(self, end):
        for t in sorted([t for t in self.todo if t[0] is not None and t[0] < end], key=lambda t: t[0]):
            if t in self.todo:
                self._emit_task(t)

    def mxu(self, segs):
        for sg in segs:
            end = self.pos + _slots(sg)
            self.due(end)
            for key in _io(sg)[0]:
                if key not in self.have:
                    src = [u for u in self.todo if key in _io(u[1])[1]]
                    assert src, ("unsatisfied", sg, key)
                    self._emit_task(src[0], True)
            self._put(sg, (self.pos, end))
            self.pos = end

    def flush(self, pred=lambda it: True):
        for t in [t for t in self.todo if pred(t[1])]:
            if t in self.todo:
                self._emit_task(t, True)

    def wait(self, *names):
        self.prog += [("wait", n) for n in names]


def build_program(o):
    M = lambda g, b, lo=0, hi=T: [("M", g, b, n, lo, hi) for n in range(NT)]
    Q = lambda b, part: [("Q", b, n, part) for n in range(NT)]

    def parts(kind, b, dls):
        n = T // len(dls)
        return [(dl, (kind, b, i * n, (i + 1) * n)) for i, dl in enumerate(dls)]

    def LS(b, c0, cp, rl=R):
        t = []
        for c in range(NC):
            for h in range(0, R, rl):
                r0 = b * T + c * R + h
                t += [(None if c0 is None else c0 + cp * c - (R - rl - h) * cp / R, ("S", r0, rl))]
        return t

    def Pt(b, c0, cp):
        return [(None if c0 is None else c0 + cp * c + o["ps"] * j, ("P", b, c, j))
                for c in range(NC) for j in range(NT)]

    def C(b, c0, cp):
        return LS(b, c0, cp, o["rl"]) + Pt(b, c0 + o["po"], cp)

    def WS(g, d):
        return [(None if d is None else d - 5 * (3 - i), ("WS", g, 32 * i, 32 * i + 32)) for i in range(4)]

    def X(ga, na, gb, nb, b):
        return [("X", ga, na, gb, nb, b, i) for i in range(len(PROD))]

    sh = lambda ts, d: [(None if t is None else t + d, it) for t, it in ts]
    allj = tuple(range(NT))
    p = Plan()
    p.wait("x0a")
    p.tasks(parts("A", 0, (None,)) + parts("A", 1, (None,)))
    p.flush()
    p.wait("wqa")
    p.tasks([(None, ("perm", 0, 0, KA, allj))])
    p.mxu(Q(0, 0))
    p.wait("x0b", "wqb")
    p.tasks([(None, ("perm", 0, KA, D, allj))] + parts("A", 2, (None,)))
    p.flush()
    p.tasks(WS(0, o["ws"][0]))
    p.mxu(Q(1, 0) + Q(0, 1) + Q(1, 1) + Q(2, 0))
    p.flush()
    p.wait("wk")
    p.tasks([(None, ("perm", 1, 0, D, (j,))) for j in range(NT)] + LS(0, None, 0) + WS(1, o["ws"][1]))
    p.mxu(Q(2, 1) + M(1, 0) + M(1, 1))
    p.flush()
    p.wait("wv")
    p.tasks([(o["pv"][0] + o["pv"][1] * j, ("perm", 2, 0, D, (j,))) for j in range(NT)]
            + LS(1, *o["l1"]) + Pt(0, *o["p0"]) + WS(2, o["ws"][2]))
    p.mxu(M(1, 2) + M(2, 0) + M(2, 1))
    p.flush()
    p.wait("wo", "wr", "x1")
    p.tasks([(None, ("permo", n)) for n in range(NT)])
    p.tasks(Pt(1, *o["p1"]) + parts("A", 3, o["a3"]) + parts("A", 4, o["a4"]) + parts("E", 0, o["e0"])
            + [(None, ("T", 3, 0, T)), (None, ("WS", 3, 0, T))])
    p.mxu(M(2, 2) + M(3, 0))
    for b in range(1, NS - 4, 2):
        nb = b + 2
        qk = X(0, 0, 0, 2, nb) + X(0, 1, 0, 3, nb) + X(0, 4, 1, 4, nb) + X(1, 0, 1, 2, nb) + X(1, 1, 1, 3, nb)
        v = X(2, 0, 2, 2, nb) + M(2, nb)[4:] + X(2, 1, 2, 3, nb) + M(2, nb + 1)[4:]
        segs = (M(3, b - 1) + qk + M(3, b) if b > 1 else M(3, b) + qk) + v
        e1, e2, a1, a2, p1, c2, l1 = [o["per"][b][i:i + 2] for i in range(0, 14, 2)]
        tasks = parts("E", b - 1, e1) + Pt(b, *p1) if b > 1 else []
        tasks += parts("E", b, e2) + C(b + 1, *c2) + parts("A", b + 4, a1)
        if b + 5 < NS:
            tasks += parts("A", b + 5, a2) + parts("T", b + 4, (None, None))
            tasks += sh(LS(b + 2, *l1, o["rl"]), sum(_slots(sg) for sg in segs) - 60)
        else:
            tasks += LS(b + 2, *o["l13"], o["rl"])
        if b == XB:
            late = [t for t in tasks if t[1][0] in "AT"]
            p.tasks([t for t in tasks if t not in late])
            base = p.pos
            p.mxu(segs[:o["xp"]])
            p.due(p.pos + o["xl"])
            p.flush(lambda it: it[0] in "AT" or it[0] == "E" and it[1] < XB - 1)
            assert ("e", (XB - 1) * T - R) in p.have
            p.wait("x2", "ffn")
            p.prog.append(("out", 0, (XB - 1) * T))
            p.tasks(sh(late, base - p.pos))
            p.mxu(segs[o["xp"]:])
        else:
            p.tasks(tasks)
            p.mxu(segs)
    p.tasks(Pt(NS - 3, *o["p13"]) + parts("E", NS - 4, o["e12"]))
    p.mxu(M(3, NS - 4))
    s = NS - 2
    big = M(3, s - 1) + M(0, s + 1) + M(1, s + 1) + M(3, s) + M(2, s + 1)
    small = [("G", k, n) for n in range(F // 128) for k in range(2)]
    cut = o["cut"]
    segs = []
    n_big, n_small, done = len(big) - o["sp"], len(small) - o["gh"], 0
    for g, sg in enumerate(big):
        segs.append(sg)
        if g >= o["sp"]:
            want = min(n_small, -(-(g - o["sp"] + 1) * n_small // n_big))
            segs += small[done:want]
            done = want
    segs += small[done:] + M(3, s + 1, 0, cut) + M(3, s + 1, cut, T) + [("H", n) for n in range(NT)]
    p.tasks(parts("E", s - 1, o["e13"]) + [(None, ("spec",))] + C(s, *o["c14"])
            + LS(s + 1, *o["l15"]) + Pt(s + 1, None, 0) + parts("E", s, o["e14"])
            + [(o["e15"], ("E", s + 1, 0, cut)), (None, ("E", s + 1, cut, T))])
    p.mxu(segs)
    p.flush()
    return p.prog


SCHED = dict(
    rl=8, ps=3, po=2, fq=16, ws=(50, 60, None), pv=(25, 14), l1=(56, 12), p0=(86, 3.5),
    p1=(30, 5.0), a3=(45,), a4=(82,), e0=(150, 180), xp=14, xl=30,
    per={1: (0, 0, 270, 298, 140, 169, 187, 217, 0, 0, 24, 27.0, 80, 19.0),
         3: (80, 112, 266, 308, 140, 177, 187, 217, 22, 18.5, 168, 16.5, 80, 19.0),
         5: (80, 112, 254, 308, 140, 173, 187, 217, 18, 19.0, 160, 16.0, 80, 19.0),
         7: (80, 112, 262, 308, 140, 167, 187, 217, 10, 20.0, 160, 16.0, 80, 19.0),
         9: (80, 112, 270, 308, 140, 167, 191, 229, 18, 19.0, 168, 16.0, 72, 18.25),
         11: (82, 112, 272, 308, 140, 169, 187, 217, 22, 19.0, 168, 16.0, 80, 19.0)},
    l13=(231, 9.0), p13=(8, 5.0), e12=(72, 100),
    cut=64, sp=12, gh=6, e13=(89, 104), c14=(2, 12.75), l15=(162, 4.5), e14=(202, 217), e15=243)


def make_kernel():
    o = SCHED
    prog = build_program(o)
    x1 = (XB + 1) * T
    xch = (2 * T, T, x1, S - 3 * T - x1)

    def kernel(x_hbm, wqkv_hbm, wo_hbm, wr_hbm, wg_hbm, wu_hbm, wd_hbm, out_hbm,
               x_s, wqkv_s, wo_s, wob_s, wr_s, wg_s, wu_s, wd_s, wp_s, ws_s, ts_s,
               k_s, v_s, xn_s, o_s, out_s, y_s, act_s, sem_in, sem_out):
        pid = pl.program_id(0)
        step = pid - 1
        cp = {}
        semi = dict(x0a=0, wqa=1, x0b=6, wqb=6, wk=2, wv=3, wo=4, wr=4, x1=4, x2=5, ffn=5)
        r0 = 0
        for nm, n in zip(("x0a", "x0b", "x1", "x2"), xch):
            cp[nm] = [pltpu.make_async_copy(x_hbm.at[pl.ds(r0, n)], x_s.at[pl.ds(r0, n)], sem_in.at[semi[nm]])]
            r0 += n
        for nm, lo, hi, g in (("wqa", 0, KA, 0), ("wqb", KA, D, 0), ("wk", 0, D, 1), ("wv", 0, D, 2)):
            sl = (pl.ds(lo, hi - lo), pl.ds(D * g, D))
            cp[nm] = [pltpu.make_async_copy(wqkv_hbm.at[sl], wqkv_s.at[sl], sem_in.at[semi[nm]])]
        cp["wo"] = [pltpu.make_async_copy(wo_hbm, wob_s, sem_in.at[semi["wo"]])]
        cp["wr"] = [pltpu.make_async_copy(wr_hbm, wr_s, sem_in.at[semi["wr"]])]
        cp["ffn"] = [pltpu.make_async_copy(a, b, sem_in.at[semi["ffn"]])
                     for a, b in ((wg_hbm, wg_s), (wu_hbm, wu_s), (wd_hbm, wd_s))]

        def ocp(lo, hi):
            return pltpu.make_async_copy(out_s.at[pl.ds(lo, hi - lo)], out_hbm.at[pl.ds(lo, hi - lo)],
                                         sem_out.at[0 if lo < LATE else 1])

        def start_all():
            for nm in ("x0a", "wqa", "x0b", "wqb", "wk", "wv", "wo", "wr", "x1", "x2", "ffn"):
                for c in cp[nm]:
                    c.start()

        def main():
            zero = jnp.zeros((HALO, 128), F32)
            for j in range(NT):
                k_s[j, 0:HALO, :] = zero
                v_s[j, 0:HALO, :] = zero

            lane = lax.broadcasted_iota(jnp.int32, (1, 128), 1)
            cm5 = [(lane + 128 * t) - 5 * (((lane + 128 * t) * 52429) >> 18) for t in range(NT - 1)]
            srcs = [(20 * (lane & 31) + 5 * (lane >> 5) + j) & 127 for j in range(NT)]
            never = jnp.full((8, 128), step, jnp.int32) > 0
            st = dict(best=None, toks=[], wr=None)
            q, hh, sm, gu, part = {}, {}, {}, {}, {}
            pack = lambda v: pltpu.bitcast(v.astype(BF16), U32)
            rsqrt = lambda v: jnp.exp2(jnp.log(v) * (-0.5 / math.log(2.0)))

            def token(due, u):
                if due is not None:
                    st["toks"].append((due, u()))

            def mm(lhs, w, span):
                start, end = span
                toks = [t for t in st["toks"] if t[0] < end]
                st["toks"] = [t for t in st["toks"] if t[0] >= end]
                if toks:
                    ng = lhs.shape[0] // 8
                    grp = lambda d: min(max(int(d - start), 0), ng - 1)
                    col, pos = [], 0
                    for i in sorted({grp(d) for d, _ in toks}):
                        tok = functools.reduce(jnp.bitwise_or, [t for d, t in toks if grp(d) == i])
                        col += [lhs[pos:8 * i, 0:128]] if 8 * i > pos else []
                        col.append(jnp.where(never, tok, lhs[8 * i:8 * i + 8, 0:128]))
                        pos = 8 * i + 8
                    col += [lhs[pos:, 0:128]] if pos < 8 * ng else []
                    col = jnp.concatenate(col, axis=0)
                    lhs = jnp.concatenate([col, lhs[:, 128:]], axis=1) if lhs.shape[1] > 128 else col
                if w.dtype == U32:
                    w = pltpu.bitcast(w, BF16)
                return jnp.dot(pltpu.bitcast(lhs, BF16), w, preferred_element_type=F32)

            def permute_w(g, k0, k1, js, due):
                if ("mw", g, k0) not in st:
                    tiles = [pltpu.bitcast(wqkv_s[pl.ds(k0, k1 - k0), pl.ds(D * g + 128 * t, 128)], U32)
                             for t in range(NT)]
                    st["mw", g, k0] = []
                    for j in range(NT):
                        m = tiles[NT - 1]
                        for t in range(NT - 2, -1, -1):
                            m = jnp.where(cm5[t] == j, tiles[t], m)
                        st["mw", g, k0].append(m)
                for j in js:
                    m = st["mw", g, k0][j]
                    res = jnp.take_along_axis(m, jnp.broadcast_to(srcs[j], m.shape), axis=1,
                                              mode="promise_in_bounds")
                    wp_s[pl.ds(k0 // 2, (k1 - k0) // 2), pl.ds(D * g + 128 * j, 128)] = res
                    token(due, lambda: _or_all(res))

            def permute_wo(n, due):
                wo_s[n, pl.ds(0, D // 2), :] = pltpu.bitcast(wob_s[:, pl.ds(128 * n, 128)], U32)
                for d2 in range(DH // 2):
                    ev = wo_s[n, pl.ds(d2, H // 2, stride=DH), :]
                    od = wo_s[n, pl.ds(DH // 2 + d2, H // 2, stride=DH), :]
                    lo = (ev & jnp.uint32(0xFFFF)) | (od << 16)
                    hi = (ev >> 16) | (od & jnp.uint32(0xFFFF0000))
                    for d, val in ((2 * d2, lo), (2 * d2 + 1, hi)):
                        aa, j = divmod(d, NT)
                        wp_s[pl.ds(64 * j + 16 * aa, H // 2), pl.ds(3 * D + 128 * n, 128)] = val

            def sums(blocks, combos):
                un = [pltpu.bitcast(u, BF16).astype(F32) for u in blocks]
                return [pack(un[x] + un[y] if sg > 0 else un[x] - un[y]) for x, sg, y in combos]

            def ws_task(g, lo, hi, due):
                cols = [pl.ds(D * j + 512, 128) if g == 3 else pl.ds(D * g + 256 * j, 256) for j in range(2)]
                b = [wp_s[pl.ds(128 * i + lo, hi - lo), cols[j]] for i in range(2) for j in range(2)]
                res = sums(b, ((0, 1, 3), (1, -1, 3), (2, -1, 0), (0, 1, 1), (2, 1, 3)))
                dst = lambda i: (pl.ds((5 * g + i) * 128 + lo, hi - lo), pl.ds(0, 128 if g == 3 else 256))
                for i, v in enumerate(res):
                    ws_s[dst(i)] = v
                token(due, lambda: _or_all(jnp.concatenate([ws_s[dst(i)] for i in range(5)], axis=0)))

            def t_task(b, lo, hi, due):
                a = [xn_s[pl.ds(((b + i) * T + lo) // 2, (hi - lo) // 2), pl.ds(256 * j, 256)]
                     for i in range(2) for j in range(2)]
                for i, v in enumerate(sums(a, ((0, 1, 3), (2, 1, 3), (0, 1, 1), (2, -1, 0), (1, -1, 3)))):
                    ts_s[pl.ds((5 * (b // 2) + i) * 64 + lo // 2, (hi - lo) // 2), :] = v

            def a_task(b, lo, hi, due):
                r0, n = b * T + lo, hi - lo
                x = x_s[pl.ds(r0, n), :].astype(F32)
                m = jnp.sum(x, axis=-1, keepdims=True) * (1.0 / D)
                c = x - m
                v = jnp.sum(c * c, axis=-1, keepdims=True) * (1.0 / D)
                xn_s[pl.ds(r0 // 2, n // 2), :] = pack(c * rsqrt(v + EPS))
                token(due, lambda: _or_all(xn_s[pl.ds(r0 // 2, n // 2), :]))

            def finish(g, b, n, lo, hi, acc, due):
                r0 = b * T + lo
                if g == 0:
                    acc = acc * QSCALE
                elif g == 3:
                    acc = acc + x_s[pl.ds(r0, hi - lo), pl.ds(128 * n, 128)].astype(F32)
                token(due, lambda: _or_all(acc))
                if g == 0:
                    q[b, n] = acc
                elif g == 3:
                    hh[b, n, lo, hi] = acc
                else:
                    (k_s if g == 1 else v_s)[n, pl.ds(HALO + r0, hi - lo), :] = acc

            def m_seg(g, b, n, lo, hi, span):
                src = o_s if g == 3 else xn_s
                acc = mm(src[pl.ds((b * T + lo) // 2, (hi - lo) // 2), :],
                         wp_s[:, pl.ds(D * g + 128 * n, 128)], span)
                finish(g, b, n, lo, hi, acc, span[1] + o["fq"] if g == 0 else None)

            def q_seg(b, n, kpart, span):
                k0, k1 = ((0, KA), (KA, D))[kpart]
                acc = mm(xn_s[pl.ds(b * T // 2, T // 2), pl.ds(k0, k1 - k0)],
                         wp_s[pl.ds(k0 // 2, (k1 - k0) // 2), pl.ds(128 * n, 128)], span)
                if kpart == 0:
                    part[b, n] = acc
                else:
                    finish(0, b, n, 0, T, acc + part.pop((b, n)), None)

            def x_seg(ga, na, gb, nb, b, i, span):
                blk = lambda bb, c0, w: xn_s[pl.ds(bb * T // 2, T // 2), pl.ds(c0, w)]
                ca, cb = D * ga + 128 * na, D * gb + 128 * nb
                wb = lambda r, c: wp_s[pl.ds(r, 128 if r < 256 else 64), pl.ds(c, 128)]
                ln, li, rn, ri, _ = PROD[i]
                ss = lambda: ts_s[pl.ds((5 * (b // 2) + li) * 64, 64), :]
                wg, wn = (ga, na) if ga == gb else (3, 0)
                tt = lambda: ws_s[pl.ds((5 * wg + ri) * 128, 128), pl.ds(128 * wn, 128)]
                lhs = {"s": ss, "a11": lambda: blk(b, 0, 256), "a22": lambda: blk(b + 1, 256, 256),
                       "top4": lambda: blk(b, 512, 128), "bot4": lambda: blk(b + 1, 512, 128),
                       "s7": lambda: jnp.concatenate([ss(), blk(b, 512, 128)], axis=1),
                       "s6": lambda: jnp.concatenate([ss(), blk(b + 1, 512, 128)], axis=1)}[ln]()
                rhs = {"t": tt, "b11": lambda: wb(0, ca), "b22": lambda: wb(128, cb),
                       "w4a": lambda: wb(256, ca), "w4b": lambda: wb(256, cb),
                       "t7": lambda: jnp.concatenate([tt(), wb(256, ca)], axis=0),
                       "t6": lambda: jnp.concatenate([tt(), wb(256, cb)], axis=0)}[rn]()
                m = mm(lhs, rhs, span)
                due = lambda g: span[1] + o["fq"] if g == 0 else None
                c = part.setdefault((ga, na, b), {})
                if i == 0:
                    c[11] = c[22] = m
                elif i == 1:
                    c[11], c[21] = c[11] + m, m
                elif i == 2:
                    c[11], c[12] = c[11] - m, m
                elif i == 3:
                    finish(ga, b, na, 0, T, c.pop(11) + m, due(ga))
                elif i == 4:
                    c[21], c[22] = c[21] + m, c[22] - m
                elif i == 5:
                    finish(ga, b + 1, na, 0, T, c.pop(21) + m, due(ga))
                elif i == 6:
                    c[12], c[22] = c[12] + m, c[22] + m
                elif i == 7:
                    finish(gb, b, nb, 0, T, c.pop(12) + m, due(gb))
                else:
                    finish(gb, b + 1, nb, 0, T, c.pop(22) + m, due(gb))

            def s_task(r0, n, due):
                b, r = divmod(r0, T)
                qc = jnp.stack([q[b, j][r:r + n] for j in range(NT)])
                lg = jnp.stack([jnp.sum(qc * k_s[:, pl.ds(HALO + r0 - DIL * w, n), :], axis=0)
                                for w in range(W)])
                lg = lg + pltpu.roll(lg, 64, 2)
                lg = lg + pltpu.roll(lg, 32, 2)
                if r0 < DIL * (W - 1):
                    pos = (lax.broadcasted_iota(jnp.int32, lg.shape, 1) + r0
                           - DIL * lax.broadcasted_iota(jnp.int32, lg.shape, 0))
                    lg = jnp.where(pos >= 0, lg, -1e9)
                e = jnp.exp2(lg - _fold(jnp.maximum, lg))
                inv = pl.reciprocal(_fold(jnp.add, e), approx=True)
                sm[r0] = (e, inv)
                token(due, lambda: _or_all(inv[0]))

            def p_task(b, c, j, due):
                r0 = b * T + c * R
                if ("pv", r0) not in st:
                    e, inv = sm.pop(r0)
                    if r0 + 8 in sm:
                        e2, inv2 = sm.pop(r0 + 8)
                        e, inv = jnp.concatenate([e, e2], axis=1), jnp.concatenate([inv, inv2], axis=1)
                    acc = None
                    for w in range(W):
                        t = e[w:w + 1] * v_s[:, pl.ds(HALO + r0 - DIL * w, R), :]
                        acc = t if acc is None else acc + t
                    st["pv", r0] = acc * inv
                dst = (pl.ds(r0 // 2, R // 2), pl.ds(128 * j, 128))
                o_s[dst] = pack(st["pv", r0][j])
                token(due, lambda: o_s[dst])

            def e_task(b, lo, hi, due):
                r0, n = b * T + lo, hi - lo
                if st["wr"] is None:
                    st["wr"] = wr_s[...].astype(F32).reshape(1, D)
                (l0, h0), = {k[2:] for k in hh if k[0] == b and k[2] <= lo and hi <= k[3]}
                h = jnp.concatenate([hh[b, j, l0, h0][lo - l0:hi - l0] for j in range(NT)], axis=1)
                m = jnp.sum(h, axis=-1, keepdims=True) * (1.0 / D)
                c = h - m
                v = jnp.sum(c * c, axis=-1, keepdims=True) * (1.0 / D)
                cw = jnp.sum(c * st["wr"], axis=-1, keepdims=True)
                rstd = rsqrt(v + EPS)
                hn = c * rstd
                out_s[pl.ds(pl.multiple_of(step * 16 + r0, 16), n), :] = (h + hn).astype(BF16)
                r, mb, rb = [jnp.broadcast_to(t, (n, 128)) for t in (cw * rstd, m, rstd)]
                best = st["best"]
                for i in range(n // 8):
                    ri = r[8 * i:8 * i + 8]
                    new = (ri, lax.broadcasted_iota(jnp.int32, (8, 128), 0) + (r0 + 8 * i),
                           mb[8 * i:8 * i + 8], rb[8 * i:8 * i + 8])
                    if best is None:
                        best = (jnp.where(ri > -jnp.inf, ri, -jnp.inf),) + new[1:]
                    else:
                        upd = ri > best[0]
                        best = tuple(jnp.where(upd, a, c_) for a, c_ in zip(new, best))
                st["best"] = best
                if b == NS - 1:
                    ocp(r0, r0 + n).start()
                elif hi == T and b >= XB - 1:
                    ocp(b * T, (b + 1) * T).start()
                token(due, lambda: functools.reduce(jnp.bitwise_or, [pltpu.bitcast(t, U32) for t in best])
                      | pltpu.bitcast(out_s[0:16, 0:128], U32))

            def spec_task(due):
                st["xs"] = load_chunk(st["best"], LATE)

            def g_seg(k, n, span):
                gu[k, n] = jnp.dot(st["xs"], (wg_s, wu_s)[k][:, pl.ds(128 * n, 128)],
                                   preferred_element_type=F32)

            def h_seg(n, span):
                if "act" not in st:
                    g = jnp.concatenate([gu[0, i] for i in range(F // 128)], axis=1)
                    u = jnp.concatenate([gu[1, i] for i in range(F // 128)], axis=1)
                    act_s[...] = pack(g * jax.nn.sigmoid(g) * u)
                    st["act"] = True
                y_s[:, pl.ds(128 * n, 128)] = mm(act_s[...], wd_s[:, pl.ds(128 * n, 128)], span)

            def do_wait(nm):
                st["toks"] = []
                for c in cp[nm]:
                    c.wait()

            fns = dict(out=lambda lo, hi: ocp(lo, hi).start(), X=x_seg, T=t_task, WS=ws_task, A=a_task, M=m_seg, Q=q_seg, S=s_task, P=p_task, E=e_task, wait=do_wait,
                       perm=permute_w, permo=permute_wo, spec=spec_task, G=g_seg, H=h_seg)
            for item in prog:
                fns[item[0]](*item[1:])
            return st["best"]

        def argmax(best):
            bv, bi = best[:2]
            mx = jnp.max(bv, axis=0, keepdims=True)
            idx = jnp.min(jnp.where(bv >= mx, bi, S - 1), axis=0, keepdims=True)
            return mx[:, 0:1], idx

        def load_chunk(best, nrows):
            idx = argmax(best)[1]
            m, rstd = [jnp.sum(jnp.where(best[1] == idx, t, 0.0), axis=0, keepdims=True)[:, 0:1] for t in best[2:]]
            blk = jnp.clip(idx[0, 0] >> 4, 0, nrows // 16 - 1)
            cur = out_s[pl.ds(pl.multiple_of(blk * 16, 16), 16), :].astype(F32)
            return ((cur - m) * (rstd / (1.0 + rstd))).astype(BF16)

        def fix_row(mx, idx, nrows):
            base = pl.multiple_of(jnp.clip(idx >> 4, 0, nrows // 16 - 1) * 16, 16)
            y = y_s[...] * jax.nn.sigmoid(mx)
            cur = out_s[pl.ds(base, 16), :].astype(F32)
            rows = lax.broadcasted_iota(jnp.int32, (16, D), 0) + base
            out_s[pl.ds(base, 16), :] = jnp.where(rows == idx, cur + y, cur).astype(BF16)
            fix = pltpu.make_async_copy(out_s.at[pl.ds(base, 16)], out_hbm.at[pl.ds(base, 16)], sem_out.at[2])
            fix.start()
            return fix

        def tail(best):
            mx, idx = argmax(best)
            idx = jnp.clip(idx[0, 0], 0, S - 1)
            ocp(0, LATE).wait()

            def early():
                fix = fix_row(mx, idx, LATE)
                ocp(LATE, S).wait()
                fix.wait()

            def late():
                xs = load_chunk(best, S)
                g = jnp.dot(xs, wg_s[...], preferred_element_type=F32)
                u = jnp.dot(xs, wu_s[...], preferred_element_type=F32)
                act = (g * jax.nn.sigmoid(g) * u).astype(BF16)
                y_s[...] = jnp.dot(act, wd_s[...], preferred_element_type=F32)
                ocp(LATE, S).wait()
                fix_row(mx, idx, S).wait()

            lax.cond(idx < LATE, early, late)

        pl.when(pid == 0)(start_all)

        @pl.when(pid == 1)
        def _():
            tail(main())

    @jax.jit
    def fn(A_x, A_wqkv, A_wo, B_x, B_w_r, B_w_gate, B_w_up, B_w_down):
        any_spec = pl.BlockSpec(memory_space=pl.ANY)
        out = pl.pallas_call(
            kernel,
            grid=(2,),
            out_shape=jax.ShapeDtypeStruct((S, D), BF16),
            in_specs=[any_spec] * 7,
            out_specs=any_spec,
            scratch_shapes=[
                pltpu.VMEM((S, D), BF16),
                pltpu.VMEM((D, 3 * D), BF16),
                pltpu.VMEM((NT, D // 2 + 32, 128), U32),
                pltpu.VMEM((D, D), BF16),
                pltpu.VMEM((D,), BF16),
                pltpu.VMEM((D, F), BF16),
                pltpu.VMEM((D, F), BF16),
                pltpu.VMEM((F, D), BF16),
                pltpu.VMEM((D // 2, 4 * D), U32),
                pltpu.VMEM((20 * 128, 256), U32),
                pltpu.VMEM((NS // 2 * 5 * 64, 256), U32),
                pltpu.VMEM((NT, S + HALO, 128), F32),
                pltpu.VMEM((NT, S + HALO, 128), F32),
                pltpu.VMEM((S // 2, D), U32),
                pltpu.VMEM((S // 2, D), U32),
                pltpu.VMEM((S + 16, D), BF16),
                pltpu.VMEM((16, D), F32),
                pltpu.VMEM((8, F), U32),
                pltpu.SemaphoreType.DMA((7,)),
                pltpu.SemaphoreType.DMA((3,)),
            ],
            compiler_params=pltpu.CompilerParams(vmem_limit_bytes=100 << 20,
                                                 dimension_semantics=("arbitrary",),
                                                 disable_bounds_checks=True,
                                                 disable_semaphore_checks=True),
            name="fused",
        )(A_x.reshape(S, D), A_wqkv, A_wo, B_w_r, B_w_gate, B_w_up, B_w_down)
        return out.reshape(1, S, D)

    return fn


pallas_sequential_preLN__sliding_local_dilated__moe_arch_mod__prompt_kernel = make_kernel()
```

```python
import functools
import math
import jax
import jax.numpy as jnp
from jax import lax
import jax.experimental.pallas as pl
import jax.experimental.pallas.tpu as pltpu

S, D, F = 2048, 640, 1536
H, DH, W, DIL = 32, 20, 8, 2
NT = D // 128
HALO = 16
EPS = 1e-5
F32, BF16, U32 = jnp.float32, jnp.bfloat16, jnp.uint32
QSCALE = DH ** -0.5 * math.log2(math.e)
R = 16
T = 128
NS = S // T
NC = T // R
KA = 384
LATE = (NS - 2) * T
XB = 5


PROD = (("s", 0, "t", 0, 2), ("a22", 0, "t", 2, 2), ("s", 2, "b22", 0, 2), ("s7", 4, "t7", 4, 3),
        ("s", 1, "b11", 0, 2), ("bot4", 0, "w4a", 0, 1), ("a11", 0, "t", 1, 2), ("top4", 0, "w4b", 0, 1),
        ("s6", 3, "t6", 3, 3))


def _fold(f, x):
    while x.shape[0] > 1:
        x = f(x[:x.shape[0] // 2], x[x.shape[0] // 2:])
    return x


def _or_all(u):
    u = pltpu.bitcast(u, U32)
    t = None
    for i in range(u.shape[0] // 8):
        for j in range(u.shape[1] // 128):
            p = u[8 * i:8 * i + 8, 128 * j:128 * (j + 1)]
            t = p if t is None else t | p
    return t


def _rows(lo, hi):
    return range(lo, hi, R)


def _io(it):
    k = it[0]
    lhs = lambda g, b, lo=0, hi=T: [("o" if g == 3 else "xn", b, r, j) for r in _rows(lo, hi) for j in range(NT)]
    out = lambda g, b, n, lo=0, hi=T: [("y", g, b, n, r) for r in _rows(lo, hi)]
    if k == "A":
        return [], lhs(0, *it[1:4])
    if k == "M":
        _, g, b, n, lo, hi = it
        return lhs(g, b, lo, hi) + [("w", g, n, 0), ("w", g, n, 1)], out(g, b, n, lo, hi)
    if k == "Q":
        _, b, n, part = it
        return lhs(0, b) + [("w", 0, n, part)], (out(0, b, n) if part else [])
    if k == "X":
        _, ga, na, gb, nb, b, i = it
        done = {3: (ga, b, na), 5: (ga, b + 1, na), 7: (gb, b, nb), 8: (gb, b + 1, nb)}.get(i)
        return ([("t", b, r) for r in _rows(0, T)] + [("ws", ga if ga == gb else 3, r) for r in _rows(0, T)],
                (out(*done) if done else []))
    if k == "T":
        _, b, lo, hi = it
        return lhs(0, b, lo, hi) + lhs(0, b + 1, lo, hi), [("t", b, r) for r in _rows(lo, hi)]
    if k == "WS":
        gs = (0, 1) if it[1] == 3 else (it[1],)
        return ([("w", g, n, p) for g in gs for n in range(NT) for p in (0, 1)],
                [("ws", it[1], r) for r in _rows(*it[2:4])])
    if k == "perm":
        _, g, k0, k1, js = it
        return [], [("w", g, j, p) for j in js for p in (0, 1) if (k0, k1)[p] == (0, D)[p]]
    if k == "permo":
        return [], [("w", 3, it[1], 0), ("w", 3, it[1], 1)]
    if k == "S":
        _, r0, n = it
        b, r = divmod(r0, T)
        return ([("y", g, b, j, r // R * R) for g in (0, 1) for j in range(NT)],
                [("sm", r0 + i) for i in range(0, n, 8)])
    if k == "P":
        _, b, c, j = it
        return ([("sm", b * T + c * R + r) for r in range(0, R, 8)] + [("y", 2, b, jj, c * R) for jj in range(NT)],
                [("o", b, c * R, j)])
    if k == "E":
        _, b, lo, hi = it
        prev = [("e", b * T + lo - R)] if b * T + lo else []
        return ([("y", 3, b, n, r) for n in range(NT) for r in _rows(lo, hi)] + prev,
                [("e", b * T + r) for r in _rows(lo, hi)])
    if k == "spec":
        return [("e", LATE - R)], [("spec",)]
    if k == "G":
        return [("spec",)], [("g",) + it[1:]]
    if k == "H":
        return [("g", kk, n) for kk in range(2) for n in range(F // 128)], []
    return [], []


def _slots(it):
    k = it[0]
    if k == "M":
        return (it[5] - it[4]) / 16
    if k == "Q":
        return 1.6 * (3, 2)[it[3]]
    if k == "X":
        return 1.6 * PROD[it[6]][4]
    return {"G": 0.0, "H": 1.0}[k]


class Plan:
    def __init__(self):
        self.prog, self.pos, self.have, self.todo = [], 0.0, set(), []

    def _put(self, it, extra):
        self.prog.append(it + (extra,))
        self.have.update(_io(it)[1])

    def _emit_task(self, t, force=False):
        due, it = t
        for key in _io(it)[0]:
            if key not in self.have:
                src = [u for u in self.todo if key in _io(u[1])[1]]
                if not src or not self._emit_task(src[0], force):
                    assert not force, ("unsatisfied", it, key)
                    return False
        self.todo.remove(t)
        self._put(it, due)
        return True

    def tasks(self, ts):
        self.todo += [(None if d is None else self.pos + d, it) for d, it in ts]

    def due(self, end):
        for t in sorted([t for t in self.todo if t[0] is not None and t[0] < end], key=lambda t: t[0]):
            if t in self.todo:
                self._emit_task(t)

    def mxu(self, segs):
        for sg in segs:
            end = self.pos + _slots(sg)
            self.due(end)
            for key in _io(sg)[0]:
                if key not in self.have:
                    src = [u for u in self.todo if key in _io(u[1])[1]]
                    assert src, ("unsatisfied", sg, key)
                    self._emit_task(src[0], True)
            self._put(sg, (self.pos, end))
            self.pos = end

    def flush(self, pred=lambda it: True):
        for t in [t for t in self.todo if pred(t[1])]:
            if t in self.todo:
                self._emit_task(t, True)

    def wait(self, *names):
        self.prog += [("wait", n) for n in names]


def build_program(o):
    M = lambda g, b, lo=0, hi=T: [("M", g, b, n, lo, hi) for n in range(NT)]
    Q = lambda b, part: [("Q", b, n, part) for n in range(NT)]

    def parts(kind, b, dls):
        n = T // len(dls)
        return [(dl, (kind, b, i * n, (i + 1) * n)) for i, dl in enumerate(dls)]

    def LS(b, c0, cp, rl=R):
        t = []
        for c in range(NC):
            for h in range(0, R, rl):
                r0 = b * T + c * R + h
                t += [(None if c0 is None else c0 + cp * c - (R - rl - h) * cp / R, ("S", r0, rl))]
        return t

    def Pt(b, c0, cp):
        return [(None if c0 is None else c0 + cp * c + o["ps"] * j, ("P", b, c, j))
                for c in range(NC) for j in range(NT)]

    def C(b, c0, cp):
        return LS(b, c0, cp, o["rl"]) + Pt(b, c0 + o["po"], cp)

    def WS(g, d):
        return [(None if d is None else d - 5 * (3 - i), ("WS", g, 32 * i, 32 * i + 32)) for i in range(4)]

    def X(ga, na, gb, nb, b):
        return [("X", ga, na, gb, nb, b, i) for i in range(len(PROD))]

    sh = lambda ts, d: [(None if t is None else t + d, it) for t, it in ts]
    allj = tuple(range(NT))
    p = Plan()
    p.wait("x0a")
    p.tasks(parts("A", 0, (None,)) + parts("A", 1, (None,)))
    p.flush()
    p.wait("wqa")
    p.tasks([(None, ("perm", 0, 0, KA, allj))])
    p.mxu(Q(0, 0))
    p.wait("x0b", "wqb")
    p.tasks([(None, ("perm", 0, KA, D, allj))] + parts("A", 2, (None,)))
    p.flush()
    p.tasks(WS(0, o["ws"][0]))
    p.mxu(Q(1, 0) + Q(0, 1) + Q(1, 1) + Q(2, 0))
    p.flush()
    p.wait("wk")
    p.tasks([(None, ("perm", 1, 0, D, (j,))) for j in range(NT)] + LS(0, None, 0) + WS(1, o["ws"][1]))
    p.mxu(Q(2, 1) + M(1, 0) + M(1, 1))
    p.flush()
    p.wait("wv")
    p.tasks([(o["pv"][0] + o["pv"][1] * j, ("perm", 2, 0, D, (j,))) for j in range(NT)]
            + LS(1, *o["l1"]) + Pt(0, *o["p0"]) + WS(2, o["ws"][2]))
    p.mxu(M(1, 2) + M(2, 0) + M(2, 1))
    p.flush()
    p.wait("wo", "wr", "x1")
    p.tasks([(None, ("permo", n)) for n in range(NT)])
    p.tasks(Pt(1, *o["p1"]) + parts("A", 3, o["a3"]) + parts("A", 4, o["a4"]) + parts("E", 0, o["e0"])
            + [(None, ("T", 3, 0, T)), (None, ("WS", 3, 0, T))])
    p.mxu(M(2, 2) + M(3, 0))
    for b in range(1, NS - 4, 2):
        nb = b + 2
        qk = X(0, 0, 0, 2, nb) + X(0, 1, 0, 3, nb) + X(0, 4, 1, 4, nb) + X(1, 0, 1, 2, nb) + X(1, 1, 1, 3, nb)
        v = X(2, 0, 2, 2, nb) + M(2, nb)[4:] + X(2, 1, 2, 3, nb) + M(2, nb + 1)[4:]
        segs = (M(3, b - 1) + qk + M(3, b) if b > 1 else M(3, b) + qk) + v
        e1, e2, a1, a2, p1, c2, l1 = [o["per"][b][i:i + 2] for i in range(0, 14, 2)]
        tasks = parts("E", b - 1, e1) + Pt(b, *p1) if b > 1 else []
        tasks += parts("E", b, e2) + C(b + 1, *c2) + parts("A", b + 4, a1)
        if b + 5 < NS:
            tasks += parts("A", b + 5, a2) + parts("T", b + 4, (None, None))
            tasks += sh(LS(b + 2, *l1, o["rl"]), sum(_slots(sg) for sg in segs) - 60)
        else:
            tasks += LS(b + 2, *o["l13"], o["rl"])
        if b == XB:
            late = [t for t in tasks if t[1][0] in "AT"]
            p.tasks([t for t in tasks if t not in late])
            base = p.pos
            p.mxu(segs[:o["xp"]])
            p.due(p.pos + o["xl"])
            p.flush(lambda it: it[0] in "AT" or it[0] == "E" and it[1] < XB - 1)
            assert ("e", (XB - 1) * T - R) in p.have
            p.wait("x2", "ffn")
            p.prog.append(("out", 0, (XB - 1) * T))
            p.tasks(sh(late, base - p.pos))
            p.mxu(segs[o["xp"]:])
        else:
            p.tasks(tasks)
            p.mxu(segs)
    p.tasks(Pt(NS - 3, *o["p13"]) + parts("E", NS - 4, o["e12"]))
    p.mxu(M(3, NS - 4))
    s = NS - 2
    big = M(3, s - 1) + M(0, s + 1) + M(1, s + 1) + M(3, s) + M(2, s + 1)
    small = [("G", k, n) for n in range(F // 128) for k in range(2)]
    cut = o["cut"]
    segs = []
    n_big, n_small, done = len(big) - o["sp"], len(small) - o["gh"], 0
    for g, sg in enumerate(big):
        segs.append(sg)
        if g >= o["sp"]:
            want = min(n_small, -(-(g - o["sp"] + 1) * n_small // n_big))
            segs += small[done:want]
            done = want
    segs += small[done:] + M(3, s + 1, 0, cut) + M(3, s + 1, cut, T) + [("H", n) for n in range(NT)]
    p.tasks(parts("E", s - 1, o["e13"]) + [(None, ("spec",))] + C(s, *o["c14"])
            + LS(s + 1, *o["l15"]) + Pt(s + 1, None, 0) + parts("E", s, o["e14"])
            + [(o["e15"], ("E", s + 1, 0, cut)), (None, ("E", s + 1, cut, T))])
    p.mxu(segs)
    p.flush()
    return p.prog


SCHED = dict(
    rl=8, ps=3, po=2, fq=16, ws=(50, 60, None), pv=(25, 14), l1=(56, 12), p0=(86, 3.25),
    p1=(42, 5.0), a3=(45,), a4=(82,), e0=(148, 180), xp=14, xl=32,
    per={1: (0, 0, 270, 298, 140, 169, 187, 217, 0, 0, 32, 27.0, 80, 19.0),
         3: (80, 112, 266, 308, 140, 177, 187, 217, 22, 18.5, 168, 16.5, 80, 19.0),
         5: (80, 112, 254, 308, 140, 173, 187, 217, 18, 19.0, 160, 16.0, 80, 19.0),
         7: (80, 112, 262, 308, 140, 167, 187, 217, 10, 20.0, 160, 16.0, 80, 19.0),
         9: (80, 112, 278, 308, 140, 167, 191, 229, 18, 19.0, 168, 16.0, 72, 18.25),
         11: (82, 112, 272, 308, 140, 169, 195, 215, 22, 19.0, 168, 16.0, 80, 19.0)},
    l13=(231, 9.0), p13=(8, 5.0), e12=(72, 100),
    cut=64, sp=12, gh=6, e13=(89, 106), c14=(2, 12.75), l15=(156, 4.5), e14=(202, 217), e15=243)


def make_kernel():
    o = SCHED
    prog = build_program(o)
    x1 = (XB + 1) * T
    xch = (2 * T, T, x1, S - 3 * T - x1)

    def kernel(x_hbm, wqkv_hbm, wo_hbm, wr_hbm, wg_hbm, wu_hbm, wd_hbm, out_hbm,
               x_s, wqkv_s, wo_s, wob_s, wr_s, wg_s, wu_s, wd_s, wp_s, ws_s, ts_s,
               k_s, v_s, xn_s, o_s, out_s, y_s, act_s, sem_in, sem_out):
        pid = pl.program_id(0)
        step = pid - 1
        cp = {}
        semi = dict(x0a=0, wqa=1, x0b=6, wqb=6, wk=2, wv=3, wo=4, wr=4, x1=4, x2=5, ffn=5)
        r0 = 0
        for nm, n in zip(("x0a", "x0b", "x1", "x2"), xch):
            cp[nm] = [pltpu.make_async_copy(x_hbm.at[pl.ds(r0, n)], x_s.at[pl.ds(r0, n)], sem_in.at[semi[nm]])]
            r0 += n
        for nm, lo, hi, g in (("wqa", 0, KA, 0), ("wqb", KA, D, 0), ("wk", 0, D, 1), ("wv", 0, D, 2)):
            sl = (pl.ds(lo, hi - lo), pl.ds(D * g, D))
            cp[nm] = [pltpu.make_async_copy(wqkv_hbm.at[sl], wqkv_s.at[sl], sem_in.at[semi[nm]])]
        cp["wo"] = [pltpu.make_async_copy(wo_hbm, wob_s, sem_in.at[semi["wo"]])]
        cp["wr"] = [pltpu.make_async_copy(wr_hbm, wr_s, sem_in.at[semi["wr"]])]
        cp["ffn"] = [pltpu.make_async_copy(a, b, sem_in.at[semi["ffn"]])
                     for a, b in ((wg_hbm, wg_s), (wu_hbm, wu_s), (wd_hbm, wd_s))]

        def ocp(lo, hi):
            return pltpu.make_async_copy(out_s.at[pl.ds(lo, hi - lo)], out_hbm.at[pl.ds(lo, hi - lo)],
                                         sem_out.at[0 if lo < LATE else 1])

        def start_all():
            for nm in ("x0a", "wqa", "x0b", "wqb", "wk", "wv", "wo", "wr", "x1", "x2", "ffn"):
                for c in cp[nm]:
                    c.start()

        def main():
            zero = jnp.zeros((HALO, 128), F32)
            for j in range(NT):
                k_s[j, 0:HALO, :] = zero
                v_s[j, 0:HALO, :] = zero

            lane = lax.broadcasted_iota(jnp.int32, (1, 128), 1)
            cm5 = [(lane + 128 * t) - 5 * (((lane + 128 * t) * 52429) >> 18) for t in range(NT - 1)]
            srcs = [(20 * (lane & 31) + 5 * (lane >> 5) + j) & 127 for j in range(NT)]
            never = jnp.full((8, 128), step, jnp.int32) > 0
            st = dict(best=None, toks=[], wr=None)
            q, hh, sm, gu, part = {}, {}, {}, {}, {}
            pack = lambda v: pltpu.bitcast(v.astype(BF16), U32)
            rsqrt = lambda v: jnp.exp2(jnp.log(v) * (-0.5 / math.log(2.0)))

            def token(due, u):
                if due is not None:
                    st["toks"].append((due, u()))

            def mm(lhs, w, span):
                start, end = span
                toks = [t for t in st["toks"] if t[0] < end]
                st["toks"] = [t for t in st["toks"] if t[0] >= end]
                if toks:
                    ng = lhs.shape[0] // 8
                    grp = lambda d: min(max(int(d - start), 0), ng - 1)
                    col, pos = [], 0
                    for i in sorted({grp(d) for d, _ in toks}):
                        tok = functools.reduce(jnp.bitwise_or, [t for d, t in toks if grp(d) == i])
                        col += [lhs[pos:8 * i, 0:128]] if 8 * i > pos else []
                        col.append(jnp.where(never, tok, lhs[8 * i:8 * i + 8, 0:128]))
                        pos = 8 * i + 8
                    col += [lhs[pos:, 0:128]] if pos < 8 * ng else []
                    col = jnp.concatenate(col, axis=0)
                    lhs = jnp.concatenate([col, lhs[:, 128:]], axis=1) if lhs.shape[1] > 128 else col
                if w.dtype == U32:
                    w = pltpu.bitcast(w, BF16)
                return jnp.dot(pltpu.bitcast(lhs, BF16), w, preferred_element_type=F32)

            def permute_w(g, k0, k1, js, due):
                if ("mw", g, k0) not in st:
                    tiles = [pltpu.bitcast(wqkv_s[pl.ds(k0, k1 - k0), pl.ds(D * g + 128 * t, 128)], U32)
                             for t in range(NT)]
                    st["mw", g, k0] = []
                    for j in range(NT):
                        m = tiles[NT - 1]
                        for t in range(NT - 2, -1, -1):
                            m = jnp.where(cm5[t] == j, tiles[t], m)
                        st["mw", g, k0].append(m)
                for j in js:
                    m = st["mw", g, k0][j]
                    res = jnp.take_along_axis(m, jnp.broadcast_to(srcs[j], m.shape), axis=1,
                                              mode="promise_in_bounds")
                    wp_s[pl.ds(k0 // 2, (k1 - k0) // 2), pl.ds(D * g + 128 * j, 128)] = res
                    token(due, lambda: _or_all(res))

            def permute_wo(n, due):
                wo_s[n, pl.ds(0, D // 2), :] = pltpu.bitcast(wob_s[:, pl.ds(128 * n, 128)], U32)
                for d2 in range(DH // 2):
                    ev = wo_s[n, pl.ds(d2, H // 2, stride=DH), :]
                    od = wo_s[n, pl.ds(DH // 2 + d2, H // 2, stride=DH), :]
                    lo = (ev & jnp.uint32(0xFFFF)) | (od << 16)
                    hi = (ev >> 16) | (od & jnp.uint32(0xFFFF0000))
                    for d, val in ((2 * d2, lo), (2 * d2 + 1, hi)):
                        aa, j = divmod(d, NT)
                        wp_s[pl.ds(64 * j + 16 * aa, H // 2), pl.ds(3 * D + 128 * n, 128)] = val

            def sums(blocks, combos):
                un = [pltpu.bitcast(u, BF16).astype(F32) for u in blocks]
                return [pack(un[x] + un[y] if sg > 0 else un[x] - un[y]) for x, sg, y in combos]

            def ws_task(g, lo, hi, due):
                cols = [pl.ds(D * j + 512, 128) if g == 3 else pl.ds(D * g + 256 * j, 256) for j in range(2)]
                b = [wp_s[pl.ds(128 * i + lo, hi - lo), cols[j]] for i in range(2) for j in range(2)]
                res = sums(b, ((0, 1, 3), (1, -1, 3), (2, -1, 0), (0, 1, 1), (2, 1, 3)))
                dst = lambda i: (pl.ds((5 * g + i) * 128 + lo, hi - lo), pl.ds(0, 128 if g == 3 else 256))
                for i, v in enumerate(res):
                    ws_s[dst(i)] = v
                token(due, lambda: _or_all(jnp.concatenate([ws_s[dst(i)] for i in range(5)], axis=0)))

            def t_task(b, lo, hi, due):
                a = [xn_s[pl.ds(((b + i) * T + lo) // 2, (hi - lo) // 2), pl.ds(256 * j, 256)]
                     for i in range(2) for j in range(2)]
                for i, v in enumerate(sums(a, ((0, 1, 3), (2, 1, 3), (0, 1, 1), (2, -1, 0), (1, -1, 3)))):
                    ts_s[pl.ds((5 * (b // 2) + i) * 64 + lo // 2, (hi - lo) // 2), :] = v

            def a_task(b, lo, hi, due):
                r0, n = b * T + lo, hi - lo
                x = x_s[pl.ds(r0, n), :].astype(F32)
                m = jnp.sum(x, axis=-1, keepdims=True) * (1.0 / D)
                c = x - m
                v = jnp.sum(c * c, axis=-1, keepdims=True) * (1.0 / D)
                xn_s[pl.ds(r0 // 2, n // 2), :] = pack(c * rsqrt(v + EPS))
                token(due, lambda: _or_all(xn_s[pl.ds(r0 // 2, n // 2), :]))

            def finish(g, b, n, lo, hi, acc, due):
                r0 = b * T + lo
                if g == 0:
                    acc = acc * QSCALE
                elif g == 3:
                    acc = acc + x_s[pl.ds(r0, hi - lo), pl.ds(128 * n, 128)].astype(F32)
                token(due, lambda: _or_all(acc))
                if g == 0:
                    q[b, n] = acc
                elif g == 3:
                    hh[b, n, lo, hi] = acc
                else:
                    (k_s if g == 1 else v_s)[n, pl.ds(HALO + r0, hi - lo), :] = acc

            def m_seg(g, b, n, lo, hi, span):
                src = o_s if g == 3 else xn_s
                acc = mm(src[pl.ds((b * T + lo) // 2, (hi - lo) // 2), :],
                         wp_s[:, pl.ds(D * g + 128 * n, 128)], span)
                finish(g, b, n, lo, hi, acc, span[1] + o["fq"] if g == 0 else None)

            def q_seg(b, n, kpart, span):
                k0, k1 = ((0, KA), (KA, D))[kpart]
                acc = mm(xn_s[pl.ds(b * T // 2, T // 2), pl.ds(k0, k1 - k0)],
                         wp_s[pl.ds(k0 // 2, (k1 - k0) // 2), pl.ds(128 * n, 128)], span)
                if kpart == 0:
                    part[b, n] = acc
                else:
                    finish(0, b, n, 0, T, acc + part.pop((b, n)), None)

            def x_seg(ga, na, gb, nb, b, i, span):
                blk = lambda bb, c0, w: xn_s[pl.ds(bb * T // 2, T // 2), pl.ds(c0, w)]
                ca, cb = D * ga + 128 * na, D * gb + 128 * nb
                wb = lambda r, c: wp_s[pl.ds(r, 128 if r < 256 else 64), pl.ds(c, 128)]
                ln, li, rn, ri, _ = PROD[i]
                ss = lambda: ts_s[pl.ds((5 * (b // 2) + li) * 64, 64), :]
                wg, wn = (ga, na) if ga == gb else (3, 0)
                tt = lambda: ws_s[pl.ds((5 * wg + ri) * 128, 128), pl.ds(128 * wn, 128)]
                lhs = {"s": ss, "a11": lambda: blk(b, 0, 256), "a22": lambda: blk(b + 1, 256, 256),
                       "top4": lambda: blk(b, 512, 128), "bot4": lambda: blk(b + 1, 512, 128),
                       "s7": lambda: jnp.concatenate([ss(), blk(b, 512, 128)], axis=1),
                       "s6": lambda: jnp.concatenate([ss(), blk(b + 1, 512, 128)], axis=1)}[ln]()
                rhs = {"t": tt, "b11": lambda: wb(0, ca), "b22": lambda: wb(128, cb),
                       "w4a": lambda: wb(256, ca), "w4b": lambda: wb(256, cb),
                       "t7": lambda: jnp.concatenate([tt(), wb(256, ca)], axis=0),
                       "t6": lambda: jnp.concatenate([tt(), wb(256, cb)], axis=0)}[rn]()
                m = mm(lhs, rhs, span)
                due = lambda g: span[1] + o["fq"] if g == 0 else None
                c = part.setdefault((ga, na, b), {})
                if i == 0:
                    c[11] = c[22] = m
                elif i == 1:
                    c[11], c[21] = c[11] + m, m
                elif i == 2:
                    c[11], c[12] = c[11] - m, m
                elif i == 3:
                    finish(ga, b, na, 0, T, c.pop(11) + m, due(ga))
                elif i == 4:
                    c[21], c[22] = c[21] + m, c[22] - m
                elif i == 5:
                    finish(ga, b + 1, na, 0, T, c.pop(21) + m, due(ga))
                elif i == 6:
                    c[12], c[22] = c[12] + m, c[22] + m
                elif i == 7:
                    finish(gb, b, nb, 0, T, c.pop(12) + m, due(gb))
                else:
                    finish(gb, b + 1, nb, 0, T, c.pop(22) + m, due(gb))

            def s_task(r0, n, due):
                b, r = divmod(r0, T)
                qc = jnp.stack([q[b, j][r:r + n] for j in range(NT)])
                lg = jnp.stack([jnp.sum(qc * k_s[:, pl.ds(HALO + r0 - DIL * w, n), :], axis=0)
                                for w in range(W)])
                lg = lg + pltpu.roll(lg, 64, 2)
                lg = lg + pltpu.roll(lg, 32, 2)
                if r0 < DIL * (W - 1):
                    pos = (lax.broadcasted_iota(jnp.int32, lg.shape, 1) + r0
                           - DIL * lax.broadcasted_iota(jnp.int32, lg.shape, 0))
                    lg = jnp.where(pos >= 0, lg, -1e9)
                e = jnp.exp2(lg - _fold(jnp.maximum, lg))
                inv = pl.reciprocal(_fold(jnp.add, e), approx=True)
                sm[r0] = (e, inv)
                token(due, lambda: _or_all(inv[0]))

            def p_task(b, c, j, due):
                r0 = b * T + c * R
                if ("pv", r0) not in st:
                    e, inv = sm.pop(r0)
                    if r0 + 8 in sm:
                        e2, inv2 = sm.pop(r0 + 8)
                        e, inv = jnp.concatenate([e, e2], axis=1), jnp.concatenate([inv, inv2], axis=1)
                    acc = None
                    for w in range(W):
                        t = e[w:w + 1] * v_s[:, pl.ds(HALO + r0 - DIL * w, R), :]
                        acc = t if acc is None else acc + t
                    st["pv", r0] = acc * inv
                dst = (pl.ds(r0 // 2, R // 2), pl.ds(128 * j, 128))
                o_s[dst] = pack(st["pv", r0][j])
                token(due, lambda: o_s[dst])

            def e_task(b, lo, hi, due):
                r0, n = b * T + lo, hi - lo
                if st["wr"] is None:
                    st["wr"] = wr_s[...].astype(F32).reshape(1, D)
                (l0, h0), = {k[2:] for k in hh if k[0] == b and k[2] <= lo and hi <= k[3]}
                h = jnp.concatenate([hh[b, j, l0, h0][lo - l0:hi - l0] for j in range(NT)], axis=1)
                m = jnp.sum(h, axis=-1, keepdims=True) * (1.0 / D)
                c = h - m
                v = jnp.sum(c * c, axis=-1, keepdims=True) * (1.0 / D)
                cw = jnp.sum(c * st["wr"], axis=-1, keepdims=True)
                rstd = rsqrt(v + EPS)
                hn = c * rstd
                out_s[pl.ds(pl.multiple_of(step * 16 + r0, 16), n), :] = (h + hn).astype(BF16)
                r, mb, rb = [jnp.broadcast_to(t, (n, 128)) for t in (cw * rstd, m, rstd)]
                best = st["best"]
                for i in range(n // 8):
                    ri = r[8 * i:8 * i + 8]
                    new = (ri, lax.broadcasted_iota(jnp.int32, (8, 128), 0) + (r0 + 8 * i),
                           mb[8 * i:8 * i + 8], rb[8 * i:8 * i + 8])
                    if best is None:
                        best = (jnp.where(ri > -jnp.inf, ri, -jnp.inf),) + new[1:]
                    else:
                        upd = ri > best[0]
                        best = tuple(jnp.where(upd, a, c_) for a, c_ in zip(new, best))
                st["best"] = best
                if b == NS - 1:
                    ocp(r0, r0 + n).start()
                elif hi == T and b >= XB - 1:
                    ocp(b * T, (b + 1) * T).start()
                token(due, lambda: functools.reduce(jnp.bitwise_or, [pltpu.bitcast(t, U32) for t in best])
                      | pltpu.bitcast(out_s[0:16, 0:128], U32))

            def spec_task(due):
                st["xs"] = load_chunk(st["best"], LATE)

            def g_seg(k, n, span):
                gu[k, n] = jnp.dot(st["xs"], (wg_s, wu_s)[k][:, pl.ds(128 * n, 128)],
                                   preferred_element_type=F32)

            def h_seg(n, span):
                if "act" not in st:
                    g = jnp.concatenate([gu[0, i] for i in range(F // 128)], axis=1)
                    u = jnp.concatenate([gu[1, i] for i in range(F // 128)], axis=1)
                    act_s[...] = pack(g * jax.nn.sigmoid(g) * u)
                    st["act"] = True
                y_s[:, pl.ds(128 * n, 128)] = mm(act_s[...], wd_s[:, pl.ds(128 * n, 128)], span)

            def do_wait(nm):
                st["toks"] = []
                for c in cp[nm]:
                    c.wait()

            fns = dict(A=a_task, T=t_task, WS=ws_task, M=m_seg, Q=q_seg, X=x_seg, S=s_task, P=p_task,
                       E=e_task, perm=permute_w, permo=permute_wo, spec=spec_task, G=g_seg, H=h_seg,
                       wait=do_wait, out=lambda lo, hi: ocp(lo, hi).start())
            for item in prog:
                fns[item[0]](*item[1:])
            return st["best"]

        def argmax(best):
            bv, bi = best[:2]
            mx = jnp.max(bv, axis=0, keepdims=True)
            idx = jnp.min(jnp.where(bv >= mx, bi, S - 1), axis=0, keepdims=True)
            return mx[:, 0:1], idx

        def load_chunk(best, nrows):
            idx = argmax(best)[1]
            m, rstd = [jnp.sum(jnp.where(best[1] == idx, t, 0.0), axis=0, keepdims=True)[:, 0:1] for t in best[2:]]
            blk = jnp.clip(idx[0, 0] >> 4, 0, nrows // 16 - 1)
            cur = out_s[pl.ds(pl.multiple_of(blk * 16, 16), 16), :].astype(F32)
            return ((cur - m) * (rstd / (1.0 + rstd))).astype(BF16)

        def fix_row(mx, idx, nrows):
            base = pl.multiple_of(jnp.clip(idx >> 4, 0, nrows // 16 - 1) * 16, 16)
            y = y_s[...] * jax.nn.sigmoid(mx)
            cur = out_s[pl.ds(base, 16), :].astype(F32)
            rows = lax.broadcasted_iota(jnp.int32, (16, D), 0) + base
            out_s[pl.ds(base, 16), :] = jnp.where(rows == idx, cur + y, cur).astype(BF16)
            fix = pltpu.make_async_copy(out_s.at[pl.ds(base, 16)], out_hbm.at[pl.ds(base, 16)], sem_out.at[2])
            fix.start()
            return fix

        def tail(best):
            mx, idx = argmax(best)
            idx = jnp.clip(idx[0, 0], 0, S - 1)
            ocp(0, LATE).wait()

            def early():
                fix = fix_row(mx, idx, LATE)
                ocp(LATE, S).wait()
                fix.wait()

            def late():
                xs = load_chunk(best, S)
                g = jnp.dot(xs, wg_s[...], preferred_element_type=F32)
                u = jnp.dot(xs, wu_s[...], preferred_element_type=F32)
                act = (g * jax.nn.sigmoid(g) * u).astype(BF16)
                y_s[...] = jnp.dot(act, wd_s[...], preferred_element_type=F32)
                ocp(LATE, S).wait()
                fix_row(mx, idx, S).wait()

            lax.cond(idx < LATE, early, late)

        pl.when(pid == 0)(start_all)

        @pl.when(pid == 1)
        def _():
            tail(main())

    @jax.jit
    def fn(A_x, A_wqkv, A_wo, B_x, B_w_r, B_w_gate, B_w_up, B_w_down):
        any_spec = pl.BlockSpec(memory_space=pl.ANY)
        out = pl.pallas_call(
            kernel,
            grid=(2,),
            out_shape=jax.ShapeDtypeStruct((S, D), BF16),
            in_specs=[any_spec] * 7,
            out_specs=any_spec,
            scratch_shapes=[
                pltpu.VMEM((S, D), BF16),
                pltpu.VMEM((D, 3 * D), BF16),
                pltpu.VMEM((NT, D // 2 + 32, 128), U32),
                pltpu.VMEM((D, D), BF16),
                pltpu.VMEM((D,), BF16),
                pltpu.VMEM((D, F), BF16),
                pltpu.VMEM((D, F), BF16),
                pltpu.VMEM((F, D), BF16),
                pltpu.VMEM((D // 2, 4 * D), U32),
                pltpu.VMEM((20 * 128, 256), U32),
                pltpu.VMEM((NS // 2 * 5 * 64, 256), U32),
                pltpu.VMEM((NT, S + HALO, 128), F32),
                pltpu.VMEM((NT, S + HALO, 128), F32),
                pltpu.VMEM((S // 2, D), U32),
                pltpu.VMEM((S // 2, D), U32),
                pltpu.VMEM((S + 16, D), BF16),
                pltpu.VMEM((16, D), F32),
                pltpu.VMEM((8, F), U32),
                pltpu.SemaphoreType.DMA((7,)),
                pltpu.SemaphoreType.DMA((3,)),
            ],
            compiler_params=pltpu.CompilerParams(vmem_limit_bytes=100 << 20,
                                                 dimension_semantics=("arbitrary",),
                                                 disable_bounds_checks=True,
                                                 disable_semaphore_checks=True),
            name="fused",
        )(A_x.reshape(S, D), A_wqkv, A_wo, B_w_r, B_w_gate, B_w_up, B_w_down)
        return out.reshape(1, S, D)

    return fn


pallas_sequential_preLN__sliding_local_dilated__moe_arch_mod__prompt_kernel = make_kernel()
```

```python
import functools
import math
import jax
import jax.numpy as jnp
from jax import lax
import jax.experimental.pallas as pl
import jax.experimental.pallas.tpu as pltpu

S, D, F = 2048, 640, 1536
H, DH, W, DIL = 32, 20, 8, 2
NT = D // 128
HALO = 16
EPS = 1e-5
F32, BF16, U32 = jnp.float32, jnp.bfloat16, jnp.uint32
QSCALE = DH ** -0.5 * math.log2(math.e)
R = 16
T = 128
NS = S // T
NC = T // R
KA = 384
LATE = (NS - 2) * T
XB = 5


PROD = (("s", 0, "t", 0, 2), ("a22", 0, "t", 2, 2), ("s", 2, "b22", 0, 2), ("s7", 4, "t7", 4, 3),
        ("s", 1, "b11", 0, 2), ("bot4", 0, "w4a", 0, 1), ("a11", 0, "t", 1, 2), ("top4", 0, "w4b", 0, 1),
        ("s6", 3, "t6", 3, 3))


def _fold(f, x):
    while x.shape[0] > 1:
        x = f(x[:x.shape[0] // 2], x[x.shape[0] // 2:])
    return x


def _or_all(u):
    u = pltpu.bitcast(u, U32)
    t = None
    for i in range(u.shape[0] // 8):
        for j in range(u.shape[1] // 128):
            p = u[8 * i:8 * i + 8, 128 * j:128 * (j + 1)]
            t = p if t is None else t | p
    return t


def _rows(lo, hi):
    return range(lo, hi, R)


def _io(it):
    k = it[0]
    lhs = lambda g, b, lo=0, hi=T: [("o" if g == 3 else "xn", b, r, j) for r in _rows(lo, hi) for j in range(NT)]
    out = lambda g, b, n, lo=0, hi=T: [("y", g, b, n, r) for r in _rows(lo, hi)]
    if k == "A":
        return [], lhs(0, *it[1:4])
    if k == "M":
        _, g, b, n, lo, hi = it
        return lhs(g, b, lo, hi) + [("w", g, n, 0), ("w", g, n, 1)], out(g, b, n, lo, hi)
    if k == "Q":
        _, b, n, part = it
        return lhs(0, b) + [("w", 0, n, part)], (out(0, b, n) if part else [])
    if k == "X":
        _, ga, na, gb, nb, b, i = it
        done = {3: (ga, b, na), 5: (ga, b + 1, na), 7: (gb, b, nb), 8: (gb, b + 1, nb)}.get(i)
        return ([("t", b, r) for r in _rows(0, T)] + [("ws", ga if ga == gb else 3, r) for r in _rows(0, T)],
                (out(*done) if done else []))
    if k == "T":
        _, b, lo, hi = it
        return lhs(0, b, lo, hi) + lhs(0, b + 1, lo, hi), [("t", b, r) for r in _rows(lo, hi)]
    if k == "WS":
        gs = (0, 1) if it[1] == 3 else (it[1],)
        return ([("w", g, n, p) for g in gs for n in range(NT) for p in (0, 1)],
                [("ws", it[1], r) for r in _rows(*it[2:4])])
    if k == "perm":
        _, g, k0, k1, js = it
        return [], [("w", g, j, p) for j in js for p in (0, 1) if (k0, k1)[p] == (0, D)[p]]
    if k == "permo":
        return [], [("w", 3, it[1], 0), ("w", 3, it[1], 1)]
    if k == "S":
        _, r0, n = it
        b, r = divmod(r0, T)
        return ([("y", g, b, j, r // R * R) for g in (0, 1) for j in range(NT)],
                [("sm", r0 + i) for i in range(0, n, 8)])
    if k == "P":
        _, b, c, j = it
        return ([("sm", b * T + c * R + r) for r in range(0, R, 8)] + [("y", 2, b, jj, c * R) for jj in range(NT)],
                [("o", b, c * R, j)])
    if k == "E":
        _, b, lo, hi = it
        prev = [("e", b * T + lo - R)] if b * T + lo else []
        return ([("y", 3, b, n, r) for n in range(NT) for r in _rows(lo, hi)] + prev,
                [("e", b * T + r) for r in _rows(lo, hi)])
    if k == "spec":
        return [("e", LATE - R)], [("spec",)]
    if k == "G":
        return [("spec",)], [("g",) + it[1:]]
    if k == "H":
        return [("g", kk, n) for kk in range(2) for n in range(F // 128)], []
    return [], []


def _slots(it):
    k = it[0]
    if k == "M":
        return (it[5] - it[4]) / 16
    if k == "Q":
        return 1.6 * (3, 2)[it[3]]
    if k == "X":
        return 1.6 * PROD[it[6]][4]
    return {"G": 0.0, "H": 1.0}[k]


class Plan:
    def __init__(self):
        self.prog, self.pos, self.have, self.todo = [], 0.0, set(), []

    def _put(self, it, extra):
        self.prog.append(it + (extra,))
        self.have.update(_io(it)[1])

    def _emit_task(self, t, force=False):
        due, it = t
        for key in _io(it)[0]:
            if key not in self.have:
                src = [u for u in self.todo if key in _io(u[1])[1]]
                if not src or not self._emit_task(src[0], force):
                    assert not force, ("unsatisfied", it, key)
                    return False
        self.todo.remove(t)
        self._put(it, due)
        return True

    def tasks(self, ts):
        self.todo += [(None if d is None else self.pos + d, it) for d, it in ts]

    def due(self, end):
        for t in sorted([t for t in self.todo if t[0] is not None and t[0] < end], key=lambda t: t[0]):
            if t in self.todo:
                self._emit_task(t)

    def mxu(self, segs):
        for sg in segs:
            end = self.pos + _slots(sg)
            self.due(end)
            for key in _io(sg)[0]:
                if key not in self.have:
                    src = [u for u in self.todo if key in _io(u[1])[1]]
                    assert src, ("unsatisfied", sg, key)
                    self._emit_task(src[0], True)
            self._put(sg, (self.pos, end))
            self.pos = end

    def flush(self, pred=lambda it: True):
        for t in [t for t in self.todo if pred(t[1])]:
            if t in self.todo:
                self._emit_task(t, True)

    def wait(self, *names):
        self.prog += [("wait", n) for n in names]


def build_program(o):
    M = lambda g, b, lo=0, hi=T: [("M", g, b, n, lo, hi) for n in range(NT)]
    Q = lambda b, part: [("Q", b, n, part) for n in range(NT)]

    def parts(kind, b, dls):
        n = T // len(dls)
        return [(dl, (kind, b, i * n, (i + 1) * n)) for i, dl in enumerate(dls)]

    def LS(b, c0, cp, rl=R):
        t = []
        for c in range(NC):
            for h in range(0, R, rl):
                r0 = b * T + c * R + h
                t += [(None if c0 is None else c0 + cp * c - (R - rl - h) * cp / R, ("S", r0, rl))]
        return t

    def Pt(b, c0, cp):
        return [(None if c0 is None else c0 + cp * c + o["ps"] * j, ("P", b, c, j))
                for c in range(NC) for j in range(NT)]

    def C(b, c0, cp):
        return LS(b, c0, cp, o["rl"]) + Pt(b, c0 + o["po"], cp)

    def WS(g, d):
        return [(None if d is None else d - 5 * (3 - i), ("WS", g, 32 * i, 32 * i + 32)) for i in range(4)]

    def X(ga, na, gb, nb, b):
        return [("X", ga, na, gb, nb, b, i) for i in range(len(PROD))]

    sh = lambda ts, d: [(None if t is None else t + d, it) for t, it in ts]
    allj = tuple(range(NT))
    p = Plan()
    p.wait("x0a")
    p.tasks(parts("A", 0, (None,)) + parts("A", 1, (None,)))
    p.flush()
    p.wait("wqa")
    p.tasks([(None, ("perm", 0, 0, KA, allj))])
    p.mxu(Q(0, 0))
    p.wait("x0b", "wqb")
    p.tasks([(None, ("perm", 0, KA, D, allj))] + parts("A", 2, (None,)))
    p.flush()
    p.tasks(WS(0, o["ws"][0]))
    p.mxu(Q(1, 0) + Q(0, 1) + Q(1, 1) + Q(2, 0))
    p.flush()
    p.wait("wk")
    p.tasks([(None, ("perm", 1, 0, D, (j,))) for j in range(NT)] + LS(0, None, 0) + WS(1, o["ws"][1]))
    p.mxu(Q(2, 1) + M(1, 0) + M(1, 1))
    p.flush()
    p.wait("wv")
    p.tasks([(o["pv"][0] + o["pv"][1] * j, ("perm", 2, 0, D, (j,))) for j in range(NT)]
            + LS(1, *o["l1"]) + Pt(0, *o["p0"]) + WS(2, o["ws"][2]))
    p.mxu(M(1, 2) + M(2, 0) + M(2, 1))
    p.flush()
    p.wait("wo", "wr", "x1")
    p.tasks([(None, ("permo", n)) for n in range(NT)])
    p.tasks(Pt(1, *o["p1"]) + parts("A", 3, o["a3"]) + parts("A", 4, o["a4"]) + parts("E", 0, o["e0"])
            + [(None, ("T", 3, 0, T)), (None, ("WS", 3, 0, T))])
    p.mxu(M(2, 2) + M(3, 0))
    for b in range(1, NS - 4, 2):
        nb = b + 2
        qk = X(0, 0, 0, 2, nb) + X(0, 1, 0, 3, nb) + X(0, 4, 1, 4, nb) + X(1, 0, 1, 2, nb) + X(1, 1, 1, 3, nb)
        v = X(2, 0, 2, 2, nb) + M(2, nb)[4:] + X(2, 1, 2, 3, nb) + M(2, nb + 1)[4:]
        segs = (M(3, b - 1) + qk + M(3, b) if b > 1 else M(3, b) + qk) + v
        e1, e2, a1, a2, p1, c2, l1 = [o["per"][b][i:i + 2] for i in range(0, 14, 2)]
        tasks = parts("E", b - 1, e1) + Pt(b, *p1) if b > 1 else []
        tasks += parts("E", b, e2) + C(b + 1, *c2) + parts("A", b + 4, a1)
        if b + 5 < NS:
            tasks += parts("A", b + 5, a2) + parts("T", b + 4, (None, None))
            tasks += sh(LS(b + 2, *l1, o["rl"]), sum(_slots(sg) for sg in segs) - 60)
        else:
            tasks += LS(b + 2, *o["l13"], o["rl"])
        if b == XB:
            late = [t for t in tasks if t[1][0] in "AT"]
            p.tasks([t for t in tasks if t not in late])
            base = p.pos
            p.mxu(segs[:o["xp"]])
            p.due(p.pos + o["xl"])
            p.flush(lambda it: it[0] in "AT" or it[0] == "E" and it[1] < XB - 1)
            assert ("e", (XB - 1) * T - R) in p.have
            p.wait("x2", "ffn")
            p.prog.append(("out", 0, (XB - 1) * T))
            p.tasks(sh(late, base - p.pos))
            p.mxu(segs[o["xp"]:])
        else:
            p.tasks(tasks)
            p.mxu(segs)
    p.tasks(Pt(NS - 3, *o["p13"]) + parts("E", NS - 4, o["e12"]))
    p.mxu(M(3, NS - 4))
    s = NS - 2
    big = M(3, s - 1) + M(0, s + 1) + M(1, s + 1) + M(3, s) + M(2, s + 1)
    small = [("G", k, n) for n in range(F // 128) for k in range(2)]
    cut = o["cut"]
    segs = []
    n_big, n_small, done = len(big) - o["sp"], len(small) - o["gh"], 0
    for g, sg in enumerate(big):
        segs.append(sg)
        if g >= o["sp"]:
            want = min(n_small, -(-(g - o["sp"] + 1) * n_small // n_big))
            segs += small[done:want]
            done = want
    segs += small[done:] + M(3, s + 1, 0, cut) + M(3, s + 1, cut, T) + [("H", n) for n in range(NT)]
    p.tasks(parts("E", s - 1, o["e13"]) + [(None, ("spec",))] + C(s, *o["c14"])
            + LS(s + 1, *o["l15"]) + Pt(s + 1, None, 0) + parts("E", s, o["e14"])
            + [(o["e15"], ("E", s + 1, 0, cut)), (None, ("E", s + 1, cut, T))])
    p.mxu(segs)
    p.flush()
    return p.prog


SCHED = dict(
    rl=8, ps=3, po=2, fq=16, ws=(50, 60, None), pv=(25, 14), l1=(52, 8), p0=(94, 3.75),
    p1=(42, 5.0), a3=(47,), a4=(82,), e0=(148, 180), xp=14, xl=32,
    per={1: (0, 0, 270, 298, 140, 169, 187, 217, 0, 0, 32, 27.0, 80, 18.0),
         3: (80, 112, 266, 308, 140, 177, 195, 217, 22, 18.5, 168, 16.5, 80, 19.0),
         5: (80, 112, 254, 308, 140, 173, 183, 217, 18, 19.0, 160, 16.0, 80, 19.0),
         7: (80, 112, 262, 308, 140, 167, 187, 217, 10, 20.0, 160, 16.0, 80, 19.0),
         9: (80, 112, 278, 308, 140, 167, 191, 229, 18, 19.0, 168, 16.0, 72, 18.25),
         11: (82, 112, 272, 308, 140, 169, 195, 215, 22, 19.0, 168, 16.0, 79, 19.0)},
    l13=(231, 9.0), p13=(0, 5.0), e12=(72, 100),
    cut=64, sp=12, gh=6, e13=(89, 106), c14=(2, 12.75), l15=(156, 5.5), e14=(218, 237), e15=243)


def make_kernel():
    o = SCHED
    prog = build_program(o)
    x1 = (XB + 1) * T
    xch = (2 * T, T, x1, S - 3 * T - x1)

    def kernel(x_hbm, wqkv_hbm, wo_hbm, wr_hbm, wg_hbm, wu_hbm, wd_hbm, out_hbm,
               x_s, wqkv_s, wo_s, wob_s, wr_s, wg_s, wu_s, wd_s, wp_s, ws_s, ts_s,
               k_s, v_s, xn_s, o_s, out_s, y_s, act_s, sem_in, sem_out):
        pid = pl.program_id(0)
        step = pid - 1
        cp = {}
        semi = dict(x0a=0, wqa=1, x0b=6, wqb=6, wk=2, wv=3, wo=4, wr=4, x1=4, x2=5, ffn=5)
        r0 = 0
        for nm, n in zip(("x0a", "x0b", "x1", "x2"), xch):
            cp[nm] = [pltpu.make_async_copy(x_hbm.at[pl.ds(r0, n)], x_s.at[pl.ds(r0, n)], sem_in.at[semi[nm]])]
            r0 += n
        for nm, lo, hi, g in (("wqa", 0, KA, 0), ("wqb", KA, D, 0), ("wk", 0, D, 1), ("wv", 0, D, 2)):
            sl = (pl.ds(lo, hi - lo), pl.ds(D * g, D))
            cp[nm] = [pltpu.make_async_copy(wqkv_hbm.at[sl], wqkv_s.at[sl], sem_in.at[semi[nm]])]
        cp["wo"] = [pltpu.make_async_copy(wo_hbm, wob_s, sem_in.at[semi["wo"]])]
        cp["wr"] = [pltpu.make_async_copy(wr_hbm, wr_s, sem_in.at[semi["wr"]])]
        cp["ffn"] = [pltpu.make_async_copy(a, b, sem_in.at[semi["ffn"]])
                     for a, b in ((wg_hbm, wg_s), (wu_hbm, wu_s), (wd_hbm, wd_s))]

        def ocp(lo, hi):
            return pltpu.make_async_copy(out_s.at[pl.ds(lo, hi - lo)], out_hbm.at[pl.ds(lo, hi - lo)],
                                         sem_out.at[0 if lo < LATE else 1])

        def start_all():
            for nm in ("x0a", "wqa", "x0b", "wqb", "wk", "wv", "wo", "wr", "x1", "x2", "ffn"):
                for c in cp[nm]:
                    c.start()

        def main():
            zero = jnp.zeros((HALO, 128), F32)
            for j in range(NT):
                k_s[j, 0:HALO, :] = zero
                v_s[j, 0:HALO, :] = zero

            lane = lax.broadcasted_iota(jnp.int32, (1, 128), 1)
            cm5 = [(lane + 128 * t) - 5 * (((lane + 128 * t) * 52429) >> 18) for t in range(NT - 1)]
            srcs = [(20 * (lane & 31) + 5 * (lane >> 5) + j) & 127 for j in range(NT)]
            never = jnp.full((8, 128), step, jnp.int32) > 0
            st = dict(best=None, toks=[], wr=None)
            q, hh, sm, gu, part = {}, {}, {}, {}, {}
            pack = lambda v: pltpu.bitcast(v.astype(BF16), U32)
            rsqrt = lambda v: jnp.exp2(jnp.log(v) * (-0.5 / math.log(2.0)))

            def token(due, u):
                if due is not None:
                    st["toks"].append((due, u()))

            def mm(lhs, w, span):
                start, end = span
                toks = [t for t in st["toks"] if t[0] < end]
                st["toks"] = [t for t in st["toks"] if t[0] >= end]
                if toks:
                    ng = lhs.shape[0] // 8
                    grp = lambda d: min(max(int(d - start), 0), ng - 1)
                    col, pos = [], 0
                    for i in sorted({grp(d) for d, _ in toks}):
                        tok = functools.reduce(jnp.bitwise_or, [t for d, t in toks if grp(d) == i])
                        col += [lhs[pos:8 * i, 0:128]] if 8 * i > pos else []
                        col.append(jnp.where(never, tok, lhs[8 * i:8 * i + 8, 0:128]))
                        pos = 8 * i + 8
                    col += [lhs[pos:, 0:128]] if pos < 8 * ng else []
                    col = jnp.concatenate(col, axis=0)
                    lhs = jnp.concatenate([col, lhs[:, 128:]], axis=1) if lhs.shape[1] > 128 else col
                if w.dtype == U32:
                    w = pltpu.bitcast(w, BF16)
                return jnp.dot(pltpu.bitcast(lhs, BF16), w, preferred_element_type=F32)

            def permute_w(g, k0, k1, js, due):
                if ("mw", g, k0) not in st:
                    tiles = [pltpu.bitcast(wqkv_s[pl.ds(k0, k1 - k0), pl.ds(D * g + 128 * t, 128)], U32)
                             for t in range(NT)]
                    st["mw", g, k0] = []
                    for j in range(NT):
                        m = tiles[NT - 1]
                        for t in range(NT - 2, -1, -1):
                            m = jnp.where(cm5[t] == j, tiles[t], m)
                        st["mw", g, k0].append(m)
                for j in js:
                    m = st["mw", g, k0][j]
                    res = jnp.take_along_axis(m, jnp.broadcast_to(srcs[j], m.shape), axis=1,
                                              mode="promise_in_bounds")
                    wp_s[pl.ds(k0 // 2, (k1 - k0) // 2), pl.ds(D * g + 128 * j, 128)] = res
                    token(due, lambda: _or_all(res))

            def permute_wo(n, due):
                wo_s[n, pl.ds(0, D // 2), :] = pltpu.bitcast(wob_s[:, pl.ds(128 * n, 128)], U32)
                for d2 in range(DH // 2):
                    ev = wo_s[n, pl.ds(d2, H // 2, stride=DH), :]
                    od = wo_s[n, pl.ds(DH // 2 + d2, H // 2, stride=DH), :]
                    lo = (ev & jnp.uint32(0xFFFF)) | (od << 16)
                    hi = (ev >> 16) | (od & jnp.uint32(0xFFFF0000))
                    for d, val in ((2 * d2, lo), (2 * d2 + 1, hi)):
                        aa, j = divmod(d, NT)
                        wp_s[pl.ds(64 * j + 16 * aa, H // 2), pl.ds(3 * D + 128 * n, 128)] = val

            def sums(blocks, combos):
                un = [pltpu.bitcast(u, BF16).astype(F32) for u in blocks]
                return [pack(un[x] + un[y] if sg > 0 else un[x] - un[y]) for x, sg, y in combos]

            def ws_task(g, lo, hi, due):
                cols = [pl.ds(D * j + 512, 128) if g == 3 else pl.ds(D * g + 256 * j, 256) for j in range(2)]
                b = [wp_s[pl.ds(128 * i + lo, hi - lo), cols[j]] for i in range(2) for j in range(2)]
                res = sums(b, ((0, 1, 3), (1, -1, 3), (2, -1, 0), (0, 1, 1), (2, 1, 3)))
                dst = lambda i: (pl.ds((5 * g + i) * 128 + lo, hi - lo), pl.ds(0, 128 if g == 3 else 256))
                for i, v in enumerate(res):
                    ws_s[dst(i)] = v
                token(due, lambda: _or_all(jnp.concatenate([ws_s[dst(i)] for i in range(5)], axis=0)))

            def t_task(b, lo, hi, due):
                a = [xn_s[pl.ds(((b + i) * T + lo) // 2, (hi - lo) // 2), pl.ds(256 * j, 256)]
                     for i in range(2) for j in range(2)]
                for i, v in enumerate(sums(a, ((0, 1, 3), (2, 1, 3), (0, 1, 1), (2, -1, 0), (1, -1, 3)))):
                    ts_s[pl.ds((5 * (b // 2) + i) * 64 + lo // 2, (hi - lo) // 2), :] = v

            def a_task(b, lo, hi, due):
                r0, n = b * T + lo, hi - lo
                x = x_s[pl.ds(r0, n), :].astype(F32)
                m = jnp.sum(x, axis=-1, keepdims=True) * (1.0 / D)
                c = x - m
                v = jnp.sum(c * c, axis=-1, keepdims=True) * (1.0 / D)
                xn_s[pl.ds(r0 // 2, n // 2), :] = pack(c * rsqrt(v + EPS))
                token(due, lambda: _or_all(xn_s[pl.ds(r0 // 2, n // 2), :]))

            def finish(g, b, n, lo, hi, acc, due):
                r0 = b * T + lo
                if g == 0:
                    acc = acc * QSCALE
                elif g == 3:
                    acc = acc + x_s[pl.ds(r0, hi - lo), pl.ds(128 * n, 128)].astype(F32)
                token(due, lambda: _or_all(acc))
                if g == 0:
                    q[b, n] = acc
                elif g == 3:
                    hh[b, n, lo, hi] = acc
                else:
                    (k_s if g == 1 else v_s)[n, pl.ds(HALO + r0, hi - lo), :] = acc

            def m_seg(g, b, n, lo, hi, span):
                src = o_s if g == 3 else xn_s
                acc = mm(src[pl.ds((b * T + lo) // 2, (hi - lo) // 2), :],
                         wp_s[:, pl.ds(D * g + 128 * n, 128)], span)
                finish(g, b, n, lo, hi, acc, span[1] + o["fq"] if g == 0 else None)

            def q_seg(b, n, kpart, span):
                k0, k1 = ((0, KA), (KA, D))[kpart]
                acc = mm(xn_s[pl.ds(b * T // 2, T // 2), pl.ds(k0, k1 - k0)],
                         wp_s[pl.ds(k0 // 2, (k1 - k0) // 2), pl.ds(128 * n, 128)], span)
                if kpart == 0:
                    part[b, n] = acc
                else:
                    finish(0, b, n, 0, T, acc + part.pop((b, n)), None)

            def x_seg(ga, na, gb, nb, b, i, span):
                blk = lambda bb, c0, w: xn_s[pl.ds(bb * T // 2, T // 2), pl.ds(c0, w)]
                ca, cb = D * ga + 128 * na, D * gb + 128 * nb
                wb = lambda r, c: wp_s[pl.ds(r, 128 if r < 256 else 64), pl.ds(c, 128)]
                ln, li, rn, ri, _ = PROD[i]
                ss = lambda: ts_s[pl.ds((5 * (b // 2) + li) * 64, 64), :]
                wg, wn = (ga, na) if ga == gb else (3, 0)
                tt = lambda: ws_s[pl.ds((5 * wg + ri) * 128, 128), pl.ds(128 * wn, 128)]
                lhs = {"s": ss, "a11": lambda: blk(b, 0, 256), "a22": lambda: blk(b + 1, 256, 256),
                       "top4": lambda: blk(b, 512, 128), "bot4": lambda: blk(b + 1, 512, 128),
                       "s7": lambda: jnp.concatenate([ss(), blk(b, 512, 128)], axis=1),
                       "s6": lambda: jnp.concatenate([ss(), blk(b + 1, 512, 128)], axis=1)}[ln]()
                rhs = {"t": tt, "b11": lambda: wb(0, ca), "b22": lambda: wb(128, cb),
                       "w4a": lambda: wb(256, ca), "w4b": lambda: wb(256, cb),
                       "t7": lambda: jnp.concatenate([tt(), wb(256, ca)], axis=0),
                       "t6": lambda: jnp.concatenate([tt(), wb(256, cb)], axis=0)}[rn]()
                m = mm(lhs, rhs, span)
                due = lambda g: span[1] + o["fq"] if g == 0 else None
                c = part.setdefault((ga, na, b), {})
                if i == 0:
                    c[11] = c[22] = m
                elif i == 1:
                    c[11], c[21] = c[11] + m, m
                elif i == 2:
                    c[11], c[12] = c[11] - m, m
                elif i == 3:
                    finish(ga, b, na, 0, T, c.pop(11) + m, due(ga))
                elif i == 4:
                    c[21], c[22] = c[21] + m, c[22] - m
                elif i == 5:
                    finish(ga, b + 1, na, 0, T, c.pop(21) + m, due(ga))
                elif i == 6:
                    c[12], c[22] = c[12] + m, c[22] + m
                elif i == 7:
                    finish(gb, b, nb, 0, T, c.pop(12) + m, due(gb))
                else:
                    finish(gb, b + 1, nb, 0, T, c.pop(22) + m, due(gb))

            def s_task(r0, n, due):
                b, r = divmod(r0, T)
                qc = jnp.stack([q[b, j][r:r + n] for j in range(NT)])
                lg = jnp.stack([jnp.sum(qc * k_s[:, pl.ds(HALO + r0 - DIL * w, n), :], axis=0)
                                for w in range(W)])
                lg = lg + pltpu.roll(lg, 64, 2)
                lg = lg + pltpu.roll(lg, 32, 2)
                if r0 < DIL * (W - 1):
                    pos = (lax.broadcasted_iota(jnp.int32, lg.shape, 1) + r0
                           - DIL * lax.broadcasted_iota(jnp.int32, lg.shape, 0))
                    lg = jnp.where(pos >= 0, lg, -1e9)
                e = jnp.exp2(lg - _fold(jnp.maximum, lg))
                inv = pl.reciprocal(_fold(jnp.add, e), approx=True)
                sm[r0] = (e, inv)
                token(due, lambda: _or_all(inv[0]))

            def p_task(b, c, j, due):
                r0 = b * T + c * R
                if ("pv", r0) not in st:
                    e, inv = sm.pop(r0)
                    if r0 + 8 in sm:
                        e2, inv2 = sm.pop(r0 + 8)
                        e, inv = jnp.concatenate([e, e2], axis=1), jnp.concatenate([inv, inv2], axis=1)
                    acc = None
                    for w in range(W):
                        t = e[w:w + 1] * v_s[:, pl.ds(HALO + r0 - DIL * w, R), :]
                        acc = t if acc is None else acc + t
                    st["pv", r0] = acc * inv
                dst = (pl.ds(r0 // 2, R // 2), pl.ds(128 * j, 128))
                o_s[dst] = pack(st["pv", r0][j])
                token(due, lambda: o_s[dst])

            def e_task(b, lo, hi, due):
                r0, n = b * T + lo, hi - lo
                if st["wr"] is None:
                    st["wr"] = wr_s[...].astype(F32).reshape(1, D)
                (l0, h0), = {k[2:] for k in hh if k[0] == b and k[2] <= lo and hi <= k[3]}
                h = jnp.concatenate([hh[b, j, l0, h0][lo - l0:hi - l0] for j in range(NT)], axis=1)
                m = jnp.sum(h, axis=-1, keepdims=True) * (1.0 / D)
                c = h - m
                v = jnp.sum(c * c, axis=-1, keepdims=True) * (1.0 / D)
                cw = jnp.sum(c * st["wr"], axis=-1, keepdims=True)
                rstd = rsqrt(v + EPS)
                out_s[pl.ds(pl.multiple_of(step * 16 + r0, 16), n), :] = (c * (1.0 + rstd) + m).astype(BF16)
                r, mb, rb = [jnp.broadcast_to(t, (n, 128)) for t in (cw * rstd, m, rstd)]
                best = st["best"]
                for i in range(n // 8):
                    ri = r[8 * i:8 * i + 8]
                    new = (ri, lax.broadcasted_iota(jnp.int32, (8, 128), 0) + (r0 + 8 * i),
                           mb[8 * i:8 * i + 8], rb[8 * i:8 * i + 8])
                    if best is None:
                        best = (jnp.where(ri > -jnp.inf, ri, -jnp.inf),) + new[1:]
                    else:
                        upd = ri > best[0]
                        best = tuple(jnp.where(upd, a, c_) for a, c_ in zip(new, best))
                st["best"] = best
                if b == NS - 1:
                    ocp(r0, r0 + n).start()
                elif hi == T and b >= XB - 1:
                    ocp(b * T, (b + 1) * T).start()
                token(due, lambda: functools.reduce(jnp.bitwise_or, [pltpu.bitcast(t, U32) for t in best])
                      | pltpu.bitcast(out_s[0:16, 0:128], U32))

            def spec_task(due):
                st["xs"] = load_chunk(st["best"], LATE)

            def g_seg(k, n, span):
                gu[k, n] = jnp.dot(st["xs"], (wg_s, wu_s)[k][:, pl.ds(128 * n, 128)],
                                   preferred_element_type=F32)

            def h_seg(n, span):
                if "act" not in st:
                    g = jnp.concatenate([gu[0, i] for i in range(F // 128)], axis=1)
                    u = jnp.concatenate([gu[1, i] for i in range(F // 128)], axis=1)
                    act_s[...] = pack(g * jax.nn.sigmoid(g) * u)
                    st["act"] = True
                y_s[:, pl.ds(128 * n, 128)] = mm(act_s[...], wd_s[:, pl.ds(128 * n, 128)], span)

            def do_wait(nm):
                st["toks"] = []
                for c in cp[nm]:
                    c.wait()

            fns = dict(A=a_task, T=t_task, WS=ws_task, M=m_seg, Q=q_seg, X=x_seg, S=s_task, P=p_task,
                       E=e_task, perm=permute_w, permo=permute_wo, spec=spec_task, G=g_seg, H=h_seg,
                       wait=do_wait, out=lambda lo, hi: ocp(lo, hi).start())
            for item in prog:
                fns[item[0]](*item[1:])
            return st["best"]

        def argmax(best):
            bv, bi = best[:2]
            mx = jnp.max(bv, axis=0, keepdims=True)
            idx = jnp.min(jnp.where(bv >= mx, bi, S - 1), axis=0, keepdims=True)
            return mx[:, 0:1], idx

        def load_chunk(best, nrows):
            idx = argmax(best)[1]
            m, rstd = [jnp.sum(jnp.where(best[1] == idx, t, 0.0), axis=0, keepdims=True)[:, 0:1] for t in best[2:]]
            blk = jnp.clip(idx[0, 0] >> 4, 0, nrows // 16 - 1)
            cur = out_s[pl.ds(pl.multiple_of(blk * 16, 16), 16), :].astype(F32)
            return ((cur - m) * (rstd / (1.0 + rstd))).astype(BF16)

        def fix_row(mx, idx, nrows):
            base = pl.multiple_of(jnp.clip(idx >> 4, 0, nrows // 16 - 1) * 16, 16)
            y = y_s[...] * jax.nn.sigmoid(mx)
            cur = out_s[pl.ds(base, 16), :].astype(F32)
            rows = lax.broadcasted_iota(jnp.int32, (16, D), 0) + base
            out_s[pl.ds(base, 16), :] = jnp.where(rows == idx, cur + y, cur).astype(BF16)
            fix = pltpu.make_async_copy(out_s.at[pl.ds(base, 16)], out_hbm.at[pl.ds(base, 16)], sem_out.at[2])
            fix.start()
            return fix

        def tail(best):
            mx, idx = argmax(best)
            idx = jnp.clip(idx[0, 0], 0, S - 1)
            ocp(0, LATE).wait()

            def early():
                fix = fix_row(mx, idx, LATE)
                ocp(LATE, S).wait()
                fix.wait()

            def late():
                xs = load_chunk(best, S)
                g = jnp.dot(xs, wg_s[...], preferred_element_type=F32)
                u = jnp.dot(xs, wu_s[...], preferred_element_type=F32)
                act = (g * jax.nn.sigmoid(g) * u).astype(BF16)
                y_s[...] = jnp.dot(act, wd_s[...], preferred_element_type=F32)
                ocp(LATE, S).wait()
                fix_row(mx, idx, S).wait()

            lax.cond(idx < LATE, early, late)

        pl.when(pid == 0)(start_all)

        @pl.when(pid == 1)
        def _():
            tail(main())

    @jax.jit
    def fn(A_x, A_wqkv, A_wo, B_x, B_w_r, B_w_gate, B_w_up, B_w_down):
        any_spec = pl.BlockSpec(memory_space=pl.ANY)
        out = pl.pallas_call(
            kernel,
            grid=(2,),
            out_shape=jax.ShapeDtypeStruct((S, D), BF16),
            in_specs=[any_spec] * 7,
            out_specs=any_spec,
            scratch_shapes=[
                pltpu.VMEM((S, D), BF16),
                pltpu.VMEM((D, 3 * D), BF16),
                pltpu.VMEM((NT, D // 2 + 32, 128), U32),
                pltpu.VMEM((D, D), BF16),
                pltpu.VMEM((D,), BF16),
                pltpu.VMEM((D, F), BF16),
                pltpu.VMEM((D, F), BF16),
                pltpu.VMEM((F, D), BF16),
                pltpu.VMEM((D // 2, 4 * D), U32),
                pltpu.VMEM((20 * 128, 256), U32),
                pltpu.VMEM((NS // 2 * 5 * 64, 256), U32),
                pltpu.VMEM((NT, S + HALO, 128), F32),
                pltpu.VMEM((NT, S + HALO, 128), F32),
                pltpu.VMEM((S // 2, D), U32),
                pltpu.VMEM((S // 2, D), U32),
                pltpu.VMEM((S + 16, D), BF16),
                pltpu.VMEM((16, D), F32),
                pltpu.VMEM((8, F), U32),
                pltpu.SemaphoreType.DMA((7,)),
                pltpu.SemaphoreType.DMA((3,)),
            ],
            compiler_params=pltpu.CompilerParams(vmem_limit_bytes=100 << 20,
                                                 dimension_semantics=("arbitrary",),
                                                 disable_bounds_checks=True,
                                                 disable_semaphore_checks=True),
            name="fused",
        )(A_x.reshape(S, D), A_wqkv, A_wo, B_w_r, B_w_gate, B_w_up, B_w_down)
        return out.reshape(1, S, D)

    return fn


pallas_sequential_preLN__sliding_local_dilated__moe_arch_mod__prompt_kernel = make_kernel()
```
